```python
import jax
import jax.numpy as jnp

def _softmax(x, axis=-1):
    return jax.nn.softmax(x, axis=axis)
def _gelu(x):
    return jax.nn.gelu(x, approximate=True)
def _silu(x):
    return jax.nn.silu(x)
def _sigmoid(x):
    return jax.nn.sigmoid(x)
def _layernorm(x, axis=-1, eps=1e-5):
    m = jnp.mean(x, axis=axis, keepdims=True)
    v = jnp.var(x, axis=axis, keepdims=True)
    return (x - m) / jnp.sqrt(v + eps)
def _scatter_add(tgt, idx, src, axis=0):
    return tgt.at[idx].add(src)
def _segment_sum(src, seg, n):
    return jax.ops.segment_sum(src, seg, n)
class _Rng:
    def __init__(self, key):
        self._k = key
    def _next(self):
        self._k, sub = jax.random.split(self._k)
        return sub
    def normal(self, shape):
        return jax.random.normal(self._next(), shape, dtype=jnp.bfloat16)
    def randint(self, lo, hi, shape):
        return jax.random.randint(self._next(), shape, lo, hi, dtype=jnp.int32)
    def uniform(self, shape, lo=0.0, hi=1.0):
        return jax.random.uniform(self._next(), shape, jnp.bfloat16, lo, hi)
    def permutation(self, n):
        return jax.random.permutation(self._next(), n)


kernel_name = 'recurrent_scan__sliding_local_dilated__moe_arch_mod__prompt'

def setup_inputs():
    _rng = _Rng(jax.random.key(int.from_bytes(__import__("os").urandom(4), "little")))
    _w = (lambda a: (lambda t: t.astype(jnp.bfloat16) if jnp.issubdtype(t.dtype, jnp.floating) else t)(jnp.asarray(a)))
    def _A_setup():
        B, S, D = 1, 2048, 640
        return {
            "x": _w((lambda *s: _rng.normal(s) * 0.05)(B, S, D)),
            "wqkv": _w((lambda *s: _rng.normal(s) * 0.05)(D, 3 * D)),
            "wo": _w((lambda *s: _rng.normal(s) * 0.05)(D, D)),
        }
    _A_in = _A_setup()

    def _B_setup():
        B, S, D, F, C = 1, 2048, 640, 1728, 2
        return {
            "x": _w((lambda *s: _rng.normal(s) * 0.05)(B, S, D)),
            "w_r": _w((lambda *s: _rng.normal(s) * 0.05)(D)),
            "w_gate": _w((lambda *s: _rng.normal(s) * 0.05)(D, F)),
            "w_up": _w((lambda *s: _rng.normal(s) * 0.05)(D, F)),
            "w_down": _w((lambda *s: _rng.normal(s) * 0.05)(F, D)),
        }
    _B_in = _B_setup()

    return {
        "A_x": _A_in["x"],
        "A_wqkv": _A_in["wqkv"],
        "A_wo": _A_in["wo"],
        "B_x": _B_in["x"],
        "B_w_r": _B_in["w_r"],
        "B_w_gate": _B_in["w_gate"],
        "B_w_up": _B_in["w_up"],
        "B_w_down": _B_in["w_down"],
    }

def reference(A_x, A_wqkv, A_wo, B_x, B_w_r, B_w_gate, B_w_up, B_w_down):
    def _A_ref(x, wqkv, wo):
        B, S, D = x.shape
        H = 32; Dh = D // H
        W, dil = 8, 2
        qkv = (lambda x, *d: x.transpose(*d))((x @ wqkv).reshape(B, S, 3, H, Dh), 2, 0, 3, 1, 4)
        q, k, v = qkv[0], qkv[1], qkv[2]
        scale = Dh ** -0.5
        pos = jnp.arange(S)
        off = jnp.arange(W) * dil
        idx = pos[:, None] - off[None, :]
        mask = idx >= 0
        idx_c = jnp.where(mask, idx, 0).reshape(-1)
        kg = k[:, :, idx_c, :].reshape(B, H, S, W, Dh)
        vg = v[:, :, idx_c, :].reshape(B, H, S, W, Dh)
        logits = jnp.einsum("bhsd,bhswd->bhsw", q, kg) * scale
        logits = jnp.where(mask[None, None, :, :], logits, -1e9)
        attn = _softmax(logits, axis=-1)
        o = jnp.einsum("bhsw,bhswd->bhsd", attn, vg)
        return (lambda x, *d: x.transpose(*d))(o, 0, 2, 1, 3).reshape(B, S, D) @ wo

    def _B_ref(x, w_r, w_gate, w_up, w_down):
        B, S, D = x.shape
        C = 2
        r = x @ w_r
        idx = jnp.argsort(-r, axis=-1)[:, :C]
        idx_e = jnp.repeat(idx.reshape(B, C, 1), D, axis=2)
        x_sel = jnp.take_along_axis(x, idx_e, axis=1)
        g = _silu(x_sel @ w_gate)
        u = x_sel @ w_up
        y = (g * u) @ w_down
        r_sel = _sigmoid(jnp.take_along_axis(r, idx, axis=1))
        y = y * r_sel.reshape(B, C, 1)
        b_off = (jnp.arange(B) * S).reshape(B, 1)
        flat_idx = (idx + b_off).reshape(B * C)
        zero = (x * 0.0).reshape(B * S, D)
        upd = _scatter_add(zero, flat_idx, y.reshape(B * C, D), axis=0)
        return x + upd.reshape(B, S, D)

    x = A_x
    xn = _layernorm(x, axis=-1)
    s = _A_ref(xn, A_wqkv, A_wo)
    g = _silu(_B_ref(xn, B_w_r, B_w_gate, B_w_up, B_w_down))
    return x + s * g
```

```python
import functools
import math

import jax
import jax.numpy as jnp
import numpy as np
from jax import lax
from jax.experimental import pallas as pl
from jax.experimental.pallas import tpu as pltpu

S, D, F = 2048, 640, 1728
H, DH, W, DIL = 32, 20, 8, 2
NT = D // 128
HALO = 16
LOG2E = math.log2(math.e)
QSCALE = DH ** -0.5 * LOG2E
NEG = -1e9 * LOG2E
EPS_BF16 = float(np.asarray(1e-5, dtype=jnp.bfloat16).astype(np.float32))
f32, bf16, i32 = jnp.float32, jnp.bfloat16, jnp.int32


def _rb(x):
    return x.astype(bf16).astype(f32)


def make_kernel(T=256, G=16, LNG=32):
    NB = S // T

    def kernel(x_hbm, wqkv_hbm, wo_hbm, wr_ref, wg_hbm, wu_hbm, wd_hbm, out_hbm,
               x_v, xn_v, wqkv_raw, wqkv_p, wo_raw, wo_f, wo_p, wg_v, wu_v, wd_v,
               q_a, q_b, k_a, k_b, v_a, v_b, o_v, out_v, sem_x, sem_w, sem_o):
        def x_copy(i):
            return pltpu.make_async_copy(x_hbm.at[pl.ds(i * T, T), :], x_v.at[pl.ds(i * T, T), :], sem_x.at[i])

        w_copies = [pltpu.make_async_copy(s, d, sem_w.at[j]) for j, (s, d) in enumerate(
            [(wqkv_hbm, wqkv_raw), (wo_hbm, wo_raw), (wg_hbm, wg_v), (wu_hbm, wu_v), (wd_hbm, wd_v)])]

        x_copy(0).start()
        w_copies[0].start()
        for i in range(1, NB):
            x_copy(i).start()
        for c in w_copies[1:]:
            c.start()

        lane = lax.broadcasted_iota(i32, (8, 128), 1)
        sub = lax.broadcasted_iota(i32, (8, 128), 0)

        wr = wr_ref[...].astype(f32).reshape(1, D)

        def ln_block(i, r_acc):
            x_copy(i).wait()
            for g in range(T // LNG):
                r0 = pl.multiple_of(i * T + g * LNG, LNG)
                x = x_v[pl.ds(r0, LNG), :].astype(f32)
                m = jnp.sum(x, axis=1, keepdims=True) * (1.0 / D)
                c = x - m
                var = jnp.sum(c * c, axis=1, keepdims=True) * (1.0 / D)
                den = _rb(jnp.sqrt(_rb(_rb(var) + EPS_BF16)))
                xn = (_rb(x - _rb(m)) * (1.0 / den)).astype(bf16)
                xn_v[pl.ds(r0, LNG), :] = xn
                r = jnp.sum(xn.astype(f32) * wr, axis=1, keepdims=True)
                for s in range(LNG // 8):
                    gi = (i * T + g * LNG) // 8 + s
                    rs = jnp.broadcast_to(r[s * 8:(s + 1) * 8], (8, 128))
                    r_acc = (jnp.where(lane == gi, rs, r_acc[0]), jnp.where(lane == gi - 128, rs, r_acc[1]))
            return r_acc

        r_lo, r_hi = lax.fori_loop(0, NB, ln_block, (jnp.zeros((8, 128), f32), jnp.zeros((8, 128), f32)))

        w_copies[0].wait()
        for c in range(NT):
            col = 20 * (lane % 32) + 5 * (lane // 32) + c
            src_lane = col % 128
            tl = ((c - lane) * 2) % 5
            for p in range(3):
                for rb_ in range(D // 16):
                    rows = pl.ds(rb_ * 16, 16)
                    tiles = [pltpu.bitcast(wqkv_raw[rows, pl.ds(p * D + t * 128, 128)], i32) for t in range(NT)]
                    sel = tiles[0]
                    for t in range(1, NT):
                        sel = jnp.where(tl == t, tiles[t], sel)
                    out = jnp.take_along_axis(sel, src_lane, axis=1, mode="promise_in_bounds")
                    wqkv_p[rows, pl.ds(p * D + c * 128, 128)] = pltpu.bitcast(out, bf16)

        def qkv(i, q_s, k_s, v_s):
            r0 = pl.multiple_of(i * T, T)
            res = jnp.dot(xn_v[pl.ds(r0, T), :], wqkv_p[...], preferred_element_type=f32)
            for c in range(NT):
                q_s[c] = res[:, c * 128:(c + 1) * 128] * QSCALE
                k_s[c, pl.ds(HALO, T), :] = res[:, D + c * 128:D + (c + 1) * 128]
                v_s[c, pl.ds(HALO, T), :] = res[:, 2 * D + c * 128:2 * D + (c + 1) * 128]

        def halo(k_dst, v_dst, k_src, v_src):
            for c in range(NT):
                k_dst[c, pl.ds(0, HALO), :] = k_src[c, pl.ds(T, HALO), :]
                v_dst[c, pl.ds(0, HALO), :] = v_src[c, pl.ds(T, HALO), :]

        def attn(i, q_s, k_s, v_s):
            for g in range(T // G):
                q = [q_s[c, pl.ds(g * G, G), :] for c in range(NT)]
                logits = []
                for w in range(W):
                    rows = pl.ds(HALO + g * G - DIL * w, G)
                    p = q[0] * k_s[0, rows, :]
                    for c in range(1, NT):
                        p = p + q[c] * k_s[c, rows, :]
                    p = p + pltpu.roll(p, 64, 1)
                    p = p + pltpu.roll(p, 32, 1)
                    if g * G < DIL * w:
                        pos = i * T + g * G + lax.broadcasted_iota(i32, (G, 128), 0)
                        p = jnp.where(pos >= DIL * w, p, NEG)
                    logits.append(p)
                m = functools.reduce(jnp.maximum, logits)
                e = [jnp.exp2(l - m) for l in logits]
                inv = 1.0 / functools.reduce(jnp.add, e)
                r0 = pl.multiple_of(i * T + g * G, G)
                for c in range(NT):
                    acc = e[0] * v_s[c, pl.ds(HALO + g * G, G), :]
                    for w in range(1, W):
                        acc = acc + e[w] * v_s[c, pl.ds(HALO + g * G - DIL * w, G), :]
                    o_v[pl.ds(r0, G), pl.ds(c * 128, 128)] = (acc * inv).astype(bf16)

        qkv(0, q_a, k_a, v_a)
        for c in range(NT):
            k_a[c, pl.ds(0, HALO), :] = jnp.broadcast_to(k_a[c, pl.ds(HALO, 1), :], (HALO, 128))
            v_a[c, pl.ds(0, HALO), :] = jnp.broadcast_to(v_a[c, pl.ds(HALO, 1), :], (HALO, 128))

        def pair(j, carry):
            i = 2 * j
            halo(k_b, v_b, k_a, v_a)
            qkv(i + 1, q_b, k_b, v_b)
            attn(i, q_a, k_a, v_a)
            halo(k_a, v_a, k_b, v_b)
            qkv(i + 2, q_a, k_a, v_a)
            attn(i + 1, q_b, k_b, v_b)
            return carry

        lax.fori_loop(0, NB // 2 - 1, pair, 0)
        halo(k_b, v_b, k_a, v_a)
        qkv(NB - 1, q_b, k_b, v_b)
        attn(NB - 2, q_a, k_a, v_a)
        attn(NB - 1, q_b, k_b, v_b)

        w_copies[1].wait()
        for t in range(NT):
            wo_f[t] = wo_raw[:, pl.ds(t * 128, 128)].astype(f32)
        for c in range(NT):
            for g in range(4):
                for t in range(NT):
                    blk = wo_f[t, pl.ds(5 * g + c, 32, stride=20), :]
                    wo_p[pl.ds(c * 128 + g * 32, 32), pl.ds(t * 128, 128)] = blk.astype(bf16)

        r_all = _rb(jnp.concatenate([r_lo, r_hi], axis=0))
        idx = jnp.concatenate([lane * 8 + sub, (lane + 128) * 8 + sub], axis=0).astype(f32)
        key = jnp.where(r_all == r_all, r_all, -jnp.inf)
        m1 = jnp.max(key, keepdims=True)
        i1 = jnp.min(jnp.where(key == m1, idx, float(S)), keepdims=True)
        key2 = jnp.where(idx == i1, -jnp.inf, key)
        m2 = jnp.max(key2, keepdims=True)
        i2 = jnp.min(jnp.where((key2 == m2) & (idx != i1), idx, float(S)), keepdims=True)
        rs1 = jnp.sum(jnp.where(idx == i1, r_all, 0.0), keepdims=True)
        rs2 = jnp.sum(jnp.where(idx == i2, r_all, 0.0), keepdims=True)
        t1 = i1.astype(i32)[0, 0]
        t2 = i2.astype(i32)[0, 0]
        row = lax.broadcasted_iota(i32, (16, D), 0)

        def tile_of(t):
            return pl.ds(pl.multiple_of((t // 16) * 16, 16), 16)

        def pick(t):
            return jnp.sum(jnp.where(row == t % 16, xn_v[tile_of(t), :].astype(f32), 0.0), axis=0, keepdims=True)

        xs = jnp.where(row == 0, pick(t1), pick(t2)).astype(bf16)
        for c in w_copies[2:]:
            c.wait()
        gate = _rb(lax.dot_general(xs, wg_v[...], (((1,), (1,)), ((), ())), preferred_element_type=f32))
        up = _rb(lax.dot_general(xs, wu_v[...], (((1,), (1,)), ((), ())), preferred_element_type=f32))
        hid = (_rb(gate * jax.nn.sigmoid(gate)) * up).astype(bf16)
        y = _rb(jnp.dot(hid, wd_v[...], preferred_element_type=f32))
        for t, yy, rs in ((t1, y[0:1], rs1), (t2, y[1:2], rs2)):
            upd = _rb(yy * _rb(jax.nn.sigmoid(rs)))
            z = xn_v[tile_of(t), :].astype(f32)
            xn_v[tile_of(t), :] = jnp.where(row == t % 16, z + upd, z).astype(bf16)

        def o_copy(i):
            r0 = pl.multiple_of(i * T, T)
            return pltpu.make_async_copy(out_v.at[pl.ds(r0, T), :], out_hbm.at[pl.ds(r0, T), :], sem_o.at[i])

        def fin(i, carry):
            r0 = pl.multiple_of(i * T, T)
            s = jnp.dot(o_v[pl.ds(r0, T), :], wo_p[...], preferred_element_type=f32)
            z = xn_v[pl.ds(r0, T), :].astype(f32)
            x = x_v[pl.ds(r0, T), :].astype(f32)
            gte = z * jax.nn.sigmoid(z)
            out_v[pl.ds(r0, T), :] = (x + s * gte).astype(bf16)
            o_copy(i).start()
            return carry

        lax.fori_loop(0, NB, fin, 0)
        for i in range(NB):
            o_copy(i).wait()

    scratch = [
        pltpu.VMEM((S, D), bf16),
        pltpu.VMEM((S, D), bf16),
        pltpu.VMEM((D, 3 * D), bf16),
        pltpu.VMEM((D, 3 * D), bf16),
        pltpu.VMEM((D, D), bf16),
        pltpu.VMEM((NT, D, 128), f32),
        pltpu.VMEM((D, D), bf16),
        pltpu.VMEM((F, D), bf16),
        pltpu.VMEM((F, D), bf16),
        pltpu.VMEM((F, D), bf16),
        pltpu.VMEM((NT, T, 128), f32),
        pltpu.VMEM((NT, T, 128), f32),
        pltpu.VMEM((NT, T + HALO, 128), f32),
        pltpu.VMEM((NT, T + HALO, 128), f32),
        pltpu.VMEM((NT, T + HALO, 128), f32),
        pltpu.VMEM((NT, T + HALO, 128), f32),
        pltpu.VMEM((S, D), bf16),
        pltpu.VMEM((S, D), bf16),
        pltpu.SemaphoreType.DMA((NB,)),
        pltpu.SemaphoreType.DMA((5,)),
        pltpu.SemaphoreType.DMA((NB,)),
    ]
    any_spec = pl.BlockSpec(memory_space=pltpu.HBM)
    return pl.pallas_call(
        kernel,
        out_shape=jax.ShapeDtypeStruct((S, D), bf16),
        in_specs=[any_spec, any_spec, any_spec, pl.BlockSpec(memory_space=pltpu.VMEM), any_spec, any_spec, any_spec],
        out_specs=any_spec,
        scratch_shapes=scratch,
        compiler_params=pltpu.CompilerParams(vmem_limit_bytes=100 * 1024 * 1024),
        name="fused",
    )


@jax.jit
def pallas_recurrent_scan__sliding_local_dilated__moe_arch_mod__prompt_kernel(
    A_x: jax.Array,
    A_wqkv: jax.Array,
    A_wo: jax.Array,
    B_x: jax.Array,
    B_w_r: jax.Array,
    B_w_gate: jax.Array,
    B_w_up: jax.Array,
    B_w_down: jax.Array,
):
    del B_x
    out = make_kernel()(A_x.reshape(S, D), A_wqkv, A_wo, B_w_r, B_w_gate.T, B_w_up.T, B_w_down)
    return out.reshape(1, S, D)
```

```python
import collections
import functools
import itertools
import math

import jax
import jax.numpy as jnp
import numpy as np
from jax import lax
from jax.experimental import pallas as pl
from jax.experimental.pallas import tpu as pltpu

S, D, F = 2048, 640, 1728
H, DH, W, DIL = 32, 20, 8, 2
NT = D // 128
HALO = 16
M = 128
NM = S // M
G = 16
NG = M // G
NSTAT = 32
NP = 8
PIECE = M * NT // 4
LOG2E = math.log2(math.e)
QSCALE = DH ** -0.5 * LOG2E
NEG = -1e9 * LOG2E
EPS_BF16 = float(np.asarray(1e-5, dtype=jnp.bfloat16).astype(np.float32))
f32, bf16, i32 = jnp.float32, jnp.bfloat16, jnp.int32
NT_DIMS = (((1,), (1,)), ((), ()))


def _rb(x):
    return x.astype(bf16).astype(f32)


def _unpack(x):
    return pltpu.bitcast(x, bf16)


def _recip(x):
    r = pltpu.reciprocal(x, approx=True)
    return r * (2.0 - x * r)


def make_kernel(att_off=600, att_last=56, ffn=(30, 16), fin_lag=3, xsplit=(2, 4, 8, 16),
                wo_prep=(40, 4), out_rows=1, lag0=(0, 4, 8, 9, 10), lag=(0, 2, 4, 5, 6), ln_start=21,
                qk_lag=1, win=400, pv_off=230, pv_gap=20, sm_off=48, ln_off=(140, 120, 200, 266, 284), top_gap=400,
                att_start=75, att_q=14, ln_stop=300,
                defer=2, GA=16, pv_split=((0,), (1,), (2,), (3,), (4,))):
    NA = M // GA

    def kernel(x_hbm, wqkv_hbm, wo_hbm, wr_hbm, wg_hbm, wu_hbm, wd_hbm, out_hbm,
               wr_ref, x_v, z_v, wqkv_raw, wqkv_t, wqkv_p, wo_raw, wo_f, wo_p, wg_v, wu_v, wd_v,
               xn_v, q_s, k_s, v_s, o_v, m_s, d_s, i_s, p_s, out_v, sem_x, sem_w, sem_o):
        xb = (0,) + tuple(b for b in xsplit if b <= NM)
        x_copies = [pltpu.make_async_copy(x_hbm.at[pl.ds(a * M, (b - a) * M), :], x_v.at[pl.ds(a * M, (b - a) * M), :],
                                          sem_x.at[j]) for j, (a, b) in enumerate(zip(xb[:-1], xb[1:]))]
        qkv_copies = [pltpu.make_async_copy(wqkv_hbm.at[:, pl.ds(p * D, D)], wqkv_raw.at[:, pl.ds(p * D, D)],
                                            sem_w.at[p]) for p in range(3)]
        late_copies = [pltpu.make_async_copy(s, d, sem_w.at[3 + j]) for j, (s, d) in enumerate(
            [(wo_hbm, wo_raw.at[pl.ds(0, D), :]), (wg_hbm, wg_v), (wu_hbm, wu_v), (wd_hbm, wd_v)])]

        wr_copy = pltpu.make_async_copy(wr_hbm, wr_ref, sem_w.at[7])

        def dma_point(start, wait):
            for c in start:
                c.start()
            for c in wait:
                c.wait()

        dma_point([wr_copy, x_copies[0], qkv_copies[0]], [wr_copy, x_copies[0]])

        lane = lax.broadcasted_iota(i32, (8, 128), 1)
        sub = lax.broadcasted_iota(i32, (8, 128), 0)
        wr = wr_ref[...].astype(f32).reshape(1, D)
        bits = pltpu.bitcast(jnp.broadcast_to(wr[:, :128], (8, 128)), i32) >> 16
        zero = (bits * (bits + 1)) & 1
        zero0 = zero[0, 0]
        fresh = itertools.count(1)
        st = dict(r=[jnp.zeros((8, 128), f32), jnp.zeros((8, 128), f32)])

        def opaque(align):
            return pl.multiple_of(zero0 * (next(fresh) * align), align)

        def after(ref):
            return pltpu.bitcast(ref[pl.ds(opaque(8), 8), pl.ds(0, 128)], i32)

        def hold(ref, idx):
            if st["go"] is not None:
                go = pltpu.bitcast(st["go"], i32) if ref.dtype == i32 else st["go"].astype(ref.dtype)
                ref[idx] = go

        def pull(token):
            return pltpu.bitcast(pltpu.reciprocal(pltpu.bitcast(token, f32), approx=True), i32)

        def x_rows(g):
            hold(x_v, (pl.ds(S, 8), pl.ds(0, 128)))
            return x_v[pl.ds(g * G + opaque(G), G), :].astype(f32)

        def put(ref, g, v):
            ref[g % NSTAT][pl.ds(0, G), :] = jnp.broadcast_to(v, (G, 128))
            return after(ref[g % NSTAT])

        def get(ref, g):
            return ref[g % NSTAT][pl.ds(opaque(8), G), :]

        def wide(v):
            return jnp.concatenate([v] * NT, axis=1)

        def x_wait(j):
            dma_point(late_copies if j == len(x_copies) - 1 else x_copies[j + 1:j + 2], [x_copies[j]])

        def ln_mean(g):
            return put(m_s, g, jnp.sum(x_rows(g), axis=1, keepdims=True) * (1.0 / D))

        def ln_var(g):
            c = x_rows(g) - wide(get(m_s, g))
            return put(d_s, g, jnp.sum(c * c, axis=1, keepdims=True))

        def ln_scale(g):
            hold(d_s[g % NSTAT], (pl.ds(G, 8), slice(None)))
            den = _rb(jnp.sqrt(_rb(_rb(get(d_s, g) * (1.0 / D)) + EPS_BF16)))
            return put(i_s, g, 1.0 / den)

        def ln_norm(g):
            xn = (_rb(x_rows(g) - wide(_rb(get(m_s, g)))) * wide(get(i_s, g))).astype(bf16)
            z_v.bitcast(bf16)[pl.ds(g * G, G), :] = xn
            xn_v[g // NG].bitcast(bf16)[pl.ds(g % NG * G, G), :] = xn
            return pull(after(xn_v[g // NG]))

        def ln_dot(g):
            hold(z_v, (pl.ds(S // 2, 8), pl.ds(0, 128)))
            xn = _unpack(z_v[pl.ds(g * G // 2 + opaque(8), G // 2), :])
            r = jnp.sum(xn.astype(f32) * wr, axis=1, keepdims=True)
            for s in range(G // 8):
                half, l = divmod(g * G // 8 + s, 128)
                rs = jnp.broadcast_to(r[s * 8:(s + 1) * 8], (8, 128))
                st["r"][half] = jnp.where(lane == l, rs, st["r"][half])
            return pltpu.bitcast(st["r"][half], i32)

        def mod5(n):
            return n - ((n * 205) >> 10) * 5

        src_lane = [(20 * (lane & 31) + 5 * (lane >> 5) + c) & 127 for c in range(NT)]
        src_tile = [mod5((c + 130 - lane) * 2) for c in range(NT)]

        def prep_select(p):
            for b in range(D // 16):
                rows = pl.ds(b * 16, 16)
                tiles = [pltpu.bitcast(wqkv_raw[rows, pl.ds(p * D + t * 128, 128)], i32) for t in range(NT)]
                for c in range(NT):
                    sel = tiles[0]
                    for t in range(1, NT):
                        sel = jnp.where(src_tile[c] == t, tiles[t], sel)
                    wqkv_t[c][pl.ds(b * 8, 8), :] = sel

        def prep_gather(p, c):
            z = opaque(8)
            for b in range(D // 16):
                wqkv_p[p * NT + c][pl.ds(b * 8, 8), :] = jnp.take_along_axis(
                    wqkv_t[c][pl.ds(z + b * 8, 8), :], src_lane[c], axis=1, mode="promise_in_bounds")

        def wo_widen(t, j):
            hold(wo_raw, (pl.ds(D, 8), pl.ds(0, 128)))
            wo_f[t][pl.ds(j * 128, 128), :] = wo_raw[pl.ds(j * 128 + opaque(16), 128), pl.ds(t * 128, 128)].astype(f32)
            return pull(after(wo_f[t]))

        def wo_perm(t, c):
            hold(wo_f[t], (pl.ds(D, 8), slice(None)))
            z = opaque(8)
            for g in range(4):
                blk = wo_f[t][pl.ds(z + (5 * g + c), 32, stride=20), :]
                wo_p[t][pl.ds(c * 64 + g * 16, 16), :] = pltpu.bitcast(blk.astype(bf16), i32)
            return pull(after(wo_p[t]))

        def window_pair(ref, c, row, w):
            t = ref[c, pl.ds(row + (HALO - 8 - DIL * w), GA + 8), :]
            return t[8:], t[:GA]

        def attn_qk(g):
            mb, j = divmod(g, NA)
            z = opaque(8)
            hold(q_s[mb], (0, pl.ds(M, 8), slice(None)))
            q = [q_s[mb][c, pl.ds(z + j * GA, GA), :] for c in range(NT)]
            for w in range(W // 2):
                ps = None
                for c in range(NT):
                    t = [q[c] * k for k in window_pair(k_s[mb], c, z + j * GA, w)]
                    ps = t if ps is None else [a + b for a, b in zip(ps, t)]
                for ww, p in zip((w, w + W // 2), ps):
                    p_s[g % NP][pl.ds(ww * GA, GA), :] = p + pltpu.roll(p, 64, 1)
            return after(p_s[g % NP])

        def attn_softmax(g):
            z = opaque(8)
            hold(p_s[g % NP], (pl.ds(W * GA, 8), slice(None)))
            ps = [p_s[g % NP][pl.ds(z + w * GA, GA), :] for w in range(W)]
            ps = [p + pltpu.roll(p, 32, 1) for p in ps]
            for w in range(W):
                if g * GA < DIL * w:
                    pos = g * GA + lax.broadcasted_iota(i32, (GA, 128), 0)
                    ps[w] = jnp.where(pos >= DIL * w, ps[w], NEG)
            m = functools.reduce(jnp.maximum, ps)
            e = [jnp.exp2(l - m) for l in ps]
            inv = _recip(functools.reduce(jnp.add, e))
            st["e", g] = e, inv
            return pltpu.bitcast(inv[GA - 8:], i32)

        def attn_pv(g, cs):
            mb, j = divmod(g, NA)
            z = opaque(8)
            hold(v_s[mb], (0, pl.ds(M + HALO, 8), slice(None)))
            e, inv = st["e", g]
            token = None
            for c in cs:
                acc = None
                for w in range(W // 2):
                    for ww, v in zip((w, w + W // 2), window_pair(v_s[mb], c, z + j * GA, w)):
                        acc = e[ww] * v if acc is None else acc + e[ww] * v
                acc = acc * inv
                for r in range(GA // 8):
                    t = pltpu.bitcast(acc[r * 8:(r + 1) * 8], i32)
                    token = t if token is None else token | t
                if GA == 8:
                    if g % 2 == 0:
                        st["o", c] = acc
                        continue
                    acc = jnp.concatenate([st.pop(("o", c)), acc], axis=0)
                o_v[mb].bitcast(bf16)[pl.ds(j * GA // 16 * 16, 16), pl.ds(c * 128, 128)] = acc.astype(bf16)
            return pull(token)

        row = lax.broadcasted_iota(i32, (16, D), 0)

        def tile_of(t):
            return pl.ds(pl.multiple_of((t // 16) * 8, 8), 8)

        def tok(v):
            return pltpu.bitcast(jnp.broadcast_to(v, (8, 128)), i32)

        def top(k):
            if k == 0:
                st["r_all"] = r_all = _rb(jnp.concatenate(st["r"], axis=0))
                st["idx"] = jnp.concatenate([lane * 8 + sub, (lane + 128) * 8 + sub], axis=0).astype(f32)
                st["key"] = jnp.where(r_all == r_all, r_all, -jnp.inf)
                st["free"] = jnp.full((16, 128), True)
                st["i"] = []
            if k % 2 == 0:
                st["max"] = jnp.max(st["key"], keepdims=True)
                return tok(st["max"])
            i = jnp.min(jnp.where((st["key"] == st["max"]) & st["free"], st["idx"], S - 1.0), keepdims=True)
            st["i"].append(i)
            st["free"] = st["idx"] != i
            st["key"] = jnp.where(st["free"], st["key"], -jnp.inf)
            return tok(i)

        def gather():
            st["rs"] = [jnp.sum(jnp.where(st["idx"] == i, st["r_all"], 0.0), keepdims=True) for i in st["i"]]
            st["t"] = [i.astype(i32)[0, 0] for i in st["i"]]

            def pick(t):
                z = _unpack(z_v[tile_of(t), :]).astype(f32)
                return jnp.sum(jnp.where(row == t % 16, z, 0.0), axis=0, keepdims=True)

            xs = jnp.where(row == 0, pick(st["t"][0]), pick(st["t"][1]))
            st["xs"] = xs.astype(bf16)
            return pltpu.bitcast(xs[:8, :128], i32) | tok(st["rs"][0]) | tok(st["rs"][1])

        def late_wait():
            for c in late_copies:
                c.wait()

        def ffn_up():
            gate = _rb(lax.dot_general(st["xs"], wg_v[...], NT_DIMS, preferred_element_type=f32))
            up = _rb(lax.dot_general(st["xs"], wu_v[...], NT_DIMS, preferred_element_type=f32))
            st["hid"] = (_rb(gate * jax.nn.sigmoid(gate)) * up).astype(bf16)

        def ffn_down():
            st["y"] = _rb(jnp.dot(st["hid"], wd_v[...], preferred_element_type=f32))

        def patch():
            for j in range(2):
                t = st["t"][j]
                upd = _rb(st["y"][j:j + 1] * _rb(jax.nn.sigmoid(st["rs"][j])))
                z = _unpack(z_v[tile_of(t), :]).astype(f32)
                z_v[tile_of(t), :] = pltpu.bitcast(jnp.where(row == t % 16, z + upd, z).astype(bf16), i32)

        def o_copy(j):
            rows = pl.ds(j * out_rows * M, out_rows * M)
            return pltpu.make_async_copy(out_v.at[rows, :], out_hbm.at[rows, :], sem_o.at[j])

        def piece_dot(lhs_ref, rhs_ref, deps):
            z = opaque(8)
            cols = []
            for k in range(NT):
                col = lhs_ref[pl.ds(z, M // 2), pl.ds(k * 128, 128)]
                if any(kk == k for kk, _ in deps):
                    parts = [col[r * 8:(r + 1) * 8] for r in range(M // 16)]
                    for (kk, r), t in deps.items():
                        if kk == k:
                            parts[r] = parts[r] | (t & zero)
                    col = jnp.concatenate(parts, axis=0)
                cols.append(col)
            lhs = _unpack(jnp.concatenate(cols, axis=1))
            return jnp.dot(lhs, _unpack(rhs_ref[pl.ds(z, D // 2), :]), preferred_element_type=f32)

        def qkv_dot(mb, n, deps):
            return piece_dot(xn_v[mb], wqkv_p[n], deps)

        def qkv_store(mb, n, res):
            p, c = divmod(n, NT)
            if p == 0:
                q_s[mb][c, pl.ds(0, M), :] = res * QSCALE
            else:
                dst = (k_s, v_s)[p - 1]
                dst[mb][c, pl.ds(HALO, M), :] = res
                if mb == 0:
                    dst[0][c, pl.ds(0, HALO), :] = jnp.broadcast_to(res[0:1], (HALO, 128))
                if mb + 1 < NM:
                    dst[mb + 1][c, pl.ds(0, HALO), :] = res[M - HALO:]

        def out_dot(mb, c, deps):
            return piece_dot(o_v[mb], wo_p[c], deps)

        def out_store(mb, c, s):
            cols = pl.ds(c * 128, 128)
            z = _unpack(z_v[pl.ds(mb * M // 2 + opaque(8), M // 2), cols]).astype(f32)
            gate = z * pltpu.reciprocal(1.0 + jnp.exp2(z * -LOG2E), approx=True)
            res = x_v[pl.ds(mb * M + opaque(16), M), cols].astype(f32) + s * gate
            out_v[pl.ds(mb * M, M), cols] = res.astype(bf16)
            if c == NT - 1 and (mb + 1) % out_rows == 0:
                o_copy(mb // out_rows).start()
            return pltpu.bitcast(res[M - 8:], i32)

        qkv, out = (qkv_dot, qkv_store), (out_dot, out_store)
        pieces = [(qkv, mb, p * NT + c) for p in range(3) for mb in range(2) for c in range(NT)]
        pieces += [(qkv, mb, n) for mb in range(2, NM) for n in range(3 * NT)]
        nq = len(pieces)
        pieces += [(out, mb, c) for mb in range(NM) for c in range(NT)]
        tasks = []

        def at(t, win, fn, *args):
            tasks.append((t, len(tasks), win, fn, args))

        stages = (ln_mean, ln_var, ln_scale, ln_norm, ln_dot)
        for t in range(2 * NG + lag0[-1]):
            for k, fn in reversed(list(zip(lag0, stages))):
                if 0 <= t - k < 2 * NG:
                    at(0, 0, fn, t - k)
        for p, first in enumerate((0, 8, 16)):
            at(first * PIECE, 0, dma_point, (qkv_copies[1:], x_copies[1:2], [])[p], [qkv_copies[p]])
            at(first * PIECE, 0, prep_select, p)
            for c in range(NT):
                at((first + c) * PIECE if p else 0, 0, prep_gather, p, c)
        frame = 15 * PIECE // NG
        base = att_start * PIECE
        nsteps = (NM - 2) * NG + lag[-1]
        t0 = ln_start * PIECE
        for t in range(nsteps):
            lo, hi, a, b = (0, NG + lag[3], t0, 27 * PIECE) if t < NG + lag[3] else \
                (NG + lag[3], nsteps, 27 * PIECE, base - ln_stop)
            period = (b - a) // (hi - lo)
            t_ln = a + (t - lo) * (b - a) // (hi - lo)
            for k, fn, off in zip(lag, stages, ln_off):
                g = 2 * NG + t - k
                if 2 * NG <= g < NM * NG:
                    if fn is ln_mean and g % NG == 0 and g // NG in xb:
                        at(t_ln // (4 * PIECE) * (4 * PIECE), 0, x_wait, xb.index(g // NG))
                    at(t_ln + off * period // frame, min(win, period + 160), fn, g)
        t_ln += frame

        def slot(g):
            if g < att_q * NA:
                return base + (g + qk_lag) * (nq * PIECE + att_off - base) // (att_q * NA + qk_lag)
            return nq * PIECE + att_off + (g - att_q * NA) * att_last * PIECE // ((NM - att_q) * NA)

        for g in range(NM * NA):
            at(slot(g - qk_lag), win, attn_qk, g)
            at(slot(g) + sm_off, win, attn_softmax, g)
            for n, cs in enumerate(pv_split):
                at(slot(g) + pv_off + n * pv_gap, win, attn_pv, g, cs)
        for k in range(4):
            at(t_ln + (k + 1) * top_gap, win, top, k)
        at(t_ln + 5 * top_gap, win, gather)
        at((nq - wo_prep[0]) // 4 * 4 * PIECE, 0, late_wait)
        for j in range(2 * NT * NT):
            t = (nq - wo_prep[0] + 1) * PIECE + j * (wo_prep[0] - wo_prep[1] - 1) * PIECE // (2 * NT * NT)
            at(t, win, (wo_widen, wo_perm)[j // NT % 2], j // (2 * NT), j % NT)
        at((nq - ffn[0]) * PIECE, 0, ffn_up)
        at((nq - ffn[1]) * PIECE, 0, ffn_down)
        at((nq - 2) * PIECE, 0, patch)

        due = collections.defaultdict(list)
        for task in sorted(tasks, key=lambda task: task[:2]):
            due[task[0] // PIECE].append(task)

        def lhs_slot(i, t):
            start = M * (NT * i // 4)
            return (0, (t - start) // 16) if t - start < M else (NT - 1, (t - start - M) // 16)

        def result_at(t):
            i = min((t - 130) // PIECE, len(results) - 1)
            while i >= 0 and M * ((NT * i + NT - 1) // 4) + 130 > t:
                i -= 1
            if i < 0:
                return None
            r = min((t - 130 - M * ((NT * i + NT - 1) // 4)) // 8, M // 8 - 1)
            return results[i][r * 8:(r + 1) * 8]

        results = []
        deps = collections.defaultdict(dict)

        def tie(t, token):
            if token is not None:
                slots, key = deps[t // PIECE], lhs_slot(t // PIECE, t)
                slots[key] = slots[key] | token if key in slots else token

        for i, ((dot, _), mb, n) in enumerate(pieces):
            for t, _, limit, fn, args in due.pop(i, []):
                st["go"] = result_at(t) if limit else None
                token = fn(*args)
                if limit:
                    tie(t + limit, token)
            if i >= defer:
                (_, store), mb_s, n_s = pieces[i - defer]
                tie((i - defer + fin_lag) * PIECE, store(mb_s, n_s, results[i - defer]))
            results.append(dot(mb, n, deps.pop(i, {})))
        for i in range(len(pieces) - defer, len(pieces)):
            (_, store), mb_s, n_s = pieces[i]
            store(mb_s, n_s, results[i])
        assert not due
        for j in range(NM // out_rows):
            o_copy(j).wait()

    scratch = [
        pltpu.VMEM((D,), bf16),
        pltpu.VMEM((S + 16, D), bf16),
        pltpu.VMEM((S // 2 + 8, D), i32),
        pltpu.VMEM((D, 3 * D), bf16),
        [pltpu.VMEM((D // 2, 128), i32)] * NT,
        [pltpu.VMEM((D // 2, 128), i32)] * (3 * NT),
        pltpu.VMEM((D + 16, D), bf16),
        [pltpu.VMEM((D + 8, 128), f32)] * NT,
        [pltpu.VMEM((D // 2, 128), i32)] * NT,
        pltpu.VMEM((F, D), bf16),
        pltpu.VMEM((F, D), bf16),
        pltpu.VMEM((F, D), bf16),
        [pltpu.VMEM((M // 2, D), i32)] * NM,
        [pltpu.VMEM((NT, M + 8, 128), f32)] * NM,
        [pltpu.VMEM((NT, M + HALO, 128), f32)] * NM,
        [pltpu.VMEM((NT, M + HALO + 8, 128), f32)] * NM,
        [pltpu.VMEM((M // 2, D), i32)] * NM,
        [pltpu.VMEM((G, 128), f32)] * NSTAT,
        [pltpu.VMEM((G + 8, 128), f32)] * NSTAT,
        [pltpu.VMEM((G, 128), f32)] * NSTAT,
        [pltpu.VMEM((W * GA + 8, 128), f32)] * NP,
        pltpu.VMEM((S, D), bf16),
        pltpu.SemaphoreType.DMA((len(xsplit),)),
        pltpu.SemaphoreType.DMA((8,)),
        pltpu.SemaphoreType.DMA((NM // out_rows,)),
    ]
    hbm = pl.BlockSpec(memory_space=pltpu.HBM)
    return pl.pallas_call(
        kernel,
        out_shape=jax.ShapeDtypeStruct((S, D), bf16),
        in_specs=[hbm] * 7,
        out_specs=hbm,
        scratch_shapes=scratch,
        compiler_params=pltpu.CompilerParams(vmem_limit_bytes=100 * 1024 * 1024),
        name="fused",
    )


@jax.jit
def pallas_recurrent_scan__sliding_local_dilated__moe_arch_mod__prompt_kernel(
    A_x: jax.Array,
    A_wqkv: jax.Array,
    A_wo: jax.Array,
    B_x: jax.Array,
    B_w_r: jax.Array,
    B_w_gate: jax.Array,
    B_w_up: jax.Array,
    B_w_down: jax.Array,
):
    del B_x
    out = make_kernel()(A_x.reshape(S, D), A_wqkv, A_wo, B_w_r, B_w_gate.T, B_w_up.T, B_w_down)
    return out.reshape(1, S, D)
```

```python
import bisect
import collections
import functools
import itertools
import math

import jax
import jax.numpy as jnp
import numpy as np
from jax import lax
from jax.experimental import pallas as pl
from jax.experimental.pallas import tpu as pltpu

S, D, F = 2048, 640, 1728
H, DH, W, DIL = 32, 20, 8, 2
NT = D // 128
HALO = 16
M = 128
NM = S // M
G = 16
NG = M // G
NSTAT = 32
NP = 8
QS, KS = M + 8, M + HALO
PIECE = M * NT // 4
LATENCY = 130
LOG2E = math.log2(math.e)
QSCALE = DH ** -0.5 * LOG2E
NEG = -1e9 * LOG2E
EPS_BF16 = float(np.asarray(1e-5, dtype=jnp.bfloat16).astype(np.float32))
f32, bf16, i32 = jnp.float32, jnp.bfloat16, jnp.int32
NT_DIMS = (((1,), (1,)), ((), ()))


def _rb(x):
    return x.astype(bf16).astype(f32)


def _unpack(x):
    return pltpu.bitcast(x, bf16)


def _tree(op, xs):
    while len(xs) > 1:
        xs = [op(a, b) for a, b in zip(xs[::2], xs[1::2])] + xs[len(xs) // 2 * 2:]
    return xs[0]


NF = 3


def make_kernel(att_off=600, att_last=64, fin_lag=3, wo_prep=(-60, -4), out_rows=1, qk_lag=2, win=400, pv_off=270, pv_gap=20, sm_off=0,
                ln_off=(0, 18, 40, 55, 72, 90, 95), ln_done=2, scale_lag=1, scale_limit=150, top_gap=400, att_start=96, att_q=13,
                ln_stop=300, defer=2, GA=16, pv_split=((0,), (1,), (2,), (3,), (4,)), w_wait=(12, 24), x_wait=32,
                late=144, quiet=250, quiet_off=350, ffn_gap=2, sel_off=150, sel_gap=32,
                qk_split=((0,), (1,), (2,), (3,)), qk_off=140, st_off=200, qk_gap=22, exp_off=250, flags=None):
    NA = M // GA

    def kernel(x_hbm, wqkv_hbm, wo_hbm, wr_hbm, wg_hbm, wu_hbm, wd_hbm, out_hbm,
               x_v, z_v, wqkv_raw, wqkv_t, wqkv_p, wo_raw, wo_f, wo_p, wg_v, wu_v, wd_v,
               xn_v, q_s, k_s, v_s, o_v, m_s, d_s, i_s, f_s, p_s, out_v, d_v, xs_v, hid_v, wr_ref, sem_x, sem_w, sem_o):
        xb = (0, 1, NF, NM)
        x_copies = [pltpu.make_async_copy(x_hbm.at[pl.ds(a * M, (b - a) * M), :], x_v.at[pl.ds(a * M, (b - a) * M), :],
                                          sem_x.at[j]) for j, (a, b) in enumerate(zip(xb[:-1], xb[1:]))]
        qkv_copies = [pltpu.make_async_copy(wqkv_hbm.at[:, pl.ds(p * D, D)], wqkv_raw.at[pl.ds(0, D), pl.ds(p * D, D)],
                                            sem_w.at[p]) for p in range(3)]
        late_copies = [pltpu.make_async_copy(s, d, sem_w.at[3 + j]) for j, (s, d) in enumerate(
            [(wo_hbm, wo_raw.at[pl.ds(0, D), :]), (wg_hbm, wg_v), (wu_hbm, wu_v), (wd_hbm, wd_v)])]

        wr_copy = pltpu.make_async_copy(wr_hbm, wr_ref, sem_w.at[7])

        def dma_point(start, wait):
            for c in start:
                c.start()
            for c in wait:
                c.wait()

        dma_point([wr_copy, x_copies[0], qkv_copies[0], x_copies[1]], [wr_copy, x_copies[0]])

        lane = lax.broadcasted_iota(i32, (8, 128), 1)
        sub = lax.broadcasted_iota(i32, (8, 128), 0)
        wr = wr_ref[...].astype(f32).reshape(1, D)
        bits = pltpu.bitcast(jnp.broadcast_to(wr[:, :128], (8, 128)), i32) >> 16
        zero = (bits * (bits + 1)) & 1
        zero0 = zero[0, 0]
        fresh = itertools.count(1)
        folds = itertools.count()
        st = dict(folded=[], sums=[], r=[jnp.zeros((8, 128), f32), jnp.zeros((8, 128), f32)])

        def opaque(align):
            return pl.multiple_of(zero0 * (next(fresh) * align), align)

        def after(ref):
            return pltpu.bitcast(ref[pl.ds(opaque(8), 8), pl.ds(0, 128)], i32)

        def hold(ref, idx):
            if st["go"] is not None:
                ref[idx] = pltpu.bitcast(st["go"], i32) if ref.dtype == i32 else st["go"].astype(ref.dtype)

        def x_rows(g):
            return x_v[pl.ds(g * G + opaque(G), G), :].astype(f32)

        def wide(v):
            return jnp.concatenate([v] * NT, axis=1)

        def get(ref, g):
            return ref[g % NSTAT][pl.ds(opaque(8), G), :]

        def put(ref, g, v):
            ref[g % NSTAT][pl.ds(0, G), :] = jnp.broadcast_to(v, (G, 128))
            return after(ref[g % NSTAT])

        def fold(g, then, v):
            slot_ref = f_s[next(folds) % NSTAT]
            slot_ref[pl.ds(0, G), :] = _tree(jnp.add, [v[:, c * 128:(c + 1) * 128] for c in range(NT)])
            st["folded"].append((then, g, slot_ref))
            return after(slot_ref)

        def ln_reduce():
            sums = []
            for then, g, slot_ref in st["folded"]:
                hold(slot_ref, (pl.ds(G, 8), slice(None)))
                sums.append((then, g, jnp.sum(slot_ref[pl.ds(opaque(8), G), :], axis=1, keepdims=True)))
            st["folded"] = []
            st["sums"].append(sums)

        def ln_finish():
            tokens = [then(g, v) for then, g, v in st["sums"].pop(0)]
            return functools.reduce(jnp.bitwise_or, tokens) if tokens else None

        def ln_mean(g):
            return fold(g, lambda g, v: put(m_s, g, v * (1.0 / D)), x_rows(g))

        def ln_var(g):
            d = x_rows(g) - wide(_rb(get(m_s, g)))
            d_v[g % NSTAT][...] = d.astype(bf16)
            return fold(g, lambda g, v: put(d_s, g, v * (1.0 / D)), d * d)

        def ln_scale(g):
            hold(d_s[g % NSTAT], (pl.ds(G, 8), slice(None)))
            m = get(m_s, g)
            shift = m - _rb(m)
            var = jnp.maximum(get(d_s, g) - shift * shift, 0.0)
            root = lax.rsqrt(_rb(jnp.sqrt(_rb(_rb(var) + EPS_BF16))))
            return put(i_s, g, root * root)

        def ln_norm(g):
            xn = (d_v[g % NSTAT][pl.ds(opaque(G), G), :].astype(f32) * wide(get(i_s, g))).astype(bf16)
            z_v.bitcast(bf16)[pl.ds(g * G, G), :] = xn
            xn_v[g // NG].bitcast(bf16)[pl.ds(g % NG * G, G), :] = xn
            return after(xn_v[g // NG])

        def keep_score(g, r):
            for s in range(G // 8):
                half, l = divmod(g * G // 8 + s, 128)
                rs = jnp.broadcast_to(r[s * 8:(s + 1) * 8], (8, 128))
                st["r"][half] = jnp.where(lane == l, rs, st["r"][half])
            return pltpu.bitcast(st["r"][half], i32)

        def ln_dot(g):
            xn = _unpack(z_v[pl.ds(g * G // 2 + opaque(8), G // 2), :])
            return fold(g, keep_score, xn.astype(f32) * wr)

        def mod5(n):
            return n - ((n * 205) >> 10) * 5

        src_lane = [(20 * (lane & 31) + 5 * (lane >> 5) + c) & 127 for c in range(NT)]
        src_tile = [mod5((c + 130 - lane) * 2) for c in range(NT)]

        def select(p, b, cs, z):
            rows = pl.ds(z + b * 16, 16)
            tiles = [pltpu.bitcast(wqkv_raw[rows, pl.ds(p * D + t * 128, 128)], i32) for t in range(NT)]
            for c in cs:
                sel = tiles[0]
                for t in range(1, NT):
                    sel = jnp.where(src_tile[c] == t, tiles[t], sel)
                yield c, sel

        def gather_lanes(p, c, b, v):
            wqkv_p[p * NT + c][pl.ds(b * 8, 8), :] = jnp.take_along_axis(
                v, src_lane[c], axis=1, mode="promise_in_bounds")

        def prep_first(p):
            z = opaque(64)
            for b in range(D // 16):
                for c, sel in select(p, b, [0], z):
                    gather_lanes(p, c, b, sel)

        def prep_select(p, j):
            z = opaque(64)
            for b in range(j * 5, (j + 1) * 5):
                for c, sel in select(p, b, range(1, NT), z):
                    wqkv_t[c][pl.ds(b * 8, 8), :] = sel
            return after(wqkv_t[NT - 1])

        def prep_gather(p, c):
            z = opaque(8)
            for b in range(D // 16):
                gather_lanes(p, c, b, wqkv_t[c][pl.ds(z + b * 8, 8), :])

        def wo_widen(t, j):
            wo_f[t][pl.ds(j * 128, 128), :] = wo_raw[pl.ds(j * 128 + opaque(16), 128), pl.ds(t * 128, 128)].astype(f32)
            return after(wo_f[t])

        def wo_perm(t, c):
            z = opaque(8)
            for g in range(4):
                blk = wo_f[t][pl.ds(z + (5 * g + c), 32, stride=20), :]
                wo_p[t][pl.ds(c * 64 + g * 16, 16), :] = pltpu.bitcast(blk.astype(bf16), i32)
            return after(wo_p[t])

        def window_pair(ref, z, c, row, w):
            t = ref[pl.ds(z + (row + c * KS + HALO - 8 - DIL * w), GA + 8), :]
            return t[8:], t[:GA]

        def attn_qk(g, ws):
            mb, j = divmod(g, NA)
            z = opaque(8)
            hold((q_s if ws[0] == 0 else k_s)[mb], (pl.ds(M if ws[0] == 0 else NT * KS, 8), slice(None)))
            if ws[0] == 0:
                st["q"] = [q_s[mb][pl.ds(z + (c * QS + j * GA), GA), :] for c in range(NT)]
            for w in ws:
                ps = None
                for c in range(NT):
                    t = [st["q"][c] * k for k in window_pair(k_s[mb], z, c, j * GA, w)]
                    ps = t if ps is None else [a + b for a, b in zip(ps, t)]
                st["p", g, w] = [(p, pltpu.roll(p, 64, 1)) for p in ps]

        def attn_qk_store(g, ws):
            for w in ws:
                for ww, (p, r) in zip((w, w + W // 2), st.pop(("p", g, w))):
                    p_s[g % NP][pl.ds(ww * GA, GA), :] = p + r
            return after(p_s[g % NP])

        def attn_logits(g):
            z = opaque(8)
            hold(p_s[g % NP], (pl.ds(W * GA, 8), slice(None)))
            ps = [p_s[g % NP][pl.ds(z + w * GA, GA), :] for w in range(W)]
            st["l", g] = [p + pltpu.roll(p, 32, 1) for p in ps]

        def attn_softmax(g):
            ps = st.pop(("l", g))
            for w in range(W):
                if g * GA < DIL * w:
                    pos = g * GA + lax.broadcasted_iota(i32, (GA, 128), 0)
                    ps[w] = jnp.where(pos >= DIL * w, ps[w], NEG)
            m = _tree(jnp.maximum, ps)
            e = [jnp.exp2(l - m) for l in ps]
            inv = pltpu.reciprocal(_tree(jnp.add, e), approx=True)
            st["e", g] = e, inv
            return pltpu.bitcast(inv[:8], i32) | pltpu.bitcast(inv[GA - 8:], i32)

        def attn_pv(g, cs):
            mb, j = divmod(g, NA)
            z = opaque(8)
            e, inv = st["e", g]
            token = None
            for c in cs:
                acc = None
                for w in range(W // 2):
                    near, far = window_pair(v_s[mb], z, c, j * GA, w)
                    t = e[w] * near + e[w + W // 2] * far
                    acc = t if acc is None else acc + t
                acc = acc * inv
                for r in range(GA // 8):
                    t = pltpu.bitcast(acc[r * 8:(r + 1) * 8], i32)
                    token = t if token is None else token | t
                if GA == 8:
                    if g % 2 == 0:
                        st["o", c] = acc
                        continue
                    acc = jnp.concatenate([st.pop(("o", c)), acc], axis=0)
                o_v[mb].bitcast(bf16)[pl.ds(j * GA // 16 * 16, 16), pl.ds(c * 128, 128)] = acc.astype(bf16)
            return token

        row = lax.broadcasted_iota(i32, (16, D), 0)

        def tile_of(t):
            return pl.ds(pl.multiple_of((t // 16) * 8, 8), 8)

        def tok(v):
            return pltpu.bitcast(jnp.broadcast_to(v, (8, 128)), i32)

        def top(k):
            if k == 0:
                st["r_all"] = r_all = _rb(jnp.concatenate(st["r"], axis=0))
                st["idx"] = jnp.concatenate([lane * 8 + sub, (lane + 128) * 8 + sub], axis=0).astype(f32)
                st["key"] = jnp.where(r_all == r_all, r_all, -jnp.inf)
                st["free"] = jnp.full((16, 128), True)
                st["i"] = []
            if k % 2 == 0:
                st["max"] = jnp.max(st["key"], keepdims=True)
                return tok(st["max"])
            i = jnp.min(jnp.where((st["key"] == st["max"]) & st["free"], st["idx"], S - 1.0), keepdims=True)
            st["i"].append(i)
            st["free"] = st["idx"] != i
            st["key"] = jnp.where(st["free"], st["key"], -jnp.inf)
            return tok(i)

        def gather():
            st["rs"] = [jnp.sum(jnp.where(st["idx"] == i, st["r_all"], 0.0), keepdims=True) for i in st["i"]]
            st["t"] = [i.astype(i32)[0, 0] for i in st["i"]]

            def pick(t):
                z = _unpack(z_v[tile_of(t), :]).astype(f32)
                return jnp.sum(jnp.where(row == t % 16, z, 0.0), axis=0, keepdims=True)

            xs = jnp.where(row == 0, pick(st["t"][0]), pick(st["t"][1]))
            xs_v[...] = xs.astype(bf16)
            return pltpu.bitcast(xs[:8, :128], i32) | tok(st["rs"][0]) | tok(st["rs"][1])

        def ffn_rows(j):
            return pl.ds(j * 128, min(128, F - j * 128))

        def ffn_gate(j):
            st["gate"] = lax.dot_general(xs_v[...], wg_v[ffn_rows(j), :], NT_DIMS, preferred_element_type=f32)

        def ffn_up(j):
            gate = _rb(st.pop("gate"))
            up = _rb(lax.dot_general(xs_v[...], wu_v[ffn_rows(j), :], NT_DIMS, preferred_element_type=f32))
            hid_v[:, ffn_rows(j)] = (_rb(gate * jax.nn.sigmoid(gate)) * up).astype(bf16)

        def ffn_down(j):
            y = jnp.dot(hid_v[:, ffn_rows(j)], wd_v[ffn_rows(j), :], preferred_element_type=f32)[:8]
            st["y"] = y if j == 0 else st["y"] + y

        def patch():
            for j in range(2):
                t = st["t"][j]
                upd = _rb(_rb(st["y"][j:j + 1]) * _rb(jax.nn.sigmoid(st["rs"][j])))
                z = _unpack(z_v[tile_of(t), :]).astype(f32)
                z_v[tile_of(t), :] = pltpu.bitcast(jnp.where(row == t % 16, z + upd, z).astype(bf16), i32)

        def o_copy(j):
            rows = pl.ds(j * out_rows * M, out_rows * M)
            return pltpu.make_async_copy(out_v.at[rows, :], out_hbm.at[rows, :], sem_o.at[j])

        def piece_dot(lhs_ref, rhs_ref, deps):
            z = opaque(8)
            cols = []
            for k in range(NT):
                col = lhs_ref[pl.ds(z, M // 2), pl.ds(k * 128, 128)]
                if any(kk == k for kk, _ in deps):
                    parts = [col[r * 8:(r + 1) * 8] for r in range(M // 16)]
                    for (kk, r), t in deps.items():
                        if kk == k:
                            parts[r] = parts[r] | (t & zero)
                    col = jnp.concatenate(parts, axis=0)
                cols.append(col)
            lhs = _unpack(jnp.concatenate(cols, axis=1))
            return jnp.dot(lhs, _unpack(rhs_ref[pl.ds(z, D // 2), :]), preferred_element_type=f32)

        def qkv_dot(mb, n, deps):
            return piece_dot(xn_v[mb], wqkv_p[n], deps)

        def qkv_store(mb, n, res):
            p, c = divmod(n, NT)
            if p == 0:
                q_s[mb][pl.ds(c * QS, M), :] = res * QSCALE
            else:
                dst = (k_s, v_s)[p - 1]
                dst[mb][pl.ds(c * KS + HALO, M), :] = res
                if mb == 0:
                    dst[0][pl.ds(c * KS, HALO), :] = jnp.broadcast_to(res[0:1], (HALO, 128))
                if mb + 1 < NM:
                    dst[mb + 1][pl.ds(c * KS, HALO), :] = res[M - HALO:]

        def out_dot(mb, c, deps):
            return piece_dot(o_v[mb], wo_p[c], deps)

        def out_store(mb, c, s):
            cols = pl.ds(c * 128, 128)
            z = _unpack(z_v[pl.ds(mb * M // 2 + opaque(8), M // 2), cols]).astype(f32)
            gate = z * pltpu.reciprocal(1.0 + jnp.exp2(z * -LOG2E), approx=True)
            res = x_v[pl.ds(mb * M + opaque(16), M), cols].astype(f32) + s * gate
            out_v[pl.ds(mb * M, M), cols] = res.astype(bf16)
            if c == NT - 1 and (mb + 1) % out_rows == 0:
                o_copy(mb // out_rows).start()
            return pltpu.bitcast(res[M - 8:], i32)

        qkv, out = (qkv_dot, qkv_store), (out_dot, out_store)
        pieces = [(qkv, mb, p * NT + c) for p in range(3) for mb in range(NF) for c in range(NT)]
        pieces += [(qkv, mb, n) for mb in range(NF, NM) for n in range(3 * NT)]
        nq = len(pieces)
        pieces += [(out, mb, c) for mb in range(NM) for c in range(NT)]
        nf = pl.cdiv(F, 128)
        extra = {}
        for j in range(nf):
            extra[late + 1 + 2 * j * ffn_gap] = ffn_gate, j
            extra[late + 1 + (2 * j + 1) * ffn_gap] = ffn_up, j
            extra[late + 4 + (2 * nf + j) * ffn_gap] = ffn_down, j
        busy, start = [0] * 4, []
        for i in range(len(pieces)):
            for rows in ([16] * NT if i in extra else []) + [M] * NT:
                m = busy.index(min(busy))
                if rows == M:
                    start.append(busy[m])
                busy[m] += rows
        start = np.reshape(start, (-1, NT)).tolist()
        begin = [0]
        for i in range(1, len(pieces)):
            begin.append(max(start[i][0], min(begin[-1] + PIECE, start[i - 1][-1] + M - 1)))
        end_q = begin[nq]
        tasks = []

        def at(t, limit, fn, *args):
            tasks.append((t, len(tasks), limit, fn, args))

        def piece_at(t):
            return bisect.bisect_right(begin, t) - 1

        stages = (ln_mean, ln_var, ln_scale, ln_norm, ln_dot)

        def ln_steps(lo, hi, a, b, done):
            lags = (0, done + 1, 2 * done + 2, 2 * done + 3 + scale_lag, 2 * done + 4 + scale_lag)
            n = hi - lo + lags[-1] + done
            for t in range(n):
                def time(off):
                    return a + (t * 100 + off) * (b - a) // (100 * n)

                for k, fn, off in zip(lags, stages, ln_off):
                    if 0 <= t - k < hi - lo:
                        at(time(off), (scale_limit if fn is ln_scale else 1) if b else 0, fn, lo + t - k)
                if t < n - done:
                    at(time(ln_off[5]), 1 if b else 0, ln_reduce)
                if t >= done:
                    at(time(ln_off[6]), 1 if b else 0, ln_finish)

        ln_steps(0, NG, 0, 0, 2)
        at(0, 0, dma_point, qkv_copies[1:], qkv_copies[:1])
        at(0, 0, dma_point, [], x_copies[1:2])
        for p, first in enumerate((0,) + w_wait):
            if p:
                at(first * PIECE, 0, dma_point, x_copies[2:] if p == 1 else [], qkv_copies[p:p + 1])
            at(first * PIECE, 0, prep_first, p)
            for j in range(8):
                at(first * PIECE + sel_off + j * sel_gap if p else 0, 1 if p else 0, prep_select, p, j)
            for c in range(1, NT):
                at(first * PIECE + sel_off + 8 * sel_gap if p else 0, 0, prep_gather, p, c)
        ln_steps(NG, 2 * NG, 0, 0, 2)
        ln_steps(2 * NG, NF * NG, PIECE, ((NF - 1) * NT) * PIECE, 3)
        at(x_wait * PIECE, 0, dma_point, late_copies, x_copies[2:])
        base = att_start * PIECE
        ln_steps(NF * NG, NM * NG, x_wait * PIECE, base - ln_stop, ln_done)
        for k in range(4):
            at(base + k * top_gap, win, top, k)
        at(base + 4 * top_gap, win, gather)

        def slot(g):
            if g < att_q * NA:
                t = base + (g + qk_lag) * (end_q + att_off - base - quiet) // (att_q * NA + qk_lag)
                return t + quiet if t > begin[late] - quiet - quiet_off else t
            return end_q + att_off + (g - att_q * NA) * att_last * PIECE // ((NM - att_q) * NA)

        for g in range(NM * NA):
            for n, ws in enumerate(qk_split):
                at(slot(g - qk_lag) + qk_off + n * qk_gap, win, attn_qk, g, ws)
                at(slot(g - qk_lag) + qk_off + n * qk_gap + st_off, 1, attn_qk_store, g, ws)
            at(slot(g) + sm_off, win, attn_logits, g)
            at(slot(g) + sm_off + exp_off, 1, attn_softmax, g)
            for n, cs in enumerate(pv_split):
                at(slot(g) + pv_off + n * pv_gap, 1, attn_pv, g, cs)
        at(begin[late], 0, dma_point, [], late_copies)
        for j in range(2 * NT * NT):
            t = end_q + wo_prep[0] * PIECE + j * (wo_prep[1] - wo_prep[0]) * PIECE // (2 * NT * NT)
            at(t, 1, (wo_widen, wo_perm)[j // NT % 2], j // (2 * NT), j % NT)
        at(begin[nq - 2], 0, patch)

        due = collections.defaultdict(list)
        for task in sorted(tasks, key=lambda task: task[:2]):
            due[piece_at(task[0])].append(task)

        results = []
        deps = collections.defaultdict(dict)

        def result_at(t):
            i = len(results) - 1
            while i >= 0 and start[i][-1] + LATENCY > t:
                i -= 1
            if i < 0:
                return None
            r = min((t - LATENCY - start[i][-1]) // 8, M // 8 - 1)
            return results[i][r * 8:(r + 1) * 8]

        def tie(t, token):
            if token is not None:
                i = piece_at(t)
                k = 0 if t - start[i][0] < M else NT - 1
                key = k, min(max(t - start[i][k], 0) // 16, M // 16 - 1)
                deps[i][key] = deps[i][key] | token if key in deps[i] else token

        for i, ((dot, _), mb, n) in enumerate(pieces):
            for t, _, limit, fn, args in due.pop(i, []):
                st["go"] = result_at(t) if limit else None
                token = fn(*args)
                if limit:
                    tie(t + limit, token)
            if i >= defer:
                (_, store), mb_s, n_s = pieces[i - defer]
                tie(begin[min(i - defer + fin_lag, len(pieces) - 1)], store(mb_s, n_s, results[i - defer]))
            if i in extra:
                extra[i][0](extra[i][1])
            results.append(dot(mb, n, deps.pop(i, {})))
        for i in range(len(pieces) - defer, len(pieces)):
            (_, store), mb_s, n_s = pieces[i]
            store(mb_s, n_s, results[i])
        assert not due
        for j in range(NM // out_rows):
            o_copy(j).wait()

    scratch = [
        pltpu.VMEM((S, D), bf16),
        pltpu.VMEM((S // 2, D), i32),
        pltpu.VMEM((D + 64, 3 * D), bf16),
        [pltpu.VMEM((D // 2, 128), i32)] * NT,
        [pltpu.VMEM((D // 2, 128), i32)] * (3 * NT),
        pltpu.VMEM((D + 64, D), bf16),
        [pltpu.VMEM((D + 32, 128), f32)] * NT,
        [pltpu.VMEM((D // 2, 128), i32)] * NT,
        pltpu.VMEM((F, D), bf16),
        pltpu.VMEM((F, D), bf16),
        pltpu.VMEM((F, D), bf16),
        [pltpu.VMEM((M // 2, D), i32)] * NM,
        [pltpu.VMEM((NT * QS + 24, 128), f32)] * NM,
        [pltpu.VMEM((NT * KS + 16, 128), f32)] * NM,
        [pltpu.VMEM((NT * KS + 16, 128), f32)] * NM,
        [pltpu.VMEM((M // 2, D), i32)] * NM,
        [pltpu.VMEM((32, 128), f32)] * NSTAT,
        [pltpu.VMEM((32, 128), f32)] * NSTAT,
        [pltpu.VMEM((32, 128), f32)] * NSTAT,
        [pltpu.VMEM((32, 128), f32)] * NSTAT,
        [pltpu.VMEM((W * GA + 32, 128), f32)] * NP,
        pltpu.VMEM((S, D), bf16),
        [pltpu.VMEM((G, D), bf16)] * NSTAT,
        pltpu.VMEM((16, D), bf16),
        pltpu.VMEM((16, F), bf16),
        pltpu.VMEM((D,), bf16),
        pltpu.SemaphoreType.DMA((3,)),
        pltpu.SemaphoreType.DMA((8,)),
        pltpu.SemaphoreType.DMA((NM // out_rows,)),
    ]
    hbm = pl.BlockSpec(memory_space=pltpu.HBM)
    return pl.pallas_call(
        kernel,
        out_shape=jax.ShapeDtypeStruct((S, D), bf16),
        in_specs=[hbm] * 7,
        out_specs=hbm,
        scratch_shapes=scratch,
        compiler_params=pltpu.CompilerParams(vmem_limit_bytes=100 * 1024 * 1024, flags=flags),
        name="fused",
    )


@jax.jit
def pallas_recurrent_scan__sliding_local_dilated__moe_arch_mod__prompt_kernel(
    A_x: jax.Array,
    A_wqkv: jax.Array,
    A_wo: jax.Array,
    B_x: jax.Array,
    B_w_r: jax.Array,
    B_w_gate: jax.Array,
    B_w_up: jax.Array,
    B_w_down: jax.Array,
):
    del B_x
    out = make_kernel(scale_limit=200, scale_lag=2)(A_x.reshape(S, D), A_wqkv, A_wo, B_w_r, B_w_gate.T, B_w_up.T, B_w_down)
    return out.reshape(1, S, D)
```

```python
import bisect
import collections
import functools
import itertools
import math

import jax
import jax.numpy as jnp
import numpy as np
from jax import lax
from jax.experimental import pallas as pl
from jax.experimental.pallas import tpu as pltpu

S, D, F = 2048, 640, 1728
H, DH, W, DIL = 32, 20, 8, 2
NT = D // 128
HALO = 16
M = 128
NM = S // M
G = 16
NG = M // G
NSTAT = 32
NP = 8
QS, KS = M + 8, M + HALO
PIECE = M * NT // 4
LATENCY = 130
LOG2E = math.log2(math.e)
QSCALE = DH ** -0.5 * LOG2E
NEG = -1e9 * LOG2E
EPS_BF16 = float(np.asarray(1e-5, dtype=jnp.bfloat16).astype(np.float32))
f32, bf16, i32 = jnp.float32, jnp.bfloat16, jnp.int32
NT_DIMS = (((1,), (1,)), ((), ()))


def _rb(x):
    return x.astype(bf16).astype(f32)


def _unpack(x):
    return pltpu.bitcast(x, bf16)


def _tree(op, xs):
    while len(xs) > 1:
        xs = [op(a, b) for a, b in zip(xs[::2], xs[1::2])] + xs[len(xs) // 2 * 2:]
    return xs[0]


NF = 2


def make_kernel(att_off=600, att_last=65, fin_lag=3, wo_prep=(-60, -4), split_last=True, qk_lag=2, win=400, pv_off=270, pv_gap=20, sm_off=0,
                ln_off=(0, 18, 40, 55, 72, 90, 95), ln_done=3, scale_lag=2, scale_limit=200, top_gap=400, att_start=100, att_q=12,
                ln_stop=300, defer=2, GA=16, pv_split=((0,), (1,), (2,), (3,), (4,)), w_wait=(8, 44), ln_start=(21, 48), ln_mid=40, NX=6,
                late=144, quiet=250, quiet_off=350, ffn_gap=2, sel_off=(0, 180, 60), sel_gap=(0, 12, 24), gather_gap=(0, 200, 500),
                qk_split=((0,), (1,), (2,), (3,)), qk_off=140, st_off=200, qk_gap=22, exp_off=250, flags=None, nosem=False, NV=5, x_wait=16):
    NA = M // GA

    def kernel(x_hbm, wqkv_hbm, wo_hbm, wr_hbm, wg_hbm, wu_hbm, wd_hbm, out_hbm,
               x_v, z_v, wqkv_raw, wqkv_t, wqkv_p, wo_raw, wo_f, wo_p, wg_v, wu_v, wd_v,
               xn_v, q_s, k_s, v_s, o_v, m_s, d_s, i_s, f_s, p_s, out_v, d_v, xs_v, hid_v, wr_ref, sem_x, sem_w, sem_o):
        xb = (0, NF, NX, NM)
        x_copies = [pltpu.make_async_copy(x_hbm.at[pl.ds(a * M, (b - a) * M), :], x_v.at[pl.ds(a * M, (b - a) * M), :],
                                          sem_x.at[j]) for j, (a, b) in enumerate(zip(xb[:-1], xb[1:]))]
        qkv_copies = [pltpu.make_async_copy(wqkv_hbm.at[:, pl.ds(p * D, D)], wqkv_raw.at[pl.ds(0, D), pl.ds(p * D, D)],
                                            sem_w.at[p]) for p in range(3)]
        late_copies = [pltpu.make_async_copy(s, d, sem_w.at[3 + j]) for j, (s, d) in enumerate(
            [(wo_hbm, wo_raw.at[pl.ds(0, D), :]), (wg_hbm, wg_v), (wu_hbm, wu_v), (wd_hbm, wd_v)])]

        wr_copy = pltpu.make_async_copy(wr_hbm, wr_ref, sem_w.at[7])

        def dma_point(start, wait):
            for c in start:
                c.start()
            for c in wait:
                c.wait()

        dma_point([wr_copy, x_copies[0], qkv_copies[0]], [wr_copy, x_copies[0]])

        lane = lax.broadcasted_iota(i32, (8, 128), 1)
        sub = lax.broadcasted_iota(i32, (8, 128), 0)
        wr = wr_ref[...].astype(f32).reshape(1, D)
        bits = pltpu.bitcast(jnp.broadcast_to(wr[:, :128], (8, 128)), i32) >> 16
        zero = (bits * (bits + 1)) & 1
        zero0 = zero[0, 0]
        fresh = itertools.count(1)
        folds = itertools.count()
        st = dict(folded=[], sums=[], r=[jnp.zeros((8, 128), f32), jnp.zeros((8, 128), f32)])

        done = set()

        def need(*keys):
            assert done.issuperset(keys), keys

        def opaque(align):
            return pl.multiple_of(zero0 * (next(fresh) * align), align)

        def after(ref):
            return pltpu.bitcast(ref[pl.ds(opaque(8), 8), pl.ds(0, 128)], i32)

        def hold(ref, idx):
            if st["go"] is not None:
                ref[idx] = pltpu.bitcast(st["go"], i32) if ref.dtype == i32 else st["go"].astype(ref.dtype)

        def x_rows(g):
            return x_v[pl.ds(g * G + opaque(G), G), :].astype(f32)

        def wide(v):
            return jnp.concatenate([v] * NT, axis=1)

        def get(ref, g):
            need((id(ref), g))
            return ref[g % NSTAT][pl.ds(opaque(8), G), :]

        def put(ref, g, v):
            done.add((id(ref), g))
            ref[g % NSTAT][pl.ds(0, G), :] = jnp.broadcast_to(v, (G, 128))
            return after(ref[g % NSTAT])

        def fold(g, then, v):
            slot_ref = f_s[next(folds) % NSTAT]
            slot_ref[pl.ds(0, G), :] = _tree(jnp.add, [v[:, c * 128:(c + 1) * 128] for c in range(NT)])
            st["folded"].append((then, g, slot_ref))
            return after(slot_ref)

        def ln_reduce():
            sums = []
            for then, g, slot_ref in st["folded"]:
                hold(slot_ref, (pl.ds(G, 8), slice(None)))
                sums.append((then, g, jnp.sum(slot_ref[pl.ds(opaque(8), G), :], axis=1, keepdims=True)))
            st["folded"] = []
            st["sums"].append(sums)

        def ln_finish():
            tokens = [then(g, v) for then, g, v in st["sums"].pop(0)]
            return functools.reduce(jnp.bitwise_or, tokens) if tokens else None

        def ln_mean(g):
            return fold(g, lambda g, v: put(m_s, g, v * (1.0 / D)), x_rows(g))

        def ln_var(g):
            d = x_rows(g) - wide(_rb(get(m_s, g)))
            d_v[g % NSTAT][...] = d.astype(bf16)
            return fold(g, lambda g, v: put(d_s, g, v * (1.0 / D)), d * d)

        def ln_scale(g):
            hold(d_s[g % NSTAT], (pl.ds(G, 8), slice(None)))
            m = get(m_s, g)
            shift = m - _rb(m)
            var = jnp.maximum(get(d_s, g) - shift * shift, 0.0)
            den = jnp.minimum(_rb(jnp.sqrt(_rb(_rb(var) + EPS_BF16))), 3e38)
            inv = pltpu.reciprocal(den, approx=True)
            return put(i_s, g, inv * (2.0 - den * inv))

        def ln_norm(g):
            done.add(("xn", g))
            xn = (d_v[g % NSTAT][pl.ds(opaque(G), G), :].astype(f32) * wide(get(i_s, g))).astype(bf16)
            z_v.bitcast(bf16)[pl.ds(g * G, G), :] = xn
            xn_v[g // NG].bitcast(bf16)[pl.ds(g % NG * G, G), :] = xn
            return after(xn_v[g // NG])

        def keep_score(g, r):
            done.add(("r", g))
            for s in range(G // 8):
                half, l = divmod(g * G // 8 + s, 128)
                rs = jnp.broadcast_to(r[s * 8:(s + 1) * 8], (8, 128))
                st["r"][half] = jnp.where(lane == l, rs, st["r"][half])
            return pltpu.bitcast(st["r"][half], i32)

        def ln_dot(g):
            need(("xn", g))
            xn = _unpack(z_v[pl.ds(g * G // 2 + opaque(8), G // 2), :])
            return fold(g, keep_score, xn.astype(f32) * wr)

        def mod5(n):
            return n - ((n * 205) >> 10) * 5

        src_lane = [(20 * (lane & 31) + 5 * (lane >> 5) + c) & 127 for c in range(NT)]
        turn = mod5((130 - lane) * 2)

        def select(p, b, cs, z):
            rows = pl.ds(z + b * 16, 16)
            tiles = [pltpu.bitcast(wqkv_raw[rows, pl.ds(p * D + t * 128, 128)], i32) for t in range(NT)]
            for step in (1, 2, 4):
                tiles = [jnp.where(turn & step != 0, tiles[(t + step) % NT], tiles[t]) for t in range(NT)]
            return [(c, tiles[2 * c % NT]) for c in cs]

        def gather_lanes(p, c, b, v):
            done.add(("w", p * NT + c))
            wqkv_p[p * NT + c][pl.ds(b * 8, 8), :] = jnp.take_along_axis(
                v, src_lane[c], axis=1, mode="promise_in_bounds")

        def prep_first(p):
            z = opaque(64)
            for b in range(D // 16):
                for c, sel in select(p, b, [0], z):
                    gather_lanes(p, c, b, sel)

        def prep_select(p, j, first, n):
            z = opaque(64)
            for b in range(j * n, (j + 1) * n):
                for c, sel in select(p, b, range(first, NT), z):
                    wqkv_t[pl.ds(c * D // 2 + b * 8, 8), :] = sel
            return after(wqkv_t)

        def prep_gather(p, c):
            hold(wqkv_t, (pl.ds(NT * D // 2, 8), slice(None)))
            z = opaque(8)
            for b in range(D // 16):
                gather_lanes(p, c, b, wqkv_t[pl.ds(z + (c * D // 2 + b * 8), 8), :])

        def wo_widen(t, j):
            wo_f[t][pl.ds(j * 128, 128), :] = wo_raw[pl.ds(j * 128 + opaque(16), 128), pl.ds(t * 128, 128)].astype(f32)
            return after(wo_f[t])

        def wo_perm(t, c):
            done.add(("wo", t, c))
            z = opaque(8)
            for g in range(4):
                blk = wo_f[t][pl.ds(z + (5 * g + c), 32, stride=20), :]
                wo_p[t][pl.ds(c * 64 + g * 16, 16), :] = pltpu.bitcast(blk.astype(bf16), i32)
            return after(wo_p[t])

        def window_pair(ref, z, c, row, w):
            t = ref[pl.ds(z + (row + c * KS + HALO - 8 - DIL * w), GA + 8), :]
            return t[8:], t[:GA]

        def attn_qk(g, ws):
            mb, j = divmod(g, NA)
            z = opaque(8)
            need(*[("qkv", b, n) for b in {mb, max(mb - 1, 0)} for n in range(3 * NT)])
            hold((q_s if ws[0] == 0 else k_s)[mb], (pl.ds(M if ws[0] == 0 else NT * KS, 8), slice(None)))
            if ws[0] == 0:
                st["q"] = [q_s[mb][pl.ds(z + (c * QS + j * GA), GA), :] for c in range(NT)]
            for w in ws:
                ps = None
                for c in range(NT):
                    t = [st["q"][c] * k for k in window_pair(k_s[mb], z, c, j * GA, w)]
                    ps = t if ps is None else [a + b for a, b in zip(ps, t)]
                st["p", g, w] = [(p, pltpu.roll(p, 64, 1)) for p in ps]

        def attn_qk_store(g, ws):
            done.update(("p", g, w) for w in ws)
            for w in ws:
                for ww, (p, r) in zip((w, w + W // 2), st.pop(("p", g, w))):
                    p_s[g % NP][pl.ds(ww * GA, GA), :] = p + r
            return after(p_s[g % NP])

        def attn_logits(g):
            need(*[("p", g, w) for w in range(W // 2)])
            z = opaque(8)
            hold(p_s[g % NP], (pl.ds(W * GA, 8), slice(None)))
            ps = [p_s[g % NP][pl.ds(z + w * GA, GA), :] for w in range(W)]
            st["l", g] = [p + pltpu.roll(p, 32, 1) for p in ps]

        def attn_softmax(g):
            ps = st.pop(("l", g))
            for w in range(W):
                if g * GA < DIL * w:
                    pos = g * GA + lax.broadcasted_iota(i32, (GA, 128), 0)
                    ps[w] = jnp.where(pos >= DIL * w, ps[w], NEG)
            m = _tree(jnp.maximum, ps)
            e = [jnp.exp2(l - m) for l in ps]
            inv = pltpu.reciprocal(_tree(jnp.add, e), approx=True)
            st["e", g] = e, inv
            return pltpu.bitcast(inv[:8], i32) | pltpu.bitcast(inv[GA - 8:], i32)

        def attn_pv(g, cs):
            mb, j = divmod(g, NA)
            z = opaque(8)
            e, inv = st["e", g]
            done.update(("o", g, c) for c in cs)
            token = None
            for c in cs:
                acc = None
                for w in range(W // 2):
                    near, far = window_pair(v_s[mb], z, c, j * GA, w)
                    t = e[w] * near + e[w + W // 2] * far
                    acc = t if acc is None else acc + t
                acc = acc * inv
                for r in range(GA // 8):
                    t = pltpu.bitcast(acc[r * 8:(r + 1) * 8], i32)
                    token = t if token is None else token | t
                if GA == 8:
                    if g % 2 == 0:
                        st["o", c] = acc
                        continue
                    acc = jnp.concatenate([st.pop(("o", c)), acc], axis=0)
                o_v[mb].bitcast(bf16)[pl.ds(j * GA // 16 * 16, 16), pl.ds(c * 128, 128)] = acc.astype(bf16)
            return token

        row = lax.broadcasted_iota(i32, (16, D), 0)

        def tile_of(t):
            return pl.ds(pl.multiple_of((t // 16) * 8, 8), 8)

        def tok(v):
            return pltpu.bitcast(jnp.broadcast_to(v, (8, 128)), i32)

        def top(k):
            if k == 0:
                need(*[("r", g) for g in range(S // G)])
                st["r_all"] = r_all = _rb(jnp.concatenate(st["r"], axis=0))
                st["idx"] = jnp.concatenate([lane * 8 + sub, (lane + 128) * 8 + sub], axis=0).astype(f32)
                st["key"] = jnp.where(r_all == r_all, r_all, -jnp.inf)
                st["free"] = jnp.full((16, 128), True)
                st["i"] = []
            if k % 2 == 0:
                st["max"] = jnp.max(st["key"], keepdims=True)
                return tok(st["max"])
            i = jnp.min(jnp.where((st["key"] == st["max"]) & st["free"], st["idx"], S - 1.0), keepdims=True)
            st["i"].append(i)
            st["free"] = st["idx"] != i
            st["key"] = jnp.where(st["free"], st["key"], -jnp.inf)
            return tok(i)

        def gather():
            st["rs"] = [jnp.sum(jnp.where(st["idx"] == i, st["r_all"], 0.0), keepdims=True) for i in st["i"]]
            st["t"] = [i.astype(i32)[0, 0] for i in st["i"]]

            def pick(t):
                z = _unpack(z_v[tile_of(t), :]).astype(f32)
                return jnp.sum(jnp.where(row == t % 16, z, 0.0), axis=0, keepdims=True)

            xs = jnp.where(row == 0, pick(st["t"][0]), pick(st["t"][1]))
            xs_v[...] = xs.astype(bf16)
            return pltpu.bitcast(xs[:8, :128], i32) | tok(st["rs"][0]) | tok(st["rs"][1])

        def ffn_rows(j):
            return pl.ds(j * 128, min(128, F - j * 128))

        def ffn_gate(j):
            st["gate"] = lax.dot_general(xs_v[...], wg_v[ffn_rows(j), :], NT_DIMS, preferred_element_type=f32)

        def ffn_up(j):
            gate = _rb(st.pop("gate"))
            up = _rb(lax.dot_general(xs_v[...], wu_v[ffn_rows(j), :], NT_DIMS, preferred_element_type=f32))
            hid_v[:, ffn_rows(j)] = (_rb(gate * jax.nn.sigmoid(gate)) * up).astype(bf16)

        def ffn_down(j):
            done.add(("y", j))
            y = jnp.dot(hid_v[:, ffn_rows(j)], wd_v[ffn_rows(j), :], preferred_element_type=f32)[:8]
            st["y"] = y if j == 0 else st["y"] + y

        def patch():
            need(("y", pl.cdiv(F, 128) - 1))
            done.add("patch")
            for j in range(2):
                t = st["t"][j]
                upd = _rb(_rb(st["y"][j:j + 1]) * _rb(jax.nn.sigmoid(st["rs"][j])))
                z = _unpack(z_v[tile_of(t), :]).astype(f32)
                z_v[tile_of(t), :] = pltpu.bitcast(jnp.where(row == t % 16, z + upd, z).astype(bf16), i32)

        def o_copy(rows, cols):
            return pltpu.make_async_copy(out_v.at[rows, cols], out_hbm.at[rows, cols], sem_o)

        def piece_dot(lhs_ref, rhs_ref, deps):
            z = opaque(8)
            cols = []
            for k in range(NT):
                col = lhs_ref[pl.ds(z, M // 2), pl.ds(k * 128, 128)]
                if any(kk == k for kk, _ in deps):
                    parts = [col[r * 8:(r + 1) * 8] for r in range(M // 16)]
                    for (kk, r), t in deps.items():
                        if kk == k:
                            parts[r] = parts[r] | (t & zero)
                    col = jnp.concatenate(parts, axis=0)
                cols.append(col)
            lhs = _unpack(jnp.concatenate(cols, axis=1))
            return jnp.dot(lhs, _unpack(rhs_ref[pl.ds(z, D // 2), :]), preferred_element_type=f32)

        def qkv_dot(mb, n, deps):
            need(("w", n), *[("xn", mb * NG + j) for j in range(NG)])
            return piece_dot(xn_v[mb], wqkv_p[n], deps)

        def qkv_store(mb, n, res):
            done.add(("qkv", mb, n))
            p, c = divmod(n, NT)
            if p == 0:
                q_s[mb][pl.ds(c * QS, M), :] = res * QSCALE
            else:
                dst = (k_s, v_s)[p - 1]
                dst[mb][pl.ds(c * KS + HALO, M), :] = res
                if mb == 0:
                    dst[0][pl.ds(c * KS, HALO), :] = jnp.broadcast_to(res[0:1], (HALO, 128))
                if mb + 1 < NM:
                    dst[mb + 1][pl.ds(c * KS, HALO), :] = res[M - HALO:]

        def out_dot(mb, c, deps):
            need(*[("wo", c, k) for k in range(NT)], *[("o", mb * NA + j, k) for j in range(NA) for k in range(NT)])
            return piece_dot(o_v[mb], wo_p[c], deps)

        def out_store(mb, c, s):
            need("patch")
            cols = pl.ds(c * 128, 128)
            z = _unpack(z_v[pl.ds(mb * M // 2 + opaque(8), M // 2), cols]).astype(f32)
            gate = z * pltpu.reciprocal(1.0 + jnp.exp2(z * -LOG2E), approx=True)
            res = x_v[pl.ds(mb * M + opaque(16), M), cols].astype(f32) + s * gate
            out_v[pl.ds(mb * M, M), cols] = res.astype(bf16)
            if mb == NM - 1 and split_last:
                o_copy(pl.ds(mb * M, M), cols).start()
            elif c == NT - 1:
                o_copy(pl.ds(mb * M, M), slice(None)).start()
            return pltpu.bitcast(res[M - 8:], i32)

        qkv, out = (qkv_dot, qkv_store), (out_dot, out_store)
        pieces = [(qkv, mb, n) for n in range(2 * NT) for mb in range(NF)]
        pieces += [(qkv, mb, n) for mb in range(NF, NV) for n in range(2 * NT)]
        pieces += [(qkv, mb, n) for n in range(2 * NT, 3 * NT) for mb in range(NV)]
        pieces += [(qkv, mb, n) for mb in range(NV, NM) for n in range(3 * NT)]
        nq = len(pieces)
        pieces += [(out, mb, c) for mb in range(NM) for c in range(NT)]
        nf = pl.cdiv(F, 128)
        extra = {}
        for j in range(nf):
            extra[late + 1 + 2 * j * ffn_gap] = ffn_gate, j
            extra[late + 1 + (2 * j + 1) * ffn_gap] = ffn_up, j
            extra[late + 4 + (2 * nf + j) * ffn_gap] = ffn_down, j
        busy, start = [0] * 4, []
        for i in range(len(pieces)):
            for rows in ([16] * NT if i in extra else []) + [M] * NT:
                m = busy.index(min(busy))
                if rows == M:
                    start.append(busy[m])
                busy[m] += rows
        start = np.reshape(start, (-1, NT)).tolist()
        begin = [0]
        for i in range(1, len(pieces)):
            begin.append(max(start[i][0], min(begin[-1] + PIECE, start[i - 1][-1] + M - 1)))
        end_q = begin[nq]
        tasks = []

        def at(t, limit, fn, *args):
            tasks.append((t, len(tasks), limit, fn, args))

        def piece_at(t):
            return bisect.bisect_right(begin, t) - 1

        stages = (ln_mean, ln_var, ln_scale, ln_norm, ln_dot)

        def ln_steps(lo, hi, a, b, done):
            lags = (0, done + 1, 2 * done + 2, 2 * done + 3 + scale_lag, 2 * done + 4 + scale_lag)
            n = hi - lo + lags[-1] + done
            for t in range(n):
                def time(off):
                    return a + (t * 100 + off) * (b - a) // (100 * n)

                for k, fn, off in zip(lags, stages, ln_off):
                    if 0 <= t - k < hi - lo:
                        at(time(off), (scale_limit if fn is ln_scale else 1) if b else 0, fn, lo + t - k)
                if t < n - done:
                    at(time(ln_off[5]), 1 if b else 0, ln_reduce)
                if t >= done:
                    at(time(ln_off[6]), 1 if b else 0, ln_finish)

        ln_steps(0, NF * NG, 0, 0, 3)
        starts = ((qkv_copies[1], x_copies[1]), qkv_copies[2:], late_copies)
        waits = (qkv_copies[:1], qkv_copies[1:2], (qkv_copies[2], x_copies[2]))
        for p, first in enumerate((0,) + w_wait):
            t = first * PIECE
            at(t, 0, dma_point, starts[p], waits[p])
            quick = int(p < 2)
            if quick:
                at(t, 0, prep_first, p)
            for j in range(20):
                at(t + sel_off[p] + j * sel_gap[p] if p else 0, 1 if p else 0, prep_select, p, j, quick, 2)
            for c in range(quick, NT):
                at(t + sel_off[p] + 20 * sel_gap[p] + (c - quick) * gather_gap[p] if p else 0, 1, prep_gather, p, c)
        at(x_wait * PIECE, 0, dma_point, x_copies[2:], x_copies[1:2])
        ln_steps(NF * NG, (NF + 1) * NG, x_wait * PIECE, ln_start[0] * PIECE, ln_done)
        ln_steps((NF + 1) * NG, NX * NG, ln_start[0] * PIECE, ln_mid * PIECE, ln_done)
        base = att_start * PIECE
        ln_steps(NX * NG, NM * NG, ln_start[1] * PIECE, base - ln_stop, ln_done)
        for k in range(4):
            at(base + k * top_gap, win, top, k)
        at(base + 4 * top_gap, win, gather)

        def slot(g):
            if g < att_q * NA:
                t = base + (g + qk_lag) * (end_q + att_off - base - quiet) // (att_q * NA + qk_lag)
                return t + quiet if t > begin[late] - quiet - quiet_off else t
            return end_q + att_off + (g - att_q * NA) * att_last * PIECE // ((NM - att_q) * NA)

        for g in range(NM * NA):
            for n, ws in enumerate(qk_split):
                at(slot(g - qk_lag) + qk_off + n * qk_gap, win, attn_qk, g, ws)
                at(slot(g - qk_lag) + qk_off + n * qk_gap + st_off, 1, attn_qk_store, g, ws)
            at(slot(g) + sm_off, win, attn_logits, g)
            at(slot(g) + sm_off + exp_off, 1, attn_softmax, g)
            for n, cs in enumerate(pv_split):
                at(slot(g) + pv_off + n * pv_gap, 1, attn_pv, g, cs)
        at(begin[late], 0, dma_point, [], late_copies)
        for j in range(2 * NT * NT):
            t = end_q + wo_prep[0] * PIECE + j * (wo_prep[1] - wo_prep[0]) * PIECE // (2 * NT * NT)
            at(t, 1, (wo_widen, wo_perm)[j // NT % 2], j // (2 * NT), j % NT)
        at(begin[nq - 2], 0, patch)

        due = collections.defaultdict(list)
        for task in sorted(tasks, key=lambda task: task[:2]):
            due[piece_at(task[0])].append(task)

        results = []
        deps = collections.defaultdict(dict)

        def result_at(t):
            i = len(results) - 1
            while i >= 0 and start[i][-1] + LATENCY > t:
                i -= 1
            if i < 0:
                return None
            r = min((t - LATENCY - start[i][-1]) // 8, M // 8 - 1)
            return results[i][r * 8:(r + 1) * 8]

        def tie(t, token):
            if token is not None:
                i = piece_at(t)
                k = 0 if t - start[i][0] < M else NT - 1
                key = k, min(max(t - start[i][k], 0) // 16, M // 16 - 1)
                deps[i][key] = deps[i][key] | token if key in deps[i] else token

        for i, ((dot, _), mb, n) in enumerate(pieces):
            for t, _, limit, fn, args in due.pop(i, []):
                st["go"] = result_at(t) if limit else None
                token = fn(*args)
                if limit:
                    tie(t + limit, token)
            if i >= defer:
                (_, store), mb_s, n_s = pieces[i - defer]
                tie(begin[min(i - defer + fin_lag, len(pieces) - 1)], store(mb_s, n_s, results[i - defer]))
            if i in extra:
                extra[i][0](extra[i][1])
            results.append(dot(mb, n, deps.pop(i, {})))
        for i in range(len(pieces) - defer, len(pieces)):
            (_, store), mb_s, n_s = pieces[i]
            store(mb_s, n_s, results[i])
        assert not due
        pltpu.make_async_copy(out_v, out_hbm, sem_o).wait()

    scratch = [
        pltpu.VMEM((S, D), bf16),
        pltpu.VMEM((S // 2, D), i32),
        pltpu.VMEM((D + 64, 3 * D), bf16),
        pltpu.VMEM((NT * D // 2 + 32, 128), i32),
        [pltpu.VMEM((D // 2, 128), i32)] * (3 * NT),
        pltpu.VMEM((D + 64, D), bf16),
        [pltpu.VMEM((D + 32, 128), f32)] * NT,
        [pltpu.VMEM((D // 2, 128), i32)] * NT,
        pltpu.VMEM((F, D), bf16),
        pltpu.VMEM((F, D), bf16),
        pltpu.VMEM((F, D), bf16),
        [pltpu.VMEM((M // 2, D), i32)] * NM,
        [pltpu.VMEM((NT * QS + 24, 128), f32)] * NM,
        [pltpu.VMEM((NT * KS + 16, 128), f32)] * NM,
        [pltpu.VMEM((NT * KS + 16, 128), f32)] * NM,
        [pltpu.VMEM((M // 2, D), i32)] * NM,
        [pltpu.VMEM((32, 128), f32)] * NSTAT,
        [pltpu.VMEM((32, 128), f32)] * NSTAT,
        [pltpu.VMEM((32, 128), f32)] * NSTAT,
        [pltpu.VMEM((32, 128), f32)] * NSTAT,
        [pltpu.VMEM((W * GA + 32, 128), f32)] * NP,
        pltpu.VMEM((S, D), bf16),
        [pltpu.VMEM((G, D), bf16)] * NSTAT,
        pltpu.VMEM((16, D), bf16),
        pltpu.VMEM((16, F), bf16),
        pltpu.VMEM((D,), bf16),
        pltpu.SemaphoreType.DMA((3,)),
        pltpu.SemaphoreType.DMA((8,)),
        pltpu.SemaphoreType.DMA(()),
    ]
    hbm = pl.BlockSpec(memory_space=pltpu.HBM)
    return pl.pallas_call(
        kernel,
        out_shape=jax.ShapeDtypeStruct((S, D), bf16),
        in_specs=[hbm] * 7,
        out_specs=hbm,
        scratch_shapes=scratch,
        compiler_params=pltpu.CompilerParams(vmem_limit_bytes=100 * 1024 * 1024, flags=flags, disable_semaphore_checks=nosem),
        name="fused",
    )


@jax.jit
def pallas_recurrent_scan__sliding_local_dilated__moe_arch_mod__prompt_kernel(
    A_x: jax.Array,
    A_wqkv: jax.Array,
    A_wo: jax.Array,
    B_x: jax.Array,
    B_w_r: jax.Array,
    B_w_gate: jax.Array,
    B_w_up: jax.Array,
    B_w_down: jax.Array,
):
    del B_x
    out = make_kernel()(A_x.reshape(S, D), A_wqkv, A_wo, B_w_r, B_w_gate.T, B_w_up.T, B_w_down)
    return out.reshape(1, S, D)
```

```python
import bisect
import collections
import functools
import itertools
import math

import jax
import jax.numpy as jnp
import numpy as np
from jax import lax
from jax.experimental import pallas as pl
from jax.experimental.pallas import tpu as pltpu

S, D, F = 2048, 640, 1728
H, DH, W, DIL = 32, 20, 8, 2
NT = D // 128
HALO = 16
M = 128
NM = S // M
G = 16
NG = M // G
NSTAT = 32
NP = 8
QS, KS = M + 8, M + HALO
PIECE = M * NT // 4
LATENCY = 130
LOG2E = math.log2(math.e)
QSCALE = DH ** -0.5 * LOG2E
NEG = -1e9 * LOG2E
EPS_BF16 = float(np.asarray(1e-5, dtype=jnp.bfloat16).astype(np.float32))
f32, bf16, i32 = jnp.float32, jnp.bfloat16, jnp.int32
NT_DIMS = (((1,), (1,)), ((), ()))


def _rb(x):
    return x.astype(bf16).astype(f32)


def _unpack(x):
    return pltpu.bitcast(x, bf16)


def _tree(op, xs):
    while len(xs) > 1:
        xs = [op(a, b) for a, b in zip(xs[::2], xs[1::2])] + xs[len(xs) // 2 * 2:]
    return xs[0]


NF = 2


def make_kernel(att_off=600, att_last=65, fin_lag=4, wo_prep=(-60, -4), split_last=True, qk_lag=2, win=400, pv_off=270, pv_gap=20, sm_off=0,
                ln_off=(0, 18, 40, 55, 72, 90, 95), ln_done=3, scale_lag=2, scale_limit=200, top_gap=400, att_start=100, att_rate=(1.0, 1e-6, 1.0, 1.0, 0.75),
                ln_stop=300, defer=2, GA=16, pv_split=((0,), (1,), (2,), (3,), (4,)), w_wait=(8, 44), ln_start=(21, 48), ln_mid=40, NX=6,
                late=144, quiet=200, quiet_off=380, ffn_gap=2, sel_off=(64, 260, 60), sel_gap=(12, 16, 24),
                gather_gap=(150, 150, 500),
                qk_split=((0,), (1,), (2,), (3,)), qk_off=140, st_off=200, qk_gap=22, exp_off=250, flags=None, interpret=False, nosem=False, NV=5, x_wait=16):
    NA = M // GA

    def kernel(x_hbm, wqkv_hbm, wo_hbm, wr_hbm, wg_hbm, wu_hbm, wd_hbm, out_hbm,
               x_v, z_v, wqkv_raw, wqkv_t, wqkv_p, wo_raw, wo_f, wo_p, wg_v, wu_v, wd_v,
               xn_v, q_s, k_s, v_s, o_v, m_s, d_s, i_s, f_s, p_s, out_v, d_v, xs_v, hid_v, wr_ref, sem_x, sem_w, sem_o):
        xb = (0, NF, NX, NM)
        x_copies = [pltpu.make_async_copy(x_hbm.at[pl.ds(a * M, (b - a) * M), :], x_v.at[pl.ds(a * M, (b - a) * M), :],
                                          sem_x.at[j]) for j, (a, b) in enumerate(zip(xb[:-1], xb[1:]))]
        qkv_copies = [pltpu.make_async_copy(wqkv_hbm.at[:, pl.ds(p * D, D)], wqkv_raw.at[:, pl.ds(p * D, D)],
                                            sem_w.at[p]) for p in range(3)]
        late_copies = [pltpu.make_async_copy(s, d, sem_w.at[3 + j]) for j, (s, d) in enumerate(
            [(wo_hbm, wo_raw), (wg_hbm, wg_v), (wu_hbm, wu_v), (wd_hbm, wd_v)])]

        wr_copy = pltpu.make_async_copy(wr_hbm, wr_ref, sem_w.at[7])

        def dma_point(start, wait):
            for c in start:
                c.start()
            for c in wait:
                c.wait()

        dma_point([wr_copy, x_copies[0]], [wr_copy])
        dma_point(qkv_copies[:2], x_copies[:1])

        lane = lax.broadcasted_iota(i32, (8, 128), 1)
        sub = lax.broadcasted_iota(i32, (8, 128), 0)
        wr = wr_ref[...].astype(f32).reshape(1, D)
        bits = pltpu.bitcast(jnp.broadcast_to(wr[:, :128], (8, 128)), i32) >> 16
        zero = (bits * (bits + 1)) & 1
        zero0 = zero[0, 0]
        fresh = itertools.count(1)
        folds = itertools.count()
        st = dict(folded=[], sums=[], r=[jnp.zeros((8, 128), f32), jnp.zeros((8, 128), f32)])

        done = set()

        def need(*keys):
            assert done.issuperset(keys), keys

        def opaque(align):
            return pl.multiple_of(zero0 * (next(fresh) * align), align)

        def after(ref, row=0):
            return pltpu.bitcast(ref[pl.ds(opaque(8) + row, 8), pl.ds(0, 128)], i32)

        def hold(ref, idx):
            if st["go"] is not None:
                ref[idx] = pltpu.bitcast(st["go"], i32) if ref.dtype == i32 else st["go"].astype(ref.dtype)

        def x_rows(g):
            return x_v[pl.ds(g * G + opaque(G), G), :].astype(f32)

        def wide(v):
            return jnp.concatenate([v] * NT, axis=1)

        def get(ref, g):
            need((id(ref), g))
            return ref[g % NSTAT][pl.ds(opaque(8), G), :]

        def put(ref, g, v):
            done.add((id(ref), g))
            ref[g % NSTAT][pl.ds(0, G), :] = jnp.broadcast_to(v, (G, 128))
            return after(ref[g % NSTAT])

        def fold(g, then, v):
            slot_ref = f_s[next(folds) % NSTAT]
            slot_ref[pl.ds(0, G), :] = _tree(jnp.add, [v[:, c * 128:(c + 1) * 128] for c in range(NT)])
            st["folded"].append((then, g, slot_ref))
            return after(slot_ref)

        def ln_reduce():
            sums = []
            for then, g, slot_ref in st["folded"]:
                hold(slot_ref, (pl.ds(G, 8), slice(None)))
                sums.append((then, g, jnp.sum(slot_ref[pl.ds(opaque(8), G), :], axis=1, keepdims=True)))
            st["folded"] = []
            st["sums"].append(sums)

        def ln_finish():
            tokens = [then(g, v) for then, g, v in st["sums"].pop(0)]
            return functools.reduce(jnp.bitwise_or, tokens) if tokens else None

        def ln_mean(g):
            return fold(g, lambda g, v: put(m_s, g, v * (1.0 / D)), x_rows(g))

        def ln_var(g):
            d = x_rows(g) - wide(_rb(get(m_s, g)))
            d_v[g % NSTAT][...] = d.astype(bf16)
            return fold(g, lambda g, v: put(d_s, g, v * (1.0 / D)), d * d)

        def ln_scale(g):
            hold(d_s[g % NSTAT], (pl.ds(G, 8), slice(None)))
            m = get(m_s, g)
            shift = m - _rb(m)
            var = jnp.maximum(get(d_s, g) - shift * shift, 0.0)
            den = jnp.minimum(_rb(jnp.sqrt(_rb(_rb(var) + EPS_BF16))), 3e38)
            inv = pltpu.reciprocal(den, approx=True)
            return put(i_s, g, inv * (2.0 - den * inv))

        def ln_norm(g):
            done.add(("xn", g))
            xn = (d_v[g % NSTAT][pl.ds(opaque(G), G), :].astype(f32) * wide(get(i_s, g))).astype(bf16)
            z_v.bitcast(bf16)[pl.ds(g * G, G), :] = xn
            xn_v[g // NG].bitcast(bf16)[pl.ds(g % NG * G, G), :] = xn
            return after(xn_v[g // NG])

        def keep_score(g, r):
            done.add(("r", g))
            for s in range(G // 8):
                half, l = divmod(g * G // 8 + s, 128)
                rs = jnp.broadcast_to(r[s * 8:(s + 1) * 8], (8, 128))
                st["r"][half] = jnp.where(lane == l, rs, st["r"][half])
            return pltpu.bitcast(st["r"][half], i32)

        def ln_dot(g):
            need(("xn", g))
            xn = _unpack(z_v[pl.ds(g * G // 2 + opaque(8), G // 2), :])
            return fold(g, keep_score, xn.astype(f32) * wr)

        def mod5(n):
            return n - ((n * 205) >> 10) * 5

        src_lane = [(20 * (lane & 31) + 5 * (lane >> 5) + c) & 127 for c in range(NT)]
        turn = mod5((130 - lane) * 2)
        turns = [(step, turn & step != 0) for step in (1, 2, 4)]

        def select(p, b, cs, z):
            rows = pl.ds(z + b * 16, 16)
            tiles = [pltpu.bitcast(wqkv_raw[rows, pl.ds(p * D + t * 128, 128)], i32) for t in range(NT)]
            for step, mask in turns:
                tiles = [jnp.where(mask, tiles[(t + step) % NT], tiles[t]) for t in range(NT)]
            return [(c, tiles[2 * c % NT]) for c in cs]

        def gather_lanes(p, c, b, v):
            done.add(("w", p * NT + c))
            wqkv_p[p * NT + c][pl.ds(b * 8, 8), :] = jnp.take_along_axis(
                v, src_lane[c], axis=1, mode="promise_in_bounds")

        def prep_first(p):
            z = opaque(64)
            for b in range(D // 16):
                (_, first), (_, second) = select(p, b, [0, 1], z)
                gather_lanes(p, 0, b, first)
                wqkv_t[pl.ds(D // 2 + b * 8, 8), :] = second

        def prep_select(p, j, first, n):
            z = opaque(64)
            for b in range(j * n, (j + 1) * n):
                for c, sel in select(p, b, range(first, NT), z):
                    wqkv_t[pl.ds(c * D // 2 + b * 8, 8), :] = sel
            return after(wqkv_t, (NT - 1) * D // 2)

        def prep_gather(p, c):
            hold(wqkv_t, (pl.ds(NT * D // 2, 8), slice(None)))
            z = opaque(8)
            for b in range(D // 16):
                gather_lanes(p, c, b, wqkv_t[pl.ds(z + (c * D // 2 + b * 8), 8), :])

        def wo_widen(t, j):
            wo_f[t][pl.ds(j * 128, 128), :] = wo_raw[pl.ds(j * 128 + opaque(16), 128), pl.ds(t * 128, 128)].astype(f32)
            return after(wo_f[t])

        def wo_perm(t, c):
            done.add(("wo", t, c))
            z = opaque(8)
            for g in range(4):
                blk = wo_f[t][pl.ds(z + (5 * g + c), 32, stride=20), :]
                wo_p[t][pl.ds(c * 64 + g * 16, 16), :] = pltpu.bitcast(blk.astype(bf16), i32)
            return after(wo_p[t])

        def window_pair(ref, z, c, row, w):
            t = ref[pl.ds(z + (row + c * KS + HALO - 8 - DIL * w), GA + 8), :]
            return t[8:], t[:GA]

        def attn_qk(g, ws):
            mb, j = divmod(g, NA)
            z = opaque(8)
            need(*[("qkv", b, n) for b in {mb, max(mb - 1, 0)} for n in range(3 * NT)])
            hold((q_s if ws[0] == 0 else k_s)[mb], (pl.ds(M if ws[0] == 0 else NT * KS, 8), slice(None)))
            if ws[0] == 0:
                st["q"] = [q_s[mb][pl.ds(z + (c * QS + j * GA), GA), :] for c in range(NT)]
            for w in ws:
                ps = None
                for c in range(NT):
                    t = [st["q"][c] * k for k in window_pair(k_s[mb], z, c, j * GA, w)]
                    ps = t if ps is None else [a + b for a, b in zip(ps, t)]
                st["p", g, w] = [(p, pltpu.roll(p, 64, 1)) for p in ps]

        def attn_qk_store(g, ws):
            done.update(("p", g, w) for w in ws)
            for w in ws:
                for ww, (p, r) in zip((w, w + W // 2), st.pop(("p", g, w))):
                    p_s[g % NP][pl.ds(ww * GA, GA), :] = p + r
            return after(p_s[g % NP])

        def attn_logits(g):
            need(*[("p", g, w) for w in range(W // 2)])
            z = opaque(8)
            hold(p_s[g % NP], (pl.ds(W * GA, 8), slice(None)))
            ps = [p_s[g % NP][pl.ds(z + w * GA, GA), :] for w in range(W)]
            st["l", g] = [p + pltpu.roll(p, 32, 1) for p in ps]

        def attn_softmax(g):
            ps = st.pop(("l", g))
            for w in range(W):
                if g * GA < DIL * w:
                    pos = g * GA + lax.broadcasted_iota(i32, (GA, 128), 0)
                    ps[w] = jnp.where(pos >= DIL * w, ps[w], NEG)
            m = _tree(jnp.maximum, ps)
            e = [jnp.exp2(l - m) for l in ps]
            inv = pltpu.reciprocal(_tree(jnp.add, e), approx=True)
            st["e", g] = e, inv
            return pltpu.bitcast(inv[:8], i32) | pltpu.bitcast(inv[GA - 8:], i32)

        def attn_pv(g, cs):
            mb, j = divmod(g, NA)
            z = opaque(8)
            e, inv = st["e", g]
            done.update(("o", g, c) for c in cs)
            token = None
            for c in cs:
                acc = None
                for w in range(W // 2):
                    near, far = window_pair(v_s[mb], z, c, j * GA, w)
                    t = e[w] * near + e[w + W // 2] * far
                    acc = t if acc is None else acc + t
                acc = acc * inv
                for r in range(GA // 8):
                    t = pltpu.bitcast(acc[r * 8:(r + 1) * 8], i32)
                    token = t if token is None else token | t
                if GA == 8:
                    if g % 2 == 0:
                        st["o", c] = acc
                        continue
                    acc = jnp.concatenate([st.pop(("o", c)), acc], axis=0)
                o_v[mb].bitcast(bf16)[pl.ds(j * GA // 16 * 16, 16), pl.ds(c * 128, 128)] = acc.astype(bf16)
            return token

        row = lax.broadcasted_iota(i32, (16, D), 0)

        def tile_of(t):
            return pl.ds(pl.multiple_of((t // 16) * 8, 8), 8)

        def tok(v):
            return pltpu.bitcast(jnp.broadcast_to(v, (8, 128)), i32)

        def top(k):
            if k == 0:
                need(*[("r", g) for g in range(S // G)])
                st["r_all"] = r_all = _rb(jnp.concatenate(st["r"], axis=0))
                st["idx"] = jnp.concatenate([lane * 8 + sub, (lane + 128) * 8 + sub], axis=0).astype(f32)
                st["key"] = jnp.where(r_all == r_all, r_all, -jnp.inf)
                st["free"] = jnp.full((16, 128), True)
                st["i"] = []
            if k % 2 == 0:
                st["max"] = jnp.max(st["key"], keepdims=True)
                return tok(st["max"])
            i = jnp.min(jnp.where((st["key"] == st["max"]) & st["free"], st["idx"], S - 1.0), keepdims=True)
            st["i"].append(i)
            st["free"] = st["idx"] != i
            st["key"] = jnp.where(st["free"], st["key"], -jnp.inf)
            return tok(i)

        def gather():
            st["rs"] = [jnp.sum(jnp.where(st["idx"] == i, st["r_all"], 0.0), keepdims=True) for i in st["i"]]
            st["t"] = [i.astype(i32)[0, 0] for i in st["i"]]

            def pick(t):
                z = _unpack(z_v[tile_of(t), :]).astype(f32)
                return jnp.sum(jnp.where(row == t % 16, z, 0.0), axis=0, keepdims=True)

            xs = jnp.where(row == 0, pick(st["t"][0]), pick(st["t"][1]))
            xs_v[...] = xs.astype(bf16)
            return pltpu.bitcast(xs[:8, :128], i32) | tok(st["rs"][0]) | tok(st["rs"][1])

        def ffn_rows(j):
            return pl.ds(j * 128, min(128, F - j * 128))

        def ffn_gate(j):
            st["gate"] = lax.dot_general(xs_v[...], wg_v[ffn_rows(j), :], NT_DIMS, preferred_element_type=f32)

        def ffn_up(j):
            gate = _rb(st.pop("gate"))
            up = _rb(lax.dot_general(xs_v[...], wu_v[ffn_rows(j), :], NT_DIMS, preferred_element_type=f32))
            hid_v[:, ffn_rows(j)] = (_rb(gate * jax.nn.sigmoid(gate)) * up).astype(bf16)

        def ffn_down(j):
            done.add(("y", j))
            y = jnp.dot(hid_v[:, ffn_rows(j)], wd_v[ffn_rows(j), :], preferred_element_type=f32)[:8]
            st["y"] = y if j == 0 else st["y"] + y

        def patch():
            need(("y", pl.cdiv(F, 128) - 1))
            done.add("patch")
            for j in range(2):
                t = st["t"][j]
                upd = _rb(_rb(st["y"][j:j + 1]) * _rb(jax.nn.sigmoid(st["rs"][j])))
                z = _unpack(z_v[tile_of(t), :]).astype(f32)
                z_v[tile_of(t), :] = pltpu.bitcast(jnp.where(row == t % 16, z + upd, z).astype(bf16), i32)

        def o_copy(rows, cols):
            return pltpu.make_async_copy(out_v.at[rows, cols], out_hbm.at[rows, cols], sem_o)

        def piece_dot(lhs_ref, rhs_ref, deps):
            z = opaque(8)
            cols = []
            for k in range(NT):
                col = lhs_ref[pl.ds(z, M // 2), pl.ds(k * 128, 128)]
                if any(kk == k for kk, _ in deps):
                    parts = [col[r * 8:(r + 1) * 8] for r in range(M // 16)]
                    for (kk, r), t in deps.items():
                        if kk == k:
                            parts[r] = parts[r] | (t & zero)
                    col = jnp.concatenate(parts, axis=0)
                cols.append(col)
            lhs = _unpack(jnp.concatenate(cols, axis=1))
            return jnp.dot(lhs, _unpack(rhs_ref[pl.ds(z, D // 2), :]), preferred_element_type=f32)

        def qkv_dot(mb, n, deps):
            need(("w", n), *[("xn", mb * NG + j) for j in range(NG)])
            return piece_dot(xn_v[mb], wqkv_p[n], deps)

        def qkv_store(mb, n, res):
            done.add(("qkv", mb, n))
            p, c = divmod(n, NT)
            if p == 0:
                q_s[mb][pl.ds(c * QS, M), :] = res * QSCALE
            else:
                dst = (k_s, v_s)[p - 1]
                dst[mb][pl.ds(c * KS + HALO, M), :] = res
                if mb == 0:
                    dst[0][pl.ds(c * KS, HALO), :] = jnp.broadcast_to(res[0:1], (HALO, 128))
                if mb + 1 < NM:
                    dst[mb + 1][pl.ds(c * KS, HALO), :] = res[M - HALO:]

        def out_dot(mb, c, deps):
            need(*[("wo", c, k) for k in range(NT)], *[("o", mb * NA + j, k) for j in range(NA) for k in range(NT)])
            return piece_dot(o_v[mb], wo_p[c], deps)

        def out_store(mb, c, s):
            need("patch")
            cols = pl.ds(c * 128, 128)
            z = _unpack(z_v[pl.ds(mb * M // 2 + opaque(8), M // 2), cols]).astype(f32)
            gate = z * pltpu.reciprocal(1.0 + jnp.exp2(z * -LOG2E), approx=True)
            res = x_v[pl.ds(mb * M + opaque(16), M), cols].astype(f32) + s * gate
            out_v[pl.ds(mb * M, M), cols] = res.astype(bf16)
            if mb == NM - 1 and split_last:
                o_copy(pl.ds(mb * M, M), cols).start()
            elif c == NT - 1:
                o_copy(pl.ds(mb * M, M), slice(None)).start()
            return pltpu.bitcast(res[M - 8:], i32)

        qkv, out = (qkv_dot, qkv_store), (out_dot, out_store)
        pieces = [(qkv, mb, n) for n in range(2 * NT) for mb in range(NF)]
        pieces += [(qkv, mb, n) for mb in range(NF, NV) for n in range(2 * NT)]
        pieces += [(qkv, mb, n) for n in range(2 * NT, 3 * NT) for mb in range(NV)]
        pieces += [(qkv, mb, n) for mb in range(NV, NM) for n in range(3 * NT)]
        nq = len(pieces)
        pieces += [(out, mb, c) for mb in range(NM) for c in range(NT)]
        nf = pl.cdiv(F, 128)
        extra = {}
        for j in range(nf):
            extra[late + 1 + int(2 * j * ffn_gap)] = ffn_gate, j
            extra[late + 1 + int((2 * j + 1) * ffn_gap)] = ffn_up, j
            extra[late + 4 + int((2 * nf + j) * ffn_gap)] = ffn_down, j
        busy, start = [0] * 4, []
        for i in range(len(pieces)):
            for rows in ([16] * NT if i in extra else []) + [M] * NT:
                m = busy.index(min(busy))
                if rows == M:
                    start.append(busy[m])
                busy[m] += rows
        start = np.reshape(start, (-1, NT)).tolist()
        begin = [0]
        for i in range(1, len(pieces)):
            begin.append(max(start[i][0], min(begin[-1] + PIECE, start[i - 1][-1] + M - 1)))
        end_q = begin[nq]
        tasks = []

        def at(t, limit, fn, *args):
            tasks.append((t, len(tasks), limit, fn, args))

        def piece_at(t):
            return bisect.bisect_right(begin, t) - 1

        stages = (ln_mean, ln_var, ln_scale, ln_norm, ln_dot)

        def ln_steps(lo, hi, a, b, done):
            lags = (0, done + 1, 2 * done + 2, 2 * done + 3 + scale_lag, 2 * done + 4 + scale_lag)
            n = hi - lo + lags[-1] + done
            for t in range(n):
                def time(off):
                    return a + (t * 100 + off) * (b - a) // (100 * n)

                for k, fn, off in zip(lags, stages, ln_off):
                    if 0 <= t - k < hi - lo:
                        at(time(off), (scale_limit if fn is ln_scale else 1) if b else 0, fn, lo + t - k)
                if t < n - done:
                    at(time(ln_off[5]), 1 if b else 0, ln_reduce)
                if t >= done:
                    at(time(ln_off[6]), 1 if b else 0, ln_finish)

        ln_steps(0, NF * NG, 0, 0, 3)
        starts = (x_copies[1:2], qkv_copies[2:], late_copies)
        waits = (qkv_copies[:1], qkv_copies[1:2], (qkv_copies[2], x_copies[2]))
        for p, first in enumerate((0,) + w_wait):
            t = first * PIECE
            at(t, 0, dma_point, starts[p], waits[p])
            quick = 2 * (p < 2)
            if quick:
                at(t, 0, prep_first, p)
                at(t, 0, prep_gather, p, 1)
            for j in range(20):
                at(t + sel_off[p] + j * sel_gap[p], 1, prep_select, p, j, quick, 2)
            for c in range(quick, NT):
                at(t + sel_off[p] + 20 * sel_gap[p] + (c - quick) * gather_gap[p], 1, prep_gather, p, c)
        at(x_wait * PIECE, 0, dma_point, x_copies[2:], x_copies[1:2])
        ln_steps(NF * NG, (NF + 1) * NG, x_wait * PIECE, ln_start[0] * PIECE, ln_done)
        ln_steps((NF + 1) * NG, NX * NG, ln_start[0] * PIECE, ln_mid * PIECE, ln_done)
        base = att_start * PIECE
        ln_steps(NX * NG, NM * NG, ln_start[1] * PIECE, base - ln_stop, ln_done)
        for k in range(4):
            at(base + k * top_gap, win, top, k)
        at(base + 4 * top_gap, win, gather)

        knots = [base, begin[late] - quiet - quiet_off, begin[late] - quiet_off, begin[max(extra)],
                 end_q + att_off, end_q + att_off + att_last * PIECE]
        work = np.cumsum([0] + [(b - a) * rate for a, b, rate in zip(knots, knots[1:], att_rate)])

        def slot(g):
            return int(np.interp((g + qk_lag) * work[-1] / (NM * NA + qk_lag), work, knots))

        for g in range(NM * NA):
            for n, ws in enumerate(qk_split):
                at(slot(g - qk_lag) + qk_off + n * qk_gap, win, attn_qk, g, ws)
                at(slot(g - qk_lag) + qk_off + n * qk_gap + st_off, 1, attn_qk_store, g, ws)
            at(slot(g) + sm_off, win, attn_logits, g)
            at(slot(g) + sm_off + exp_off, 1, attn_softmax, g)
            for n, cs in enumerate(pv_split):
                at(slot(g) + pv_off + n * pv_gap, 1, attn_pv, g, cs)
        at(begin[late], 0, dma_point, [], late_copies)
        for j in range(2 * NT * NT):
            t = end_q + wo_prep[0] * PIECE + j * (wo_prep[1] - wo_prep[0]) * PIECE // (2 * NT * NT)
            at(t, 1, (wo_widen, wo_perm)[j // NT % 2], j // (2 * NT), j % NT)
        at(begin[nq - 2], 0, patch)

        due = collections.defaultdict(list)
        for task in sorted(tasks, key=lambda task: task[:2]):
            due[piece_at(task[0])].append(task)

        results = []
        deps = collections.defaultdict(dict)

        def result_at(t):
            i = len(results) - 1
            while i >= 0 and start[i][-1] + LATENCY > t:
                i -= 1
            if i < 0:
                return None
            r = min((t - LATENCY - start[i][-1]) // 8, M // 8 - 1)
            return results[i][r * 8:(r + 1) * 8]

        def tie(t, token):
            if token is not None:
                i = piece_at(t)
                k = 0 if t - start[i][0] < M else NT - 1
                key = k, min(max(t - start[i][k], 0) // 16, M // 16 - 1)
                deps[i][key] = deps[i][key] | token if key in deps[i] else token

        for i, ((dot, _), mb, n) in enumerate(pieces):
            for t, _, limit, fn, args in due.pop(i, []):
                st["go"] = result_at(t) if limit else None
                token = fn(*args)
                if limit:
                    tie(t + limit, token)
            if i >= defer:
                (_, store), mb_s, n_s = pieces[i - defer]
                tie(begin[min(i - defer + fin_lag, len(pieces) - 1)], store(mb_s, n_s, results[i - defer]))
            if i in extra:
                extra[i][0](extra[i][1])
            results.append(dot(mb, n, deps.pop(i, {})))
        for i in range(len(pieces) - defer, len(pieces)):
            (_, store), mb_s, n_s = pieces[i]
            store(mb_s, n_s, results[i])
        assert not due
        pltpu.make_async_copy(out_v, out_hbm, sem_o).wait()

    scratch = [
        pltpu.VMEM((S, D), bf16),
        pltpu.VMEM((S // 2, D), i32),
        pltpu.VMEM((D, 3 * D), bf16),
        pltpu.VMEM((NT * D // 2 + 32, 128), i32),
        [pltpu.VMEM((D // 2, 128), i32)] * (3 * NT),
        pltpu.VMEM((D, D), bf16),
        [pltpu.VMEM((D, 128), f32)] * NT,
        [pltpu.VMEM((D // 2, 128), i32)] * NT,
        pltpu.VMEM((F, D), bf16),
        pltpu.VMEM((F, D), bf16),
        pltpu.VMEM((F, D), bf16),
        [pltpu.VMEM((M // 2, D), i32)] * NM,
        [pltpu.VMEM((NT * QS + 24, 128), f32)] * NM,
        [pltpu.VMEM((NT * KS + 16, 128), f32)] * NM,
        [pltpu.VMEM((NT * KS + 16, 128), f32)] * NM,
        [pltpu.VMEM((M // 2, D), i32)] * NM,
        [pltpu.VMEM((32, 128), f32)] * NSTAT,
        [pltpu.VMEM((32, 128), f32)] * NSTAT,
        [pltpu.VMEM((32, 128), f32)] * NSTAT,
        [pltpu.VMEM((32, 128), f32)] * NSTAT,
        [pltpu.VMEM((W * GA + 32, 128), f32)] * NP,
        pltpu.VMEM((S, D), bf16),
        [pltpu.VMEM((G, D), bf16)] * NSTAT,
        pltpu.VMEM((16, D), bf16),
        pltpu.VMEM((16, F), bf16),
        pltpu.VMEM((D,), bf16),
        pltpu.SemaphoreType.DMA((3,)),
        pltpu.SemaphoreType.DMA((8,)),
        pltpu.SemaphoreType.DMA(()),
    ]
    hbm = pl.BlockSpec(memory_space=pltpu.HBM)
    return pl.pallas_call(
        kernel,
        out_shape=jax.ShapeDtypeStruct((S, D), bf16),
        in_specs=[hbm] * 7,
        out_specs=hbm,
        scratch_shapes=scratch,
        compiler_params=pltpu.CompilerParams(vmem_limit_bytes=100 * 1024 * 1024, flags=flags, disable_semaphore_checks=nosem),
        name="fused", interpret=interpret,
    )


@jax.jit
def pallas_recurrent_scan__sliding_local_dilated__moe_arch_mod__prompt_kernel(
    A_x: jax.Array,
    A_wqkv: jax.Array,
    A_wo: jax.Array,
    B_x: jax.Array,
    B_w_r: jax.Array,
    B_w_gate: jax.Array,
    B_w_up: jax.Array,
    B_w_down: jax.Array,
):
    del B_x
    out = make_kernel()(A_x.reshape(S, D), A_wqkv, A_wo, B_w_r, B_w_gate.T, B_w_up.T, B_w_down)
    return out.reshape(1, S, D)
```

```python
import bisect
import collections
import functools
import itertools
import math

import jax
import jax.numpy as jnp
import numpy as np
from jax import lax
from jax.experimental import pallas as pl
from jax.experimental.pallas import tpu as pltpu

S, D, F = 2048, 640, 1728
H, DH, W, DIL = 32, 20, 8, 2
NT = D // 128
HALO = 16
M = 128
NM = S // M
G = 16
NG = M // G
NSTAT = 32
NP = 8
QS, KS = M + 8, M + HALO
PIECE = M * NT // 4
LATENCY = 130
LOG2E = math.log2(math.e)
QSCALE = DH ** -0.5 * LOG2E
NEG = -1e9 * LOG2E
EPS_BF16 = float(np.asarray(1e-5, dtype=jnp.bfloat16).astype(np.float32))
f32, bf16, i32 = jnp.float32, jnp.bfloat16, jnp.int32
NT_DIMS = (((1,), (1,)), ((), ()))


def _rb(x):
    return x.astype(bf16).astype(f32)


def _unpack(x):
    return pltpu.bitcast(x, bf16)


def _tree(op, xs):
    while len(xs) > 1:
        xs = [op(a, b) for a, b in zip(xs[::2], xs[1::2])] + xs[len(xs) // 2 * 2:]
    return xs[0]


NF = 2


def make_kernel(att_off=600, att_last=65, fin_lag=4, wo_prep=(-60, -4), split_last=True, qk_lag=2, win=400, pv_off=244, pv_gap=20, sm_off=0,
                ln_off=(42, 56, 20, 56, 32, 94, 95), ln_done=4, scale_lag=3, scale_limit=260, top_gap=400, att_start=100, att_rate=(1.0, 1e-6, 1.0, 1.0, 0.85),
                ln_stop=300, defer=2, GA=16, pv_split=((0,), (1,), (2,), (3,), (4,)), w_wait=(8, 44), ln_start=(21, 48), ln_mid=40, NX=6,
                late=144, quiet=200, quiet_off=380, ffn_gap=2, sel_off=(64, 260, 60), sel_gap=(12, 16, 24),
                gather_gap=(150, 150, 500),
                qk_split=((0,), (1,), (2,), (3,)), qk_off=86, st_off=200, qk_gap=19, exp_off=224, flags=None, interpret=False, nosem=False, NV=5, x_wait=16):
    NA = M // GA
    xb = (0, NF * M, NX * M, S)

    def kernel(x_hbm, wqkv_hbm, wo_hbm, wr_hbm, wg_hbm, wu_hbm, wd_hbm, out_hbm,
               x_v, z_v, wqkv_raw, wqkv_t, wqkv_p, wo_raw, wo_f, wo_p, wg_v, wu_v, wd_v,
               xn_v, q_s, k_s, v_s, o_v, m_s, d_s, i_s, f_s, p_s, out_v, d_v, xs_v, hid_v, wr_ref, sem_x, sem_w, sem_o):
        x_copies = [pltpu.make_async_copy(x_hbm.at[pl.ds(a, b - a), :], x_v[j].bitcast(bf16), sem_x.at[j])
                    for j, (a, b) in enumerate(zip(xb, xb[1:]))]
        qkv_copies = [pltpu.make_async_copy(wqkv_hbm.at[:, pl.ds(p * D, D)], wqkv_raw[p].bitcast(bf16),
                                            sem_w.at[p]) for p in range(3)]
        late_copies = [pltpu.make_async_copy(s, d.bitcast(bf16), sem_w.at[3 + j]) for j, (s, d) in enumerate(
            [(wo_hbm, wo_raw), (wg_hbm, wg_v), (wu_hbm, wu_v), (wd_hbm, wd_v)])]

        wr_copy = pltpu.make_async_copy(wr_hbm, wr_ref, sem_w.at[7])

        done = set()

        def dma_point(start, wait):
            for c in start:
                c.start()
            for c in wait:
                c.wait()
                done.add(id(c))

        dma_point([wr_copy, x_copies[0], qkv_copies[0]], x_copies[:1])

        lane = lax.broadcasted_iota(i32, (8, 128), 1)
        sub = lax.broadcasted_iota(i32, (8, 128), 0)
        bits = x_v[0][pl.ds(0, 8), pl.ds(0, 128)] >> 16
        zero = (bits * (bits + 1)) & 1
        zero0 = zero[0, 0]
        fresh = itertools.count(1)
        folds = itertools.count()
        st = dict(folded=[], sums=[], r=[jnp.zeros((8, 128), f32), jnp.zeros((8, 128), f32)])

        def need(*keys):
            assert done.issuperset(keys), keys

        def opaque(align):
            return pl.multiple_of(zero0 * (next(fresh) * align), align)

        def after(ref, row=0):
            return pltpu.bitcast(ref[pl.ds(opaque(8) + row, 8), pl.ds(0, 128)], i32)

        def hold(ref, idx):
            if st["go"] is not None:
                ref[idx] = pltpu.bitcast(st["go"], i32) if ref.dtype == i32 else st["go"].astype(ref.dtype)

        def x_rows(row, n, cols=slice(None)):
            j = bisect.bisect_right(xb, row) - 1
            need(id(x_copies[j]))
            return _unpack(x_v[j][pl.ds((row - xb[j]) // 2 + opaque(8), n // 2), cols]).astype(f32)

        def wide(v):
            return jnp.concatenate([v] * NT, axis=1)

        def get(ref, g):
            need((id(ref), g))
            return ref[g % NSTAT][pl.ds(opaque(8), G), :]

        def put(ref, g, v):
            done.add((id(ref), g))
            ref[g % NSTAT][pl.ds(0, G), :] = jnp.broadcast_to(v, (G, 128))
            return after(ref[g % NSTAT])

        def fold(g, then, v):
            slot_ref = f_s[next(folds) % NSTAT]
            slot_ref[pl.ds(0, G), :] = _tree(jnp.add, [v[:, c * 128:(c + 1) * 128] for c in range(NT)])
            st["folded"].append((then, g, slot_ref))
            return after(slot_ref)

        def ln_reduce():
            sums = []
            for then, g, slot_ref in st["folded"]:
                hold(slot_ref, (pl.ds(G, 8), slice(None)))
                sums.append((then, g, jnp.sum(slot_ref[pl.ds(opaque(8), G), :], axis=1, keepdims=True)))
            st["folded"] = []
            st["sums"].append(sums)

        def ln_finish():
            tokens = [then(g, v) for then, g, v in st["sums"].pop(0)]
            return functools.reduce(jnp.bitwise_or, tokens) if tokens else None

        def ln_mean(g):
            return fold(g, lambda g, v: put(m_s, g, v * (1.0 / D)), x_rows(g * G, G))

        def ln_var(g):
            d = x_rows(g * G, G) - wide(_rb(get(m_s, g)))
            d_v[g % NSTAT].bitcast(bf16)[pl.ds(0, G), :] = d.astype(bf16)
            return fold(g, lambda g, v: put(d_s, g, v * (1.0 / D)), d * d)

        def ln_scale(g):
            hold(d_s[g % NSTAT], (pl.ds(G, 8), slice(None)))
            m = get(m_s, g)
            shift = m - _rb(m)
            var = jnp.maximum(get(d_s, g) - shift * shift, 0.0)
            den = jnp.minimum(_rb(jnp.sqrt(_rb(_rb(var) + EPS_BF16))), 3e38)
            inv = pltpu.reciprocal(den, approx=True)
            return put(i_s, g, inv * (2.0 - den * inv))

        def ln_norm(g):
            done.add(("xn", g))
            xn = (_unpack(d_v[g % NSTAT][pl.ds(opaque(8), G // 2), :]).astype(f32) * wide(get(i_s, g))).astype(bf16)
            z_v.bitcast(bf16)[pl.ds(g * G, G), :] = xn
            xn_v[g // NG].bitcast(bf16)[pl.ds(g % NG * G, G), :] = xn
            return after(xn_v[g // NG])

        def keep_score(g, r):
            done.add(("r", g))
            for s in range(G // 8):
                half, l = divmod(g * G // 8 + s, 128)
                rs = jnp.broadcast_to(r[s * 8:(s + 1) * 8], (8, 128))
                st["r"][half] = jnp.where(lane == l, rs, st["r"][half])
            return pltpu.bitcast(st["r"][half], i32)

        def ln_dot(g):
            need(("xn", g))
            if g == 0:
                dma_point(qkv_copies[1:2], [wr_copy])
                st["wr"] = wr_ref[...].astype(f32).reshape(1, D)
            xn = _unpack(z_v[pl.ds(g * G // 2 + opaque(8), G // 2), :])
            return fold(g, keep_score, xn.astype(f32) * st["wr"])

        def mod5(n):
            return n - ((n * 205) >> 10) * 5

        src_lane = [(20 * (lane & 31) + 5 * (lane >> 5) + c) & 127 for c in range(NT)]
        turn = mod5((130 - lane) * 2)
        turns = [(step, turn & step != 0) for step in (1, 2, 4)]

        def select(p, b, cs, z):
            need(id(qkv_copies[p]))
            tiles = [wqkv_raw[p][pl.ds(z + b * 8, 8), pl.ds(t * 128, 128)] for t in range(NT)]
            for step, mask in turns:
                tiles = [jnp.where(mask, tiles[(t + step) % NT], tiles[t]) for t in range(NT)]
            return [(c, tiles[2 * c % NT]) for c in cs]

        def gather_lanes(p, c, b, v):
            done.add(("w", p * NT + c))
            wqkv_p[p * NT + c][pl.ds(b * 8, 8), :] = jnp.take_along_axis(
                v, src_lane[c], axis=1, mode="promise_in_bounds")

        def prep_first(p):
            z = opaque(8)
            for b in range(D // 16):
                (_, first), (_, second) = select(p, b, [0, 1], z)
                gather_lanes(p, 0, b, first)
                wqkv_t[pl.ds(D // 2 + b * 8, 8), :] = second

        def prep_select(p, j, first, n):
            z = opaque(8)
            for b in range(j * n, (j + 1) * n):
                for c, sel in select(p, b, range(first, NT), z):
                    wqkv_t[pl.ds(c * D // 2 + b * 8, 8), :] = sel
            return after(wqkv_t, (NT - 1) * D // 2)

        def prep_gather(p, c):
            hold(wqkv_t, (pl.ds(NT * D // 2, 8), slice(None)))
            z = opaque(8)
            for b in range(D // 16):
                gather_lanes(p, c, b, wqkv_t[pl.ds(z + (c * D // 2 + b * 8), 8), :])

        def wo_widen(t, j):
            need(id(late_copies[0]))
            wo_f[t][pl.ds(j * 128, 128), :] = _unpack(wo_raw[pl.ds(j * 64, 64), pl.ds(t * 128, 128)]).astype(f32)
            return after(wo_f[t])

        def wo_perm(t, c):
            done.add(("wo", t, c))
            z = opaque(8)
            for g in range(4):
                blk = wo_f[t][pl.ds(z + (5 * g + c), 32, stride=20), :]
                wo_p[t][pl.ds(c * 64 + g * 16, 16), :] = pltpu.bitcast(blk.astype(bf16), i32)
            return after(wo_p[t])

        def window_pair(ref, z, c, row, w):
            t = ref[pl.ds(z + (row + c * KS + HALO - 8 - DIL * w), GA + 8), :]
            return t[8:], t[:GA]

        def attn_qk(g, ws):
            mb, j = divmod(g, NA)
            z = opaque(8)
            need(*[("qkv", b, n) for b in {mb, max(mb - 1, 0)} for n in range(3 * NT)])
            hold((q_s if ws[0] == 0 else k_s)[mb], (pl.ds(M if ws[0] == 0 else NT * KS, 8), slice(None)))
            if ws[0] == 0:
                st["q"] = [q_s[mb][pl.ds(z + (c * QS + j * GA), GA), :] for c in range(NT)]
            for w in ws:
                ps = None
                for c in range(NT):
                    t = [st["q"][c] * k for k in window_pair(k_s[mb], z, c, j * GA, w)]
                    ps = t if ps is None else [a + b for a, b in zip(ps, t)]
                st["p", g, w] = [(p, pltpu.roll(p, 64, 1)) for p in ps]

        def attn_qk_store(g, ws):
            done.update(("p", g, w) for w in ws)
            for w in ws:
                for ww, (p, r) in zip((w, w + W // 2), st.pop(("p", g, w))):
                    p_s[g % NP][pl.ds(ww * GA, GA), :] = p + r
            return after(p_s[g % NP])

        def attn_logits(g):
            need(*[("p", g, w) for w in range(W // 2)])
            z = opaque(8)
            hold(p_s[g % NP], (pl.ds(W * GA, 8), slice(None)))
            ps = [p_s[g % NP][pl.ds(z + w * GA, GA), :] for w in range(W)]
            st["l", g] = [p + pltpu.roll(p, 32, 1) for p in ps]

        def attn_softmax(g):
            ps = st.pop(("l", g))
            for w in range(W):
                if g * GA < DIL * w:
                    pos = g * GA + lax.broadcasted_iota(i32, (GA, 128), 0)
                    ps[w] = jnp.where(pos >= DIL * w, ps[w], NEG)
            m = _tree(jnp.maximum, ps)
            e = [jnp.exp2(l - m) for l in ps]
            inv = pltpu.reciprocal(_tree(jnp.add, e), approx=True)
            st["e", g] = e, inv
            return pltpu.bitcast(inv[:8], i32) | pltpu.bitcast(inv[GA - 8:], i32)

        def attn_pv(g, cs):
            mb, j = divmod(g, NA)
            z = opaque(8)
            e, inv = st["e", g]
            done.update(("o", g, c) for c in cs)
            token = None
            for c in cs:
                acc = None
                for w in range(W // 2):
                    near, far = window_pair(v_s[mb], z, c, j * GA, w)
                    t = e[w] * near + e[w + W // 2] * far
                    acc = t if acc is None else acc + t
                acc = acc * inv
                for r in range(GA // 8):
                    t = pltpu.bitcast(acc[r * 8:(r + 1) * 8], i32)
                    token = t if token is None else token | t
                if GA == 8:
                    if g % 2 == 0:
                        st["o", c] = acc
                        continue
                    acc = jnp.concatenate([st.pop(("o", c)), acc], axis=0)
                o_v[mb].bitcast(bf16)[pl.ds(j * GA // 16 * 16, 16), pl.ds(c * 128, 128)] = acc.astype(bf16)
            return token

        row = lax.broadcasted_iota(i32, (16, D), 0)

        def tile_of(t):
            return pl.ds(pl.multiple_of((t // 16) * 8, 8), 8)

        def tok(v):
            return pltpu.bitcast(jnp.broadcast_to(v, (8, 128)), i32)

        def top(k):
            if k == 0:
                need(*[("r", g) for g in range(S // G)])
                st["r_all"] = r_all = _rb(jnp.concatenate(st["r"], axis=0))
                st["idx"] = jnp.concatenate([lane * 8 + sub, (lane + 128) * 8 + sub], axis=0).astype(f32)
                st["key"] = jnp.where(r_all == r_all, r_all, -jnp.inf)
                st["free"] = jnp.full((16, 128), True)
                st["i"] = []
            if k % 2 == 0:
                st["max"] = jnp.max(st["key"], keepdims=True)
                return tok(st["max"])
            i = jnp.min(jnp.where((st["key"] == st["max"]) & st["free"], st["idx"], S - 1.0), keepdims=True)
            st["i"].append(i)
            st["free"] = st["idx"] != i
            st["key"] = jnp.where(st["free"], st["key"], -jnp.inf)
            return tok(i)

        def gather():
            done.add("xs")
            st["rs"] = [jnp.sum(jnp.where(st["idx"] == i, st["r_all"], 0.0), keepdims=True) for i in st["i"]]
            st["t"] = [i.astype(i32)[0, 0] for i in st["i"]]

            def pick(t):
                z = _unpack(z_v[tile_of(t), :]).astype(f32)
                return jnp.sum(jnp.where(row == t % 16, z, 0.0), axis=0, keepdims=True)

            xs = jnp.where(row == 0, pick(st["t"][0]), pick(st["t"][1]))
            xs_v[pl.ds(0, 8), :] = pltpu.bitcast(xs.astype(bf16), i32)
            return pltpu.bitcast(xs[:8, :128], i32) | tok(st["rs"][0]) | tok(st["rs"][1])

        def ffn_rows(j):
            return pl.ds(j * 128, min(128, F - j * 128))

        def ffn_weights(ref, j):
            need("xs", *map(id, late_copies))
            return _unpack(ref[pl.ds(j * 64, min(64, F // 2 - j * 64)), :])

        def ffn_gate(j):
            st["gate"] = lax.dot_general(_unpack(xs_v[pl.ds(0, 8), :]), ffn_weights(wg_v, j), NT_DIMS, preferred_element_type=f32)

        def ffn_up(j):
            gate = _rb(st.pop("gate"))
            up = _rb(lax.dot_general(_unpack(xs_v[pl.ds(0, 8), :]), ffn_weights(wu_v, j), NT_DIMS, preferred_element_type=f32))
            hid_v[pl.ds(0, 16), ffn_rows(j)] = (_rb(gate * jax.nn.sigmoid(gate)) * up).astype(bf16)

        def ffn_down(j):
            done.add(("y", j))
            y = jnp.dot(hid_v[pl.ds(0, 16), ffn_rows(j)], ffn_weights(wd_v, j), preferred_element_type=f32)[:8]
            st["y"] = y if j == 0 else st["y"] + y

        def patch():
            need(("y", pl.cdiv(F, 128) - 1))
            done.add("patch")
            for j in range(2):
                t = st["t"][j]
                upd = _rb(_rb(st["y"][j:j + 1]) * _rb(jax.nn.sigmoid(st["rs"][j])))
                z = _unpack(z_v[tile_of(t), :]).astype(f32)
                z_v[tile_of(t), :] = pltpu.bitcast(jnp.where(row == t % 16, z + upd, z).astype(bf16), i32)

        def o_copy(mb, cols):
            rows = pl.ds(mb * M, M)
            return pltpu.make_async_copy(out_v.at[rows, cols], out_hbm.at[rows, cols], sem_o)

        def piece_dot(lhs_ref, rhs_ref, deps):
            z = opaque(8)
            cols = []
            for k in range(NT):
                col = lhs_ref[pl.ds(z, M // 2), pl.ds(k * 128, 128)]
                if any(kk == k for kk, _ in deps):
                    parts = [col[r * 8:(r + 1) * 8] for r in range(M // 16)]
                    for (kk, r), t in deps.items():
                        if kk == k:
                            parts[r] = parts[r] | (t & zero)
                    col = jnp.concatenate(parts, axis=0)
                cols.append(col)
            lhs = _unpack(jnp.concatenate(cols, axis=1))
            return jnp.dot(lhs, _unpack(rhs_ref[pl.ds(z, D // 2), :]), preferred_element_type=f32)

        def qkv_dot(mb, n, deps):
            need(("w", n), *[("xn", mb * NG + j) for j in range(NG)])
            return piece_dot(xn_v[mb], wqkv_p[n], deps)

        def qkv_store(mb, n, res):
            done.add(("qkv", mb, n))
            p, c = divmod(n, NT)
            if p == 0:
                q_s[mb][pl.ds(c * QS, M), :] = res * QSCALE
            else:
                dst = (k_s, v_s)[p - 1]
                dst[mb][pl.ds(c * KS + HALO, M), :] = res
                if mb == 0:
                    dst[0][pl.ds(c * KS, HALO), :] = jnp.broadcast_to(res[0:1], (HALO, 128))
                if mb + 1 < NM:
                    dst[mb + 1][pl.ds(c * KS, HALO), :] = res[M - HALO:]

        def out_dot(mb, c, deps):
            need(*[("wo", c, k) for k in range(NT)], *[("o", mb * NA + j, k) for j in range(NA) for k in range(NT)])
            return piece_dot(o_v[mb], wo_p[c], deps)

        def out_store(mb, c, s):
            need("patch")
            cols = pl.ds(c * 128, 128)
            z = _unpack(z_v[pl.ds(mb * M // 2 + opaque(8), M // 2), cols]).astype(f32)
            gate = z * pltpu.reciprocal(1.0 + jnp.exp2(z * -LOG2E), approx=True)
            res = x_rows(mb * M, M, cols) + s * gate
            out_v[pl.ds(mb * M, M), cols] = res.astype(bf16)
            if mb == NM - 1 and split_last:
                o_copy(mb, cols).start()
            elif c == NT - 1:
                o_copy(mb, slice(None)).start()
            return pltpu.bitcast(res[M - 8:], i32)

        qkv, out = (qkv_dot, qkv_store), (out_dot, out_store)
        pieces = [(qkv, mb, n) for n in range(2 * NT) for mb in range(NF)]
        pieces += [(qkv, mb, n) for mb in range(NF, NV) for n in range(2 * NT)]
        pieces += [(qkv, mb, n) for n in range(2 * NT, 3 * NT) for mb in range(NV)]
        pieces += [(qkv, mb, n) for mb in range(NV, NM) for n in range(3 * NT)]
        nq = len(pieces)
        pieces += [(out, mb, c) for mb in range(NM) for c in range(NT)]
        nf = pl.cdiv(F, 128)
        extra = {}
        for j in range(nf):
            extra[late + 1 + int(2 * j * ffn_gap)] = ffn_gate, j
            extra[late + 1 + int((2 * j + 1) * ffn_gap)] = ffn_up, j
            extra[late + 4 + int((2 * nf + j) * ffn_gap)] = ffn_down, j
        busy, start = [0] * 4, []
        for i in range(len(pieces)):
            for rows in ([16] * NT if i in extra else []) + [M] * NT:
                m = busy.index(min(busy))
                if rows == M:
                    start.append(busy[m])
                busy[m] += rows
        start = np.reshape(start, (-1, NT)).tolist()
        begin = [0]
        for i in range(1, len(pieces)):
            begin.append(max(start[i][0], min(begin[-1] + PIECE, start[i - 1][-1] + M - 1)))
        end_q = begin[nq]
        tasks = []

        def at(t, limit, fn, *args):
            tasks.append((t, len(tasks), limit, fn, args))

        def piece_at(t):
            return bisect.bisect_right(begin, t) - 1

        stages = (ln_mean, ln_var, ln_scale, ln_norm, ln_dot)

        def ln_steps(lo, hi, a, b, done):
            lags = (0, done + 1, 2 * done + 2, 2 * done + 3 + scale_lag, 2 * done + 4 + scale_lag)
            n = hi - lo + lags[-1] + done
            for t in range(n):
                def time(off):
                    return a + (t * 100 + off) * (b - a) // (100 * n)

                for k, fn, off in zip(lags, stages, ln_off):
                    if 0 <= t - k < hi - lo:
                        at(time(off), (scale_limit if fn is ln_scale else 1) if b else 0, fn, lo + t - k)
                if t < n - done:
                    at(time(ln_off[5]), 1 if b else 0, ln_reduce)
                if t >= done:
                    at(time(ln_off[6]), 1 if b else 0, ln_finish)

        ln_steps(0, NF * NG, 0, 0, 3)
        starts = (x_copies[1:2], qkv_copies[2:], late_copies)
        waits = (qkv_copies[:1], qkv_copies[1:2], (qkv_copies[2], x_copies[2]))
        for p, first in enumerate((0,) + w_wait):
            t = first * PIECE
            at(t, 0, dma_point, starts[p], waits[p])
            quick = 2 * (p < 2)
            if quick:
                at(t, 0, prep_first, p)
                at(t, 0, prep_gather, p, 1)
            for j in range(20):
                at(t + sel_off[p] + j * sel_gap[p], 1, prep_select, p, j, quick, 2)
            for c in range(quick, NT):
                at(t + sel_off[p] + 20 * sel_gap[p] + (c - quick) * gather_gap[p], 1, prep_gather, p, c)
        at(x_wait * PIECE, 0, dma_point, x_copies[2:], x_copies[1:2])
        ln_steps(NF * NG, (NF + 1) * NG, x_wait * PIECE, ln_start[0] * PIECE, ln_done)
        ln_steps((NF + 1) * NG, NX * NG, ln_start[0] * PIECE, ln_mid * PIECE, ln_done)
        base = att_start * PIECE
        ln_steps(NX * NG, NM * NG, ln_start[1] * PIECE, base - ln_stop, ln_done)
        for k in range(4):
            at(base + k * top_gap, win, top, k)
        at(base + 4 * top_gap, win, gather)

        knots = [base, begin[late] - quiet - quiet_off, begin[late] - quiet_off, begin[max(extra)],
                 end_q + att_off, end_q + att_off + att_last * PIECE]
        work = np.cumsum([0] + [(b - a) * rate for a, b, rate in zip(knots, knots[1:], att_rate)])

        def slot(g):
            return int(np.interp((g + qk_lag) * work[-1] / (NM * NA + qk_lag), work, knots))

        for g in range(NM * NA):
            for n, ws in enumerate(qk_split):
                at(slot(g - qk_lag) + qk_off + n * qk_gap, win, attn_qk, g, ws)
                at(slot(g - qk_lag) + qk_off + n * qk_gap + st_off, 1, attn_qk_store, g, ws)
            at(slot(g) + sm_off, win, attn_logits, g)
            at(slot(g) + sm_off + exp_off, 1, attn_softmax, g)
            for n, cs in enumerate(pv_split):
                at(slot(g) + pv_off + n * pv_gap, 1, attn_pv, g, cs)
        at(begin[late], 0, dma_point, [], late_copies)
        for j in range(2 * NT * NT):
            t = end_q + wo_prep[0] * PIECE + j * (wo_prep[1] - wo_prep[0]) * PIECE // (2 * NT * NT)
            at(t, 1, (wo_widen, wo_perm)[j // NT % 2], j // (2 * NT), j % NT)
        at(begin[nq - 2], 0, patch)

        due = collections.defaultdict(list)
        for task in sorted(tasks, key=lambda task: task[:2]):
            due[piece_at(task[0])].append(task)

        results = []
        deps = collections.defaultdict(dict)

        def result_at(t):
            i = len(results) - 1
            while i >= 0 and start[i][-1] + LATENCY > t:
                i -= 1
            if i < 0:
                return None
            r = min((t - LATENCY - start[i][-1]) // 8, M // 8 - 1)
            return results[i][r * 8:(r + 1) * 8]

        def tie(t, token):
            if token is not None:
                i = piece_at(t)
                k = 0 if t - start[i][0] < M else NT - 1
                key = k, min(max(t - start[i][k], 0) // 16, M // 16 - 1)
                deps[i][key] = deps[i][key] | token if key in deps[i] else token

        for i, ((dot, _), mb, n) in enumerate(pieces):
            for t, _, limit, fn, args in due.pop(i, []):
                st["go"] = result_at(t) if limit else None
                token = fn(*args)
                if limit:
                    tie(t + limit, token)
            if i >= defer:
                (_, store), mb_s, n_s = pieces[i - defer]
                tie(begin[min(i - defer + fin_lag, len(pieces) - 1)], store(mb_s, n_s, results[i - defer]))
            if i in extra:
                extra[i][0](extra[i][1])
            results.append(dot(mb, n, deps.pop(i, {})))
        for i in range(len(pieces) - defer, len(pieces)):
            (_, store), mb_s, n_s = pieces[i]
            store(mb_s, n_s, results[i])
        assert not due
        pltpu.make_async_copy(out_v, out_hbm, sem_o).wait()

    scratch = [
        [pltpu.VMEM(((b - a) // 2, D), i32) for a, b in zip(xb, xb[1:])],
        pltpu.VMEM((S // 2, D), i32),
        [pltpu.VMEM((D // 2, D), i32)] * 3,
        pltpu.VMEM((NT * D // 2 + 32, 128), i32),
        [pltpu.VMEM((D // 2, 128), i32)] * (3 * NT),
        pltpu.VMEM((D // 2, D), i32),
        [pltpu.VMEM((D, 128), f32)] * NT,
        [pltpu.VMEM((D // 2, 128), i32)] * NT,
        pltpu.VMEM((F // 2, D), i32),
        pltpu.VMEM((F // 2, D), i32),
        pltpu.VMEM((F // 2, D), i32),
        [pltpu.VMEM((M // 2, D), i32)] * NM,
        [pltpu.VMEM((NT * QS + 24, 128), f32)] * NM,
        [pltpu.VMEM((NT * KS + 16, 128), f32)] * NM,
        [pltpu.VMEM((NT * KS + 16, 128), f32)] * NM,
        [pltpu.VMEM((M // 2, D), i32)] * NM,
        [pltpu.VMEM((32, 128), f32)] * NSTAT,
        [pltpu.VMEM((32, 128), f32)] * NSTAT,
        [pltpu.VMEM((32, 128), f32)] * NSTAT,
        [pltpu.VMEM((32, 128), f32)] * NSTAT,
        [pltpu.VMEM((W * GA + 32, 128), f32)] * NP,
        pltpu.VMEM((S, D), bf16),
        [pltpu.VMEM((32, D), i32)] * NSTAT,
        pltpu.VMEM((32, D), i32),
        pltpu.VMEM((64, F), bf16),
        pltpu.VMEM((D,), bf16),
        pltpu.SemaphoreType.DMA((3,)),
        pltpu.SemaphoreType.DMA((8,)),
        pltpu.SemaphoreType.DMA(()),
    ]
    hbm = pl.BlockSpec(memory_space=pltpu.HBM)
    return pl.pallas_call(
        kernel,
        out_shape=jax.ShapeDtypeStruct((S, D), bf16),
        in_specs=[hbm] * 7,
        out_specs=hbm,
        scratch_shapes=scratch,
        compiler_params=pltpu.CompilerParams(vmem_limit_bytes=100 * 1024 * 1024, flags=flags, disable_semaphore_checks=nosem),
        name="fused", interpret=interpret,
    )


@jax.jit
def pallas_recurrent_scan__sliding_local_dilated__moe_arch_mod__prompt_kernel(
    A_x: jax.Array,
    A_wqkv: jax.Array,
    A_wo: jax.Array,
    B_x: jax.Array,
    B_w_r: jax.Array,
    B_w_gate: jax.Array,
    B_w_up: jax.Array,
    B_w_down: jax.Array,
):
    del B_x
    out = make_kernel()(A_x.reshape(S, D), A_wqkv, A_wo, B_w_r, B_w_gate.T, B_w_up.T, B_w_down)
    return out.reshape(1, S, D)
```

```python
import bisect
import collections
import functools
import itertools
import math

import jax
import jax.numpy as jnp
import numpy as np
from jax import lax
from jax.experimental import pallas as pl
from jax.experimental.pallas import tpu as pltpu

S, D, F = 2048, 640, 1728
DH, W, DIL = 20, 8, 2
NT = D // 128
HALO = 16
M = 128
NM = S // M
G = 16
NG = M // G
NSTAT, NP = 32, 8
QS, KS = M + 8, M + HALO
LOG2E = math.log2(math.e)
QSCALE = DH ** -0.5 * LOG2E
MASKED = -1e9 * LOG2E
EPS = float(np.asarray(1e-5, dtype=jnp.bfloat16).astype(np.float32))
f32, bf16, i32 = jnp.float32, jnp.bfloat16, jnp.int32
TRANSPOSED_RHS = (((1,), (1,)), ((), ()))

PIECE = M * NT // 4
LATENCY = 130
NF, NV, NX = 2, 5, 6
X_BOUNDS = (0, NF * M, NX * M, S)
WAIT_W, WAIT_X, WAIT_LATE = (0, 8, 44), 16, 144
SELECT_AT, SELECT_GAP, GATHER_GAP = (64, 260, 60), (12, 16, 24), (150, 150, 500)
LN_SPANS = ((NF, NF + 1, WAIT_X, 21), (NF + 1, NX, 21, 40))
LN_START, LN_PHASE, LN_SUM_STEPS = 48, (42, 56, 20, 56, 32, 94, 95), 4
ATT_START, ATT_RATE = 100, (1.0, 1e-6, 1.0, 1.0, 0.85)
QK_LAG, QK_AT, QK_GAP, QK_STORE, EXP_AT, PV_AT, PV_GAP = 2, 86, 19, 200, 224, 244, 20
LOOSE, EXACT = 400, 1
STORE_LAG, OUT_LAG = 2, 4


def _rb(x):
    return x.astype(bf16).astype(f32)


def _pack(x):
    return pltpu.bitcast(x.astype(bf16), i32)


def _unpack(x):
    return pltpu.bitcast(x, bf16)


def _tree(op, xs):
    while len(xs) > 1:
        xs = [op(a, b) for a, b in zip(xs[::2], xs[1::2])] + xs[len(xs) // 2 * 2:]
    return xs[0]


def _kernel(x_hbm, wqkv_hbm, wo_hbm, wr_hbm, wg_hbm, wu_hbm, wd_hbm, out_hbm,
            x_v, z_v, wqkv_raw, wqkv_t, wqkv_p, wo_raw, wo_f, wo_p, wg_v, wu_v, wd_v, xn_v, q_s, k_s, v_s, o_v,
            m_s, d_s, i_s, f_s, p_s, out_v, d_v, xs_v, hid_v, wr_v, sem_x, sem_w, sem_o):
    x_copies = [pltpu.make_async_copy(x_hbm.at[pl.ds(a, b - a), :], x_v[j].bitcast(bf16), sem_x.at[j])
                for j, (a, b) in enumerate(zip(X_BOUNDS, X_BOUNDS[1:]))]
    qkv_copies = [pltpu.make_async_copy(wqkv_hbm.at[:, pl.ds(p * D, D)], wqkv_raw[p].bitcast(bf16), sem_w.at[p])
                  for p in range(3)]
    late_copies = [pltpu.make_async_copy(src, dst.bitcast(bf16), sem_w.at[3 + j]) for j, (src, dst) in enumerate(
        [(wo_hbm, wo_raw), (wg_hbm, wg_v), (wu_hbm, wu_v), (wd_hbm, wd_v)])]
    wr_copy = pltpu.make_async_copy(wr_hbm, wr_v, sem_w.at[7])

    written = set()

    def need(*keys):
        assert written.issuperset(keys), keys

    def dma_point(start, wait):
        for c in start:
            c.start()
        for c in wait:
            c.wait()
            written.add(id(c))

    dma_point([wr_copy, x_copies[0], qkv_copies[0]], x_copies[:1])

    lane = lax.broadcasted_iota(i32, (8, 128), 1)
    sub = lax.broadcasted_iota(i32, (8, 128), 0)
    bits = x_v[0][pl.ds(0, 8), pl.ds(0, 128)] >> 16
    zero = (bits * (bits + 1)) & 1
    zero0 = zero[0, 0]
    fresh, folds = itertools.count(1), itertools.count()
    st = dict(folded=[], sums=[], r=[jnp.zeros((8, 128), f32), jnp.zeros((8, 128), f32)])

    def opaque():
        return pl.multiple_of(zero0 * (next(fresh) * 8), 8)

    def after(ref, row=0):
        return pltpu.bitcast(ref[pl.ds(opaque() + row, 8), pl.ds(0, 128)], i32)

    def hold(ref, row):
        if st["go"] is not None:
            ref[pl.ds(row, 8), :] = pltpu.bitcast(st["go"], ref.dtype)

    def x_rows(row, n, cols=slice(None)):
        j = bisect.bisect_right(X_BOUNDS, row) - 1
        need(id(x_copies[j]))
        return _unpack(x_v[j][pl.ds((row - X_BOUNDS[j]) // 2 + opaque(), n // 2), cols]).astype(f32)

    def wide(v):
        return jnp.concatenate([v] * NT, axis=1)

    def get(refs, g):
        need((id(refs), g))
        return refs[g % NSTAT][pl.ds(opaque(), G), :]

    def put(refs, g, v):
        written.add((id(refs), g))
        refs[g % NSTAT][pl.ds(0, G), :] = jnp.broadcast_to(v, (G, 128))
        return after(refs[g % NSTAT])

    def fold(g, then, v):
        ref = f_s[next(folds) % NSTAT]
        ref[pl.ds(0, G), :] = _tree(jnp.add, [v[:, c * 128:(c + 1) * 128] for c in range(NT)])
        st["folded"].append((then, g, ref))
        return after(ref)

    def ln_reduce():
        sums = []
        for then, g, ref in st["folded"]:
            hold(ref, G)
            sums.append((then, g, jnp.sum(ref[pl.ds(opaque(), G), :], axis=1, keepdims=True)))
        st["folded"] = []
        st["sums"].append(sums)

    def ln_finish():
        tokens = [then(g, v) for then, g, v in st["sums"].pop(0)]
        return functools.reduce(jnp.bitwise_or, tokens) if tokens else None

    def ln_mean(g):
        return fold(g, lambda g, v: put(m_s, g, v * (1.0 / D)), x_rows(g * G, G))

    def ln_var(g):
        d = x_rows(g * G, G) - wide(_rb(get(m_s, g)))
        d_v[g % NSTAT].bitcast(bf16)[pl.ds(0, G), :] = d.astype(bf16)
        return fold(g, lambda g, v: put(d_s, g, v * (1.0 / D)), d * d)

    def ln_scale(g):
        hold(d_s[g % NSTAT], G)
        m = get(m_s, g)
        shift = m - _rb(m)
        var = jnp.maximum(get(d_s, g) - shift * shift, 0.0)
        den = jnp.minimum(_rb(jnp.sqrt(_rb(_rb(var) + EPS))), 3e38)
        inv = pltpu.reciprocal(den, approx=True)
        return put(i_s, g, inv * (2.0 - den * inv))

    def ln_norm(g):
        written.add(("xn", g))
        d = _unpack(d_v[g % NSTAT][pl.ds(opaque(), G // 2), :]).astype(f32)
        xn = (d * wide(get(i_s, g))).astype(bf16)
        z_v.bitcast(bf16)[pl.ds(g * G, G), :] = xn
        xn_v[g // NG].bitcast(bf16)[pl.ds(g % NG * G, G), :] = xn
        return after(xn_v[g // NG])

    def keep_score(g, r):
        written.add(("r", g))
        for s in range(G // 8):
            half, l = divmod(g * G // 8 + s, 128)
            st["r"][half] = jnp.where(lane == l, jnp.broadcast_to(r[s * 8:(s + 1) * 8], (8, 128)), st["r"][half])
        return pltpu.bitcast(st["r"][half], i32)

    def ln_dot(g):
        need(("xn", g))
        if g == 0:
            dma_point(qkv_copies[1:2], [wr_copy])
            st["wr"] = wr_v[...].astype(f32).reshape(1, D)
        xn = _unpack(z_v[pl.ds(g * G // 2 + opaque(), G // 2), :])
        return fold(g, keep_score, xn.astype(f32) * st["wr"])

    src_lane = [(20 * (lane & 31) + 5 * (lane >> 5) + c) & 127 for c in range(NT)]
    turn = (130 - lane) * 2
    turn = turn - ((turn * 205) >> 10) * 5
    turns = [(step, turn & step != 0) for step in (1, 2, 4)]

    def select(p, b, z):
        need(id(qkv_copies[p]))
        tiles = [wqkv_raw[p][pl.ds(z + b * 8, 8), pl.ds(t * 128, 128)] for t in range(NT)]
        for step, mask in turns:
            tiles = [jnp.where(mask, tiles[(t + step) % NT], tiles[t]) for t in range(NT)]
        return [tiles[2 * c % NT] for c in range(NT)]

    def gather_lanes(p, c, b, v):
        written.add(("w", p * NT + c))
        wqkv_p[p * NT + c][pl.ds(b * 8, 8), :] = jnp.take_along_axis(v, src_lane[c], axis=1, mode="promise_in_bounds")

    def prep_rush(p):
        z = opaque()
        for b in range(D // 16):
            tiles = select(p, b, z)
            gather_lanes(p, 0, b, tiles[0])
            wqkv_t[pl.ds(D // 2 + b * 8, 8), :] = tiles[1]

    def prep_select(p, j, first):
        z = opaque()
        for b in (2 * j, 2 * j + 1):
            tiles = select(p, b, z)
            for c in range(first, NT):
                wqkv_t[pl.ds(c * D // 2 + b * 8, 8), :] = tiles[c]
        return after(wqkv_t, (NT - 1) * D // 2)

    def prep_gather(p, c):
        hold(wqkv_t, NT * D // 2)
        z = opaque()
        for b in range(D // 16):
            gather_lanes(p, c, b, wqkv_t[pl.ds(z + (c * D // 2 + b * 8), 8), :])

    def wo_widen(t, j):
        need(id(late_copies[0]))
        wo_f[t][pl.ds(j * 128, 128), :] = _unpack(wo_raw[pl.ds(j * 64, 64), pl.ds(t * 128, 128)]).astype(f32)
        return after(wo_f[t])

    def wo_permute(t, c):
        written.add(("wo", t, c))
        z = opaque()
        for g in range(4):
            wo_p[t][pl.ds(c * 64 + g * 16, 16), :] = _pack(wo_f[t][pl.ds(z + (5 * g + c), 32, stride=DH), :])
        return after(wo_p[t])

    def window_pair(ref, z, c, row, w):
        t = ref[pl.ds(z + (row + c * KS + HALO - 8 - DIL * w), G + 8), :]
        return t[8:], t[:G]

    def attn_qk(g, w):
        mb, j = divmod(g, NG)
        need(*[("qkv", b, n) for b in (mb, max(mb - 1, 0)) for n in range(3 * NT)])
        z = opaque()
        if w == 0:
            hold(q_s[mb], M)
            st["q"] = [q_s[mb][pl.ds(z + (c * QS + j * G), G), :] for c in range(NT)]
        else:
            hold(k_s[mb], NT * KS)
        ps = None
        for c in range(NT):
            t = [st["q"][c] * k for k in window_pair(k_s[mb], z, c, j * G, w)]
            ps = t if ps is None else [a + b for a, b in zip(ps, t)]
        st["p", g, w] = [(p, pltpu.roll(p, 64, 1)) for p in ps]

    def attn_qk_store(g, w):
        written.add(("p", g, w))
        for slot, (p, r) in zip((w, w + W // 2), st.pop(("p", g, w))):
            p_s[g % NP][pl.ds(slot * G, G), :] = p + r
        return after(p_s[g % NP])

    def attn_logits(g):
        need(*[("p", g, w) for w in range(W // 2)])
        z = opaque()
        hold(p_s[g % NP], W * G)
        ps = [p_s[g % NP][pl.ds(z + w * G, G), :] for w in range(W)]
        st["l", g] = [p + pltpu.roll(p, 32, 1) for p in ps]

    def attn_softmax(g):
        logits = st.pop(("l", g))
        for w in range(W):
            if g * G < DIL * w:
                pos = g * G + lax.broadcasted_iota(i32, (G, 128), 0)
                logits[w] = jnp.where(pos >= DIL * w, logits[w], MASKED)
        m = _tree(jnp.maximum, logits)
        e = [jnp.exp2(l - m) for l in logits]
        inv = pltpu.reciprocal(_tree(jnp.add, e), approx=True)
        st["e", g] = e, inv
        return pltpu.bitcast(inv[:8], i32) | pltpu.bitcast(inv[8:], i32)

    def attn_pv(g, c):
        written.add(("o", g, c))
        mb, j = divmod(g, NG)
        z = opaque()
        e, inv = st["e", g]
        acc = None
        for w in range(W // 2):
            near, far = window_pair(v_s[mb], z, c, j * G, w)
            t = e[w] * near + e[w + W // 2] * far
            acc = t if acc is None else acc + t
        acc = acc * inv
        token = pltpu.bitcast(acc[:8], i32) | pltpu.bitcast(acc[8:], i32)
        o_v[mb].bitcast(bf16)[pl.ds(j * G, G), pl.ds(c * 128, 128)] = acc.astype(bf16)
        return token

    row = lax.broadcasted_iota(i32, (16, D), 0)

    def tile_of(t):
        return pl.ds(pl.multiple_of((t // 16) * 8, 8), 8)

    def token_of(v):
        return pltpu.bitcast(jnp.broadcast_to(v, (8, 128)), i32)

    def top(k):
        if k == 0:
            need(*[("r", g) for g in range(S // G)])
            st["score"] = _rb(jnp.concatenate(st["r"], axis=0))
            st["pos"] = jnp.concatenate([lane * 8 + sub, (lane + 128) * 8 + sub], axis=0).astype(f32)
            st["key"] = jnp.where(st["score"] == st["score"], st["score"], -jnp.inf)
            st["free"], st["i"] = jnp.full((16, 128), True), []
        if k % 2 == 0:
            st["max"] = jnp.max(st["key"], keepdims=True)
            return token_of(st["max"])
        i = jnp.min(jnp.where((st["key"] == st["max"]) & st["free"], st["pos"], S - 1.0), keepdims=True)
        st["i"].append(i)
        st["free"] = st["pos"] != i
        st["key"] = jnp.where(st["free"], st["key"], -jnp.inf)
        return token_of(i)

    def route():
        written.add("xs")
        st["rs"] = [jnp.sum(jnp.where(st["pos"] == i, st["score"], 0.0), keepdims=True) for i in st["i"]]
        st["t"] = [i.astype(i32)[0, 0] for i in st["i"]]

        def pick(t):
            z = _unpack(z_v[tile_of(t), :]).astype(f32)
            return jnp.sum(jnp.where(row == t % 16, z, 0.0), axis=0, keepdims=True)

        xs = jnp.where(row == 0, pick(st["t"][0]), pick(st["t"][1]))
        xs_v[pl.ds(0, 8), :] = _pack(xs)
        return pltpu.bitcast(xs[:8, :128], i32) | token_of(st["rs"][0]) | token_of(st["rs"][1])

    def ffn_cols(j):
        return pl.ds(j * 128, min(128, F - j * 128))

    def ffn_weights(ref, j):
        need("xs", *map(id, late_copies))
        return _unpack(ref[pl.ds(j * 64, min(64, F // 2 - j * 64)), :])

    def ffn_in(ref, j):
        return lax.dot_general(_unpack(xs_v[pl.ds(0, 8), :]), ffn_weights(ref, j), TRANSPOSED_RHS,
                               preferred_element_type=f32)

    def ffn_gate(j):
        st["gate"] = ffn_in(wg_v, j)

    def ffn_up(j):
        gate = _rb(st.pop("gate"))
        up = _rb(ffn_in(wu_v, j))
        hid_v[pl.ds(0, 16), ffn_cols(j)] = (_rb(gate * jax.nn.sigmoid(gate)) * up).astype(bf16)

    def ffn_down(j):
        written.add(("y", j))
        y = jnp.dot(hid_v[pl.ds(0, 16), ffn_cols(j)], ffn_weights(wd_v, j), preferred_element_type=f32)[:8]
        st["y"] = y if j == 0 else st["y"] + y

    def scatter():
        need(("y", pl.cdiv(F, 128) - 1))
        written.add("z")
        for j, t in enumerate(st["t"]):
            upd = _rb(_rb(st["y"][j:j + 1]) * _rb(jax.nn.sigmoid(st["rs"][j])))
            z = _unpack(z_v[tile_of(t), :]).astype(f32)
            z_v[tile_of(t), :] = _pack(jnp.where(row == t % 16, z + upd, z))

    def piece_dot(lhs_ref, rhs_ref, ties):
        z = opaque()
        cols = []
        for k in range(NT):
            col = lhs_ref[pl.ds(z, M // 2), pl.ds(k * 128, 128)]
            if any(kk == k for kk, _ in ties):
                parts = [col[r * 8:(r + 1) * 8] for r in range(M // 16)]
                for (kk, r), token in ties.items():
                    if kk == k:
                        parts[r] = parts[r] | (token & zero)
                col = jnp.concatenate(parts, axis=0)
            cols.append(col)
        lhs = _unpack(jnp.concatenate(cols, axis=1))
        return jnp.dot(lhs, _unpack(rhs_ref[pl.ds(z, D // 2), :]), preferred_element_type=f32)

    def qkv_dot(mb, n, ties):
        need(("w", n), *[("xn", mb * NG + j) for j in range(NG)])
        return piece_dot(xn_v[mb], wqkv_p[n], ties)

    def qkv_store(mb, n, res):
        written.add(("qkv", mb, n))
        p, c = divmod(n, NT)
        if p == 0:
            q_s[mb][pl.ds(c * QS, M), :] = res * QSCALE
            return
        dst = (k_s, v_s)[p - 1]
        dst[mb][pl.ds(c * KS + HALO, M), :] = res
        if mb == 0:
            dst[0][pl.ds(c * KS, HALO), :] = jnp.broadcast_to(res[0:1], (HALO, 128))
        if mb + 1 < NM:
            dst[mb + 1][pl.ds(c * KS, HALO), :] = res[M - HALO:]

    def out_dot(mb, c, ties):
        need(*[("wo", c, k) for k in range(NT)], *[("o", mb * NG + j, k) for j in range(NG) for k in range(NT)])
        return piece_dot(o_v[mb], wo_p[c], ties)

    def out_store(mb, c, s):
        need("z")
        rows, cols = pl.ds(mb * M, M), pl.ds(c * 128, 128)
        z = _unpack(z_v[pl.ds(mb * M // 2 + opaque(), M // 2), cols]).astype(f32)
        gate = z * pltpu.reciprocal(1.0 + jnp.exp2(z * -LOG2E), approx=True)
        res = x_rows(mb * M, M, cols) + s * gate
        out_v[rows, cols] = res.astype(bf16)
        if mb == NM - 1:
            pltpu.make_async_copy(out_v.at[rows, cols], out_hbm.at[rows, cols], sem_o).start()
        elif c == NT - 1:
            pltpu.make_async_copy(out_v.at[rows, :], out_hbm.at[rows, :], sem_o).start()
        return pltpu.bitcast(res[M - 8:], i32)

    qkv, out = (qkv_dot, qkv_store), (out_dot, out_store)
    pieces = [(qkv, mb, n) for n in range(2 * NT) for mb in range(NF)]
    pieces += [(qkv, mb, n) for mb in range(NF, NV) for n in range(2 * NT)]
    pieces += [(qkv, mb, n) for n in range(2 * NT, 3 * NT) for mb in range(NV)]
    pieces += [(qkv, mb, n) for mb in range(NV, NM) for n in range(3 * NT)]
    nq = len(pieces)
    pieces += [(out, mb, c) for mb in range(NM) for c in range(NT)]
    nf = pl.cdiv(F, 128)
    ffn = {}
    for j in range(nf):
        ffn[WAIT_LATE + 1 + 4 * j] = ffn_gate, j
        ffn[WAIT_LATE + 3 + 4 * j] = ffn_up, j
        ffn[WAIT_LATE + 4 + 4 * nf + 2 * j] = ffn_down, j
    busy, start = [0] * 4, []
    for i in range(len(pieces)):
        for rows in ([16] * NT if i in ffn else []) + [M] * NT:
            m = busy.index(min(busy))
            if rows == M:
                start.append(busy[m])
            busy[m] += rows
    start = np.reshape(start, (-1, NT)).tolist()
    begin = [0]
    for i in range(1, len(pieces)):
        begin.append(max(start[i][0], min(begin[-1] + PIECE, start[i - 1][-1] + M - 1)))
    tasks = []

    def at(t, limit, fn, *args):
        tasks.append((t, len(tasks), limit, fn, args))

    def piece_at(t):
        return bisect.bisect_right(begin, t) - 1

    def layernorm(lo, hi, t0, t1, sum_steps):
        stages = (ln_mean, ln_var, ln_scale, ln_norm, ln_dot)
        lags = (0, sum_steps + 1, 2 * sum_steps + 2, 2 * sum_steps + 6, 2 * sum_steps + 7)
        groups = (hi - lo) * NG
        n = groups + lags[-1] + sum_steps
        for t in range(n):
            when = [t0 + (t * 100 + phase) * (t1 - t0) // (100 * n) for phase in LN_PHASE]
            for k, fn, tk in zip(lags, stages, when):
                if 0 <= t - k < groups:
                    at(tk, t1 and (260 if fn is ln_scale else EXACT), fn, lo * NG + t - k)
            if t < n - sum_steps:
                at(when[5], t1 and EXACT, ln_reduce)
            if t >= sum_steps:
                at(when[6], t1 and EXACT, ln_finish)

    layernorm(0, NF, 0, 0, 3)
    starts = (x_copies[1:2], qkv_copies[2:], late_copies)
    waits = (qkv_copies[:1], qkv_copies[1:2], (qkv_copies[2], x_copies[2]))
    for p, first in enumerate(WAIT_W):
        t = first * PIECE
        at(t, 0, dma_point, starts[p], waits[p])
        rushed = 2 if p < 2 else 0
        if rushed:
            at(t, 0, prep_rush, p)
            at(t, 0, prep_gather, p, 1)
        for j in range(20):
            at(t + SELECT_AT[p] + j * SELECT_GAP[p], EXACT, prep_select, p, j, rushed)
        for c in range(rushed, NT):
            at(t + SELECT_AT[p] + 20 * SELECT_GAP[p] + (c - rushed) * GATHER_GAP[p], EXACT, prep_gather, p, c)
    at(WAIT_X * PIECE, 0, dma_point, x_copies[2:], x_copies[1:2])
    for lo, hi, first, last in LN_SPANS:
        layernorm(lo, hi, first * PIECE, last * PIECE, LN_SUM_STEPS)
    base = ATT_START * PIECE
    layernorm(NX, NM, LN_START * PIECE, base - 300, LN_SUM_STEPS)
    for k in range(4):
        at(base + k * 400, LOOSE, top, k)
    at(base + 4 * 400, LOOSE, route)

    knots = [base, begin[WAIT_LATE] - 580, begin[WAIT_LATE] - 380, begin[max(ffn)],
             begin[nq] + 600, begin[nq] + 600 + 65 * PIECE]
    work = np.cumsum([0] + [(b - a) * rate for a, b, rate in zip(knots, knots[1:], ATT_RATE)])

    def frame(g):
        return int(np.interp((g + QK_LAG) * work[-1] / (NM * NG + QK_LAG), work, knots))

    for g in range(NM * NG):
        for w in range(W // 2):
            at(frame(g - QK_LAG) + QK_AT + w * QK_GAP, LOOSE, attn_qk, g, w)
            at(frame(g - QK_LAG) + QK_AT + w * QK_GAP + QK_STORE, EXACT, attn_qk_store, g, w)
        at(frame(g), LOOSE, attn_logits, g)
        at(frame(g) + EXP_AT, EXACT, attn_softmax, g)
        for c in range(NT):
            at(frame(g) + PV_AT + c * PV_GAP, EXACT, attn_pv, g, c)
    at(begin[WAIT_LATE], 0, dma_point, [], late_copies)
    for j in range(2 * NT * NT):
        t = begin[nq] - 60 * PIECE + j * 56 * PIECE // (2 * NT * NT)
        at(t, EXACT, (wo_widen, wo_permute)[j // NT % 2], j // (2 * NT), j % NT)
    at(begin[nq - 2], 0, scatter)

    due = collections.defaultdict(list)
    for task in sorted(tasks, key=lambda task: task[:2]):
        due[piece_at(task[0])].append(task)
    results = []
    ties = collections.defaultdict(dict)

    def result_at(t):
        i = len(results) - 1
        while i >= 0 and start[i][-1] + LATENCY > t:
            i -= 1
        if i < 0:
            return None
        r = min((t - LATENCY - start[i][-1]) // 8, M // 8 - 1)
        return results[i][r * 8:(r + 1) * 8]

    def tie(t, token):
        if token is not None:
            i = piece_at(t)
            k = 0 if t - start[i][0] < M else NT - 1
            key = k, min(max(t - start[i][k], 0) // 16, M // 16 - 1)
            ties[i][key] = ties[i][key] | token if key in ties[i] else token

    def store(i):
        (_, fn), mb, n = pieces[i]
        token = fn(mb, n, results[i])
        if i + OUT_LAG < len(pieces):
            tie(begin[i + OUT_LAG], token)

    for i, ((dot, _), mb, n) in enumerate(pieces):
        for t, _, limit, fn, args in due.pop(i, []):
            st["go"] = result_at(t) if limit else None
            token = fn(*args)
            if limit:
                tie(t + limit, token)
        if i >= STORE_LAG:
            store(i - STORE_LAG)
        if i in ffn:
            ffn[i][0](ffn[i][1])
        results.append(dot(mb, n, ties.pop(i, {})))
    for i in range(len(pieces) - STORE_LAG, len(pieces)):
        store(i)
    pltpu.make_async_copy(out_v, out_hbm, sem_o).wait()


def _fused():
    scratch = [
        [pltpu.VMEM(((b - a) // 2, D), i32) for a, b in zip(X_BOUNDS, X_BOUNDS[1:])],
        pltpu.VMEM((S // 2, D), i32),
        [pltpu.VMEM((D // 2, D), i32)] * 3,
        pltpu.VMEM((NT * D // 2 + 32, 128), i32),
        [pltpu.VMEM((D // 2, 128), i32)] * (3 * NT),
        pltpu.VMEM((D // 2, D), i32),
        [pltpu.VMEM((D, 128), f32)] * NT,
        [pltpu.VMEM((D // 2, 128), i32)] * NT,
        pltpu.VMEM((F // 2, D), i32),
        pltpu.VMEM((F // 2, D), i32),
        pltpu.VMEM((F // 2, D), i32),
        [pltpu.VMEM((M // 2, D), i32)] * NM,
        [pltpu.VMEM((NT * QS + 24, 128), f32)] * NM,
        [pltpu.VMEM((NT * KS + 16, 128), f32)] * NM,
        [pltpu.VMEM((NT * KS + 16, 128), f32)] * NM,
        [pltpu.VMEM((M // 2, D), i32)] * NM,
        [pltpu.VMEM((32, 128), f32)] * NSTAT,
        [pltpu.VMEM((32, 128), f32)] * NSTAT,
        [pltpu.VMEM((32, 128), f32)] * NSTAT,
        [pltpu.VMEM((32, 128), f32)] * NSTAT,
        [pltpu.VMEM((W * G + 32, 128), f32)] * NP,
        pltpu.VMEM((S, D), bf16),
        [pltpu.VMEM((32, D), i32)] * NSTAT,
        pltpu.VMEM((32, D), i32),
        pltpu.VMEM((64, F), bf16),
        pltpu.VMEM((D,), bf16),
        pltpu.SemaphoreType.DMA((3,)),
        pltpu.SemaphoreType.DMA((8,)),
        pltpu.SemaphoreType.DMA(()),
    ]
    hbm = pl.BlockSpec(memory_space=pltpu.HBM)
    return pl.pallas_call(
        _kernel,
        out_shape=jax.ShapeDtypeStruct((S, D), bf16),
        in_specs=[hbm] * 7,
        out_specs=hbm,
        scratch_shapes=scratch,
        compiler_params=pltpu.CompilerParams(vmem_limit_bytes=100 * 1024 * 1024),
        name="fused",
    )


@jax.jit
def pallas_recurrent_scan__sliding_local_dilated__moe_arch_mod__prompt_kernel(
    A_x: jax.Array,
    A_wqkv: jax.Array,
    A_wo: jax.Array,
    B_x: jax.Array,
    B_w_r: jax.Array,
    B_w_gate: jax.Array,
    B_w_up: jax.Array,
    B_w_down: jax.Array,
):
    del B_x
    out = _fused()(A_x.reshape(S, D), A_wqkv, A_wo, B_w_r, B_w_gate.T, B_w_up.T, B_w_down)
    return out.reshape(1, S, D)
```

```python
import bisect
import collections
import functools
import itertools
import math

import jax
import jax.numpy as jnp
import numpy as np
from jax import lax
from jax.experimental import pallas as pl
from jax.experimental.pallas import tpu as pltpu

S, D, F = 2048, 640, 1728
DH, W, DIL = 20, 8, 2
NT = D // 128
HALO = 16
M = 128
NM = S // M
G = 16
NG = M // G
NSTAT, NP = 32, 8
QS, KS = M + 8, M + HALO
LOG2E = math.log2(math.e)
QSCALE = DH ** -0.5 * LOG2E
MASKED = -1e9 * LOG2E
EPS = float(np.asarray(1e-5, dtype=jnp.bfloat16).astype(np.float32))
f32, bf16, i32 = jnp.float32, jnp.bfloat16, jnp.int32
TRANSPOSED_RHS = (((1,), (1,)), ((), ()))

PIECE = M * NT // 4
LATENCY = 130
NF, NV, NX = 2, 5, 6
X_BOUNDS = (0, NF * M, NX * M, S)
WAIT_W, WAIT_X, WAIT_LATE = (0, 8, 44), 16, 144
SELECT_AT, SELECT_GAP, GATHER_GAP = (64, 260, 60), (12, 16, 24), (150, 150, 500)
LN_SPANS = ((NF, NF + 1, WAIT_X, 21), (NF + 1, NX, 21, 40))
LN_START, LN_PHASE, LN_SUM_STEPS = 48, (42, 56, 20, 56, 32, 94, 95), 4
ATT_START, ATT_RATE = 100, (1.0, 1e-6, 1.0, 1.0, 0.87)
QK_LAG, QK_AT, QK_GAP, QK_STORE, EXP_AT, PV_AT, PV_GAP = 2, 86, 19, 190, 224, 244, 20
LOOSE, EXACT = 400, 1
STORE_LAG, OUT_LAG, WO_LEAD = 2, 4, 25


def _rb(x):
    return x.astype(bf16).astype(f32)


def _pack(x):
    return pltpu.bitcast(x.astype(bf16), i32)


def _unpack(x):
    return pltpu.bitcast(x, bf16)


def _tree(op, xs):
    while len(xs) > 1:
        xs = [op(a, b) for a, b in zip(xs[::2], xs[1::2])] + xs[len(xs) // 2 * 2:]
    return xs[0]


def _kernel(x_hbm, wqkv_hbm, wo_hbm, wr_hbm, wg_hbm, wu_hbm, wd_hbm, out_hbm,
            x_v, z_v, wqkv_raw, wqkv_t, wqkv_p, wo_raw, wo_p, wg_v, wu_v, wd_v, xn_v, q_s, k_s, v_s, o_v,
            m_s, d_s, i_s, f_s, p_s, out_v, d_v, xs_v, hid_v, wr_v, sem_x, sem_w, sem_o):
    x_copies = [pltpu.make_async_copy(x_hbm.at[pl.ds(a, b - a), :], x_v[j].bitcast(bf16), sem_x.at[j])
                for j, (a, b) in enumerate(zip(X_BOUNDS, X_BOUNDS[1:]))]
    qkv_copies = [pltpu.make_async_copy(wqkv_hbm.at[:, pl.ds(p * D, D)], wqkv_raw[p].bitcast(bf16), sem_w.at[p])
                  for p in range(3)]
    late = [(wo_hbm.at[:, pl.ds(t * 128, 128)], wo_raw[t]) for t in range(NT)]
    late += [(wg_hbm, wg_v), (wu_hbm, wu_v), (wd_hbm, wd_v)]
    late_copies = [pltpu.make_async_copy(src, dst.bitcast(bf16), sem_w.at[4 + j]) for j, (src, dst) in enumerate(late)]
    wr_copy = pltpu.make_async_copy(wr_hbm, wr_v, sem_w.at[3])

    written = set()

    def need(*keys):
        assert written.issuperset(keys), keys

    def dma_point(start, wait):
        for c in start:
            c.start()
        for c in wait:
            c.wait()
            written.add(id(c))

    dma_point([wr_copy, x_copies[0], qkv_copies[0]], x_copies[:1])

    lane = lax.broadcasted_iota(i32, (8, 128), 1)
    sub = lax.broadcasted_iota(i32, (8, 128), 0)
    bits = x_v[0][pl.ds(0, 8), pl.ds(0, 128)] >> 16
    zero = (bits * (bits + 1)) & 1
    zero0 = zero[0, 0]
    fresh, folds = itertools.count(1), itertools.count()
    st = dict(folded=[], sums=[], r=[jnp.zeros((8, 128), f32), jnp.zeros((8, 128), f32)])

    def opaque():
        return pl.multiple_of(zero0 * (next(fresh) * 8), 8)

    def after(ref, row=0):
        return pltpu.bitcast(ref[pl.ds(opaque() + row, 8), pl.ds(0, 128)], i32)

    def hold(ref, row):
        if st["go"] is not None:
            ref[pl.ds(row, 8), :] = pltpu.bitcast(st["go"], ref.dtype)

    def x_rows(row, n, cols=slice(None)):
        j = bisect.bisect_right(X_BOUNDS, row) - 1
        need(id(x_copies[j]))
        return _unpack(x_v[j][pl.ds((row - X_BOUNDS[j]) // 2 + opaque(), n // 2), cols]).astype(f32)

    def wide(v):
        return jnp.concatenate([v] * NT, axis=1)

    def get(refs, g):
        need((id(refs), g))
        return refs[g % NSTAT][pl.ds(opaque(), G), :]

    def put(refs, g, v):
        written.add((id(refs), g))
        refs[g % NSTAT][pl.ds(0, G), :] = jnp.broadcast_to(v, (G, 128))
        return after(refs[g % NSTAT])

    def fold(g, then, v):
        ref = f_s[next(folds) % NSTAT]
        ref[pl.ds(0, G), :] = _tree(jnp.add, [v[:, c * 128:(c + 1) * 128] for c in range(NT)])
        st["folded"].append((then, g, ref))
        return after(ref)

    def ln_reduce():
        sums = []
        for then, g, ref in st["folded"]:
            hold(ref, G)
            sums.append((then, g, jnp.sum(ref[pl.ds(opaque(), G), :], axis=1, keepdims=True)))
        st["folded"] = []
        st["sums"].append(sums)

    def ln_finish():
        tokens = [then(g, v) for then, g, v in st["sums"].pop(0)]
        return functools.reduce(jnp.bitwise_or, tokens) if tokens else None

    def ln_mean(g):
        return fold(g, lambda g, v: put(m_s, g, v * (1.0 / D)), x_rows(g * G, G))

    def ln_var(g):
        d = x_rows(g * G, G) - wide(_rb(get(m_s, g)))
        d_v[g % NSTAT].bitcast(bf16)[pl.ds(0, G), :] = d.astype(bf16)
        return fold(g, lambda g, v: put(d_s, g, v * (1.0 / D)), d * d)

    def ln_scale(g):
        hold(d_s[g % NSTAT], G)
        m = get(m_s, g)
        shift = m - _rb(m)
        var = jnp.maximum(get(d_s, g) - shift * shift, 0.0)
        den = jnp.minimum(_rb(jnp.sqrt(_rb(_rb(var) + EPS))), 3e38)
        inv = pltpu.reciprocal(den, approx=True)
        return put(i_s, g, inv * (2.0 - den * inv))

    def ln_norm(g):
        written.add(("xn", g))
        d = _unpack(d_v[g % NSTAT][pl.ds(opaque(), G // 2), :]).astype(f32)
        xn = (d * wide(get(i_s, g))).astype(bf16)
        z_v.bitcast(bf16)[pl.ds(g * G, G), :] = xn
        xn_v[g // NG].bitcast(bf16)[pl.ds(g % NG * G, G), :] = xn
        return after(xn_v[g // NG])

    def keep_score(g, r):
        written.add(("r", g))
        for s in range(G // 8):
            half, l = divmod(g * G // 8 + s, 128)
            st["r"][half] = jnp.where(lane == l, jnp.broadcast_to(r[s * 8:(s + 1) * 8], (8, 128)), st["r"][half])
        return pltpu.bitcast(st["r"][half], i32)

    def ln_dot(g):
        need(("xn", g))
        if g == 0:
            dma_point(qkv_copies[1:2], [wr_copy])
            st["wr"] = wr_v[...].astype(f32).reshape(1, D)
        xn = _unpack(z_v[pl.ds(g * G // 2 + opaque(), G // 2), :])
        return fold(g, keep_score, xn.astype(f32) * st["wr"])

    src_lane = [(20 * (lane & 31) + 5 * (lane >> 5) + c) & 127 for c in range(NT)]
    turn = (130 - lane) * 2
    turn = turn - ((turn * 205) >> 10) * 5
    turns = [(step, turn & step != 0) for step in (1, 2, 4)]

    def select(p, b, z):
        need(id(qkv_copies[p]))
        tiles = [wqkv_raw[p][pl.ds(z + b * 8, 8), pl.ds(t * 128, 128)] for t in range(NT)]
        for step, mask in turns:
            tiles = [jnp.where(mask, tiles[(t + step) % NT], tiles[t]) for t in range(NT)]
        return [tiles[2 * c % NT] for c in range(NT)]

    def gather_lanes(p, c, b, v):
        written.add(("w", p * NT + c))
        wqkv_p[p * NT + c][pl.ds(b * 8, 8), :] = jnp.take_along_axis(v, src_lane[c], axis=1, mode="promise_in_bounds")

    def prep_rush(p):
        z = opaque()
        for b in range(D // 16):
            tiles = select(p, b, z)
            gather_lanes(p, 0, b, tiles[0])
            wqkv_t[pl.ds(D // 2 + b * 8, 8), :] = tiles[1]

    def prep_select(p, j, first):
        z = opaque()
        for b in (2 * j, 2 * j + 1):
            tiles = select(p, b, z)
            for c in range(first, NT):
                wqkv_t[pl.ds(c * D // 2 + b * 8, 8), :] = tiles[c]
        return after(wqkv_t, (NT - 1) * D // 2)

    def prep_gather(p, c):
        hold(wqkv_t, NT * D // 2)
        z = opaque()
        for b in range(D // 16):
            gather_lanes(p, c, b, wqkv_t[pl.ds(z + (c * D // 2 + b * 8), 8), :])

    def wo_permute(t, c):
        need(id(late_copies[t]))
        written.add(("wo", t, c))
        z = opaque()
        for g in range(4):
            word, upper = divmod(5 * g + c, 2)
            even, odd = (wo_raw[t][pl.ds(z + (word + k), 16, stride=DH), :] for k in (0, DH // 2))
            if upper:
                pair = ((even >> 16) & 0xFFFF) | (odd & -0x10000)
            else:
                pair = (even & 0xFFFF) | (odd << 16)
            wo_p[t][pl.ds(c * 64 + g * 16, 16), :] = pair
        return after(wo_p[t])

    def window_pair(ref, z, c, row, w):
        t = ref[pl.ds(z + (row + c * KS + HALO - 8 - DIL * w), G + 8), :]
        return t[8:], t[:G]

    def attn_qk(g, w):
        mb, j = divmod(g, NG)
        need(*[("qkv", b, n) for b in (mb, max(mb - 1, 0)) for n in range(3 * NT)])
        z = opaque()
        if w == 0:
            hold(q_s[mb], M)
            st["q"] = [q_s[mb][pl.ds(z + (c * QS + j * G), G), :] for c in range(NT)]
        else:
            hold(k_s[mb], NT * KS)
        ps = None
        for c in range(NT):
            t = [st["q"][c] * k for k in window_pair(k_s[mb], z, c, j * G, w)]
            ps = t if ps is None else [a + b for a, b in zip(ps, t)]
        st["p", g, w] = [(p, pltpu.roll(p, 64, 1)) for p in ps]

    def attn_qk_store(g, w):
        written.add(("p", g, w))
        for slot, (p, r) in zip((w, w + W // 2), st.pop(("p", g, w))):
            p_s[g % NP][pl.ds(slot * G, G), :] = p + r
        return after(p_s[g % NP])

    def attn_logits(g):
        need(*[("p", g, w) for w in range(W // 2)])
        z = opaque()
        hold(p_s[g % NP], W * G)
        ps = [p_s[g % NP][pl.ds(z + w * G, G), :] for w in range(W)]
        st["l", g] = [p + pltpu.roll(p, 32, 1) for p in ps]

    def attn_softmax(g):
        logits = st.pop(("l", g))
        for w in range(W):
            if g * G < DIL * w:
                pos = g * G + lax.broadcasted_iota(i32, (G, 128), 0)
                logits[w] = jnp.where(pos >= DIL * w, logits[w], MASKED)
        m = _tree(jnp.maximum, logits)
        e = [jnp.exp2(l - m) for l in logits]
        inv = pltpu.reciprocal(_tree(jnp.add, e), approx=True)
        st["e", g] = e, inv
        return pltpu.bitcast(inv[:8], i32) | pltpu.bitcast(inv[8:], i32)

    def attn_pv(g, c):
        written.add(("o", g, c))
        mb, j = divmod(g, NG)
        z = opaque()
        e, inv = st["e", g]
        acc = None
        for w in range(W // 2):
            near, far = window_pair(v_s[mb], z, c, j * G, w)
            t = e[w] * near + e[w + W // 2] * far
            acc = t if acc is None else acc + t
        acc = acc * inv
        token = pltpu.bitcast(acc[:8], i32) | pltpu.bitcast(acc[8:], i32)
        o_v[mb].bitcast(bf16)[pl.ds(j * G, G), pl.ds(c * 128, 128)] = acc.astype(bf16)
        return token

    row = lax.broadcasted_iota(i32, (16, D), 0)

    def tile_of(t):
        return pl.ds(pl.multiple_of((t // 16) * 8, 8), 8)

    def token_of(v):
        return pltpu.bitcast(jnp.broadcast_to(v, (8, 128)), i32)

    def top(k):
        if k == 0:
            need(*[("r", g) for g in range(S // G)])
            st["score"] = _rb(jnp.concatenate(st["r"], axis=0))
            st["pos"] = jnp.concatenate([lane * 8 + sub, (lane + 128) * 8 + sub], axis=0).astype(f32)
            st["key"] = jnp.where(st["score"] == st["score"], st["score"], -jnp.inf)
            st["free"], st["i"] = jnp.full((16, 128), True), []
        if k % 2 == 0:
            st["max"] = jnp.max(st["key"], keepdims=True)
            return token_of(st["max"])
        i = jnp.min(jnp.where((st["key"] == st["max"]) & st["free"], st["pos"], S - 1.0), keepdims=True)
        st["i"].append(i)
        st["free"] = st["pos"] != i
        st["key"] = jnp.where(st["free"], st["key"], -jnp.inf)
        return token_of(i)

    def route():
        written.add("xs")
        st["rs"] = [jnp.sum(jnp.where(st["pos"] == i, st["score"], 0.0), keepdims=True) for i in st["i"]]
        st["t"] = [i.astype(i32)[0, 0] for i in st["i"]]

        def pick(t):
            z = _unpack(z_v[tile_of(t), :]).astype(f32)
            return jnp.sum(jnp.where(row == t % 16, z, 0.0), axis=0, keepdims=True)

        xs = jnp.where(row == 0, pick(st["t"][0]), pick(st["t"][1]))
        xs_v[pl.ds(0, 8), :] = _pack(xs)
        return pltpu.bitcast(xs[:8, :128], i32) | token_of(st["rs"][0]) | token_of(st["rs"][1])

    def ffn_cols(j):
        return pl.ds(j * 128, min(128, F - j * 128))

    def ffn_weights(ref, j):
        need("xs", *map(id, late_copies))
        return _unpack(ref[pl.ds(j * 64, min(64, F // 2 - j * 64)), :])

    def ffn_in(ref, j):
        return lax.dot_general(_unpack(xs_v[pl.ds(0, 8), :]), ffn_weights(ref, j), TRANSPOSED_RHS,
                               preferred_element_type=f32)

    def ffn_gate(j):
        st["gate"] = ffn_in(wg_v, j)

    def ffn_up(j):
        gate = _rb(st.pop("gate"))
        up = _rb(ffn_in(wu_v, j))
        hid_v[pl.ds(0, 16), ffn_cols(j)] = (_rb(gate * jax.nn.sigmoid(gate)) * up).astype(bf16)

    def ffn_down(j):
        written.add(("y", j))
        y = jnp.dot(hid_v[pl.ds(0, 16), ffn_cols(j)], ffn_weights(wd_v, j), preferred_element_type=f32)[:8]
        st["y"] = y if j == 0 else st["y"] + y

    def scatter():
        need(("y", pl.cdiv(F, 128) - 1))
        written.add("z")
        for j, t in enumerate(st["t"]):
            upd = _rb(_rb(st["y"][j:j + 1]) * _rb(jax.nn.sigmoid(st["rs"][j])))
            z = _unpack(z_v[tile_of(t), :]).astype(f32)
            z_v[tile_of(t), :] = _pack(jnp.where(row == t % 16, z + upd, z))

    def piece_dot(lhs_ref, rhs_ref, ties):
        z = opaque()
        cols = []
        for k in range(NT):
            col = lhs_ref[pl.ds(z, M // 2), pl.ds(k * 128, 128)]
            if any(kk == k for kk, _ in ties):
                parts = [col[r * 8:(r + 1) * 8] for r in range(M // 16)]
                for (kk, r), token in ties.items():
                    if kk == k:
                        parts[r] = parts[r] | (token & zero)
                col = jnp.concatenate(parts, axis=0)
            cols.append(col)
        lhs = _unpack(jnp.concatenate(cols, axis=1))
        return jnp.dot(lhs, _unpack(rhs_ref[pl.ds(z, D // 2), :]), preferred_element_type=f32)

    def qkv_dot(mb, n, ties):
        need(("w", n), *[("xn", mb * NG + j) for j in range(NG)])
        return piece_dot(xn_v[mb], wqkv_p[n], ties)

    def qkv_store(mb, n, res):
        written.add(("qkv", mb, n))
        p, c = divmod(n, NT)
        if p == 0:
            q_s[mb][pl.ds(c * QS, M), :] = res * QSCALE
            return
        dst = (k_s, v_s)[p - 1]
        dst[mb][pl.ds(c * KS + HALO, M), :] = res
        if mb == 0:
            dst[0][pl.ds(c * KS, HALO), :] = jnp.broadcast_to(res[0:1], (HALO, 128))
        if mb + 1 < NM:
            dst[mb + 1][pl.ds(c * KS, HALO), :] = res[M - HALO:]

    def out_dot(mb, c, ties):
        need(*[("wo", c, k) for k in range(NT)], *[("o", mb * NG + j, k) for j in range(NG) for k in range(NT)])
        return piece_dot(o_v[mb], wo_p[c], ties)

    def out_store(mb, c, s):
        need("z")
        rows, cols = pl.ds(mb * M, M), pl.ds(c * 128, 128)
        z = _unpack(z_v[pl.ds(mb * M // 2 + opaque(), M // 2), cols]).astype(f32)
        gate = z * pltpu.reciprocal(1.0 + jnp.exp2(z * -LOG2E), approx=True)
        res = x_rows(mb * M, M, cols) + s * gate
        out_v[rows, cols] = res.astype(bf16)
        if mb == NM - 1:
            pltpu.make_async_copy(out_v.at[rows, cols], out_hbm.at[rows, cols], sem_o).start()
        elif c == NT - 1:
            pltpu.make_async_copy(out_v.at[rows, :], out_hbm.at[rows, :], sem_o).start()
        return pltpu.bitcast(res[M - 8:], i32)

    qkv, out = (qkv_dot, qkv_store), (out_dot, out_store)
    pieces = [(qkv, mb, n) for n in range(2 * NT) for mb in range(NF)]
    pieces += [(qkv, mb, n) for mb in range(NF, NV) for n in range(2 * NT)]
    pieces += [(qkv, mb, n) for n in range(2 * NT, 3 * NT) for mb in range(NV)]
    pieces += [(qkv, mb, n) for mb in range(NV, NM) for n in range(3 * NT)]
    nq = len(pieces)
    pieces += [(out, mb, c) for mb in range(NM) for c in range(NT)]
    nf = pl.cdiv(F, 128)
    ffn = {}
    for j in range(nf):
        ffn[WAIT_LATE + 1 + 4 * j] = ffn_gate, j
        ffn[WAIT_LATE + 3 + 4 * j] = ffn_up, j
        ffn[WAIT_LATE + 4 + 4 * nf + 2 * j] = ffn_down, j
    busy, start = [0] * 4, []
    for i in range(len(pieces)):
        for rows in ([16] * NT if i in ffn else []) + [M] * NT:
            m = busy.index(min(busy))
            if rows == M:
                start.append(busy[m])
            busy[m] += rows
    start = np.reshape(start, (-1, NT)).tolist()
    begin = [0]
    for i in range(1, len(pieces)):
        begin.append(max(start[i][0], min(begin[-1] + PIECE, start[i - 1][-1] + M - 1)))
    tasks = []

    def at(t, limit, fn, *args):
        tasks.append((t, len(tasks), limit, fn, args))

    def piece_at(t):
        return bisect.bisect_right(begin, t) - 1

    def layernorm(lo, hi, t0, t1, sum_steps):
        stages = (ln_mean, ln_var, ln_scale, ln_norm, ln_dot)
        lags = (0, sum_steps + 1, 2 * sum_steps + 2, 2 * sum_steps + 6, 2 * sum_steps + 7)
        groups = (hi - lo) * NG
        n = groups + lags[-1] + sum_steps
        for t in range(n):
            when = [t0 + (t * 100 + phase) * (t1 - t0) // (100 * n) for phase in LN_PHASE]
            for k, fn, tk in zip(lags, stages, when):
                if 0 <= t - k < groups:
                    at(tk, t1 and (260 if fn is ln_scale else EXACT), fn, lo * NG + t - k)
            if t < n - sum_steps:
                at(when[5], t1 and EXACT, ln_reduce)
            if t >= sum_steps:
                at(when[6], t1 and EXACT, ln_finish)

    layernorm(0, NF, 0, 0, 3)
    starts = (x_copies[1:2], qkv_copies[2:], late_copies)
    waits = (qkv_copies[:1], qkv_copies[1:2], (qkv_copies[2], x_copies[2]))
    for p, first in enumerate(WAIT_W):
        t = first * PIECE
        at(t, 0, dma_point, starts[p], waits[p])
        rushed = 2 if p < 2 else 0
        if rushed:
            at(t, 0, prep_rush, p)
            at(t, 0, prep_gather, p, 1)
        for j in range(20):
            at(t + SELECT_AT[p] + j * SELECT_GAP[p], EXACT, prep_select, p, j, rushed)
        for c in range(rushed, NT):
            at(t + SELECT_AT[p] + 20 * SELECT_GAP[p] + (c - rushed) * GATHER_GAP[p], EXACT, prep_gather, p, c)
    at(WAIT_X * PIECE, 0, dma_point, x_copies[2:], x_copies[1:2])
    for lo, hi, first, last in LN_SPANS:
        layernorm(lo, hi, first * PIECE, last * PIECE, LN_SUM_STEPS)
    base = ATT_START * PIECE
    layernorm(NX, NM, LN_START * PIECE, base - 300, LN_SUM_STEPS)
    for k in range(4):
        at(base + k * 400, LOOSE, top, k)
    at(base + 4 * 400, LOOSE, route)

    knots = [base, begin[WAIT_LATE] - 580, begin[WAIT_LATE] - 380, begin[max(ffn)],
             begin[nq] + 600, begin[nq] + 600 + 65 * PIECE]
    work = np.cumsum([0] + [(b - a) * rate for a, b, rate in zip(knots, knots[1:], ATT_RATE)])

    def frame(g):
        return int(np.interp((g + QK_LAG) * work[-1] / (NM * NG + QK_LAG), work, knots))

    for g in range(NM * NG):
        for w in range(W // 2):
            at(frame(g - QK_LAG) + QK_AT + w * QK_GAP, LOOSE, attn_qk, g, w)
            at(frame(g - QK_LAG) + QK_AT + w * QK_GAP + QK_STORE, EXACT, attn_qk_store, g, w)
        at(frame(g), LOOSE, attn_logits, g)
        at(frame(g) + EXP_AT, EXACT, attn_softmax, g)
        for c in range(NT):
            at(frame(g) + PV_AT + c * PV_GAP, EXACT, attn_pv, g, c)
    at(begin[WAIT_LATE], 0, dma_point, [], late_copies)
    for j in range(NT * NT):
        at(begin[nq] - (WO_LEAD * (NT * NT - j) // (NT * NT) + 2) * PIECE, EXACT, wo_permute, *divmod(j, NT))
    at(begin[nq - 2], 0, scatter)

    due = collections.defaultdict(list)
    for task in sorted(tasks, key=lambda task: task[:2]):
        due[piece_at(task[0])].append(task)
    results = []
    ties = collections.defaultdict(dict)

    def result_at(t):
        i = len(results) - 1
        while i >= 0 and start[i][-1] + LATENCY > t:
            i -= 1
        if i < 0:
            return None
        r = min((t - LATENCY - start[i][-1]) // 8, M // 8 - 1)
        return results[i][r * 8:(r + 1) * 8]

    def tie(t, token):
        if token is not None:
            i = piece_at(t)
            k = 0 if t - start[i][0] < M else NT - 1
            key = k, min(max(t - start[i][k], 0) // 16, M // 16 - 1)
            ties[i][key] = ties[i][key] | token if key in ties[i] else token

    def store(i):
        (_, fn), mb, n = pieces[i]
        token = fn(mb, n, results[i])
        if i + OUT_LAG < len(pieces):
            tie(begin[i + OUT_LAG], token)

    for i, ((dot, _), mb, n) in enumerate(pieces):
        for t, _, limit, fn, args in due.pop(i, []):
            st["go"] = result_at(t) if limit else None
            token = fn(*args)
            if limit:
                tie(t + limit, token)
        if i >= STORE_LAG:
            store(i - STORE_LAG)
        if i in ffn:
            ffn[i][0](ffn[i][1])
        results.append(dot(mb, n, ties.pop(i, {})))
    for i in range(len(pieces) - STORE_LAG, len(pieces)):
        store(i)
    pltpu.make_async_copy(out_v, out_hbm, sem_o).wait()


def _fused():
    scratch = [
        [pltpu.VMEM(((b - a) // 2, D), i32) for a, b in zip(X_BOUNDS, X_BOUNDS[1:])],
        pltpu.VMEM((S // 2, D), i32),
        [pltpu.VMEM((D // 2, D), i32)] * 3,
        pltpu.VMEM((NT * D // 2 + 32, 128), i32),
        [pltpu.VMEM((D // 2, 128), i32)] * (3 * NT),
        [pltpu.VMEM((D // 2, 128), i32)] * NT,
        [pltpu.VMEM((D // 2, 128), i32)] * NT,
        pltpu.VMEM((F // 2, D), i32),
        pltpu.VMEM((F // 2, D), i32),
        pltpu.VMEM((F // 2, D), i32),
        [pltpu.VMEM((M // 2, D), i32)] * NM,
        [pltpu.VMEM((NT * QS + 24, 128), f32)] * NM,
        [pltpu.VMEM((NT * KS + 16, 128), f32)] * NM,
        [pltpu.VMEM((NT * KS + 16, 128), f32)] * NM,
        [pltpu.VMEM((M // 2, D), i32)] * NM,
        [pltpu.VMEM((32, 128), f32)] * NSTAT,
        [pltpu.VMEM((32, 128), f32)] * NSTAT,
        [pltpu.VMEM((32, 128), f32)] * NSTAT,
        [pltpu.VMEM((32, 128), f32)] * NSTAT,
        [pltpu.VMEM((W * G + 32, 128), f32)] * NP,
        pltpu.VMEM((S, D), bf16),
        [pltpu.VMEM((32, D), i32)] * NSTAT,
        pltpu.VMEM((32, D), i32),
        pltpu.VMEM((64, F), bf16),
        pltpu.VMEM((D,), bf16),
        pltpu.SemaphoreType.DMA((3,)),
        pltpu.SemaphoreType.DMA((12,)),
        pltpu.SemaphoreType.DMA(()),
    ]
    hbm = pl.BlockSpec(memory_space=pltpu.HBM)
    return pl.pallas_call(
        _kernel,
        out_shape=jax.ShapeDtypeStruct((S, D), bf16),
        in_specs=[hbm] * 7,
        out_specs=hbm,
        scratch_shapes=scratch,
        compiler_params=pltpu.CompilerParams(vmem_limit_bytes=100 * 1024 * 1024),
        name="fused",
    )


@jax.jit
def pallas_recurrent_scan__sliding_local_dilated__moe_arch_mod__prompt_kernel(
    A_x: jax.Array,
    A_wqkv: jax.Array,
    A_wo: jax.Array,
    B_x: jax.Array,
    B_w_r: jax.Array,
    B_w_gate: jax.Array,
    B_w_up: jax.Array,
    B_w_down: jax.Array,
):
    del B_x
    out = _fused()(A_x.reshape(S, D), A_wqkv, A_wo, B_w_r, B_w_gate.T, B_w_up.T, B_w_down)
    return out.reshape(1, S, D)
```

```python
import bisect
import collections
import functools
import itertools
import math

import jax
import jax.numpy as jnp
import numpy as np
from jax import lax
from jax.experimental import pallas as pl
from jax.experimental.pallas import tpu as pltpu

S, D, F = 2048, 640, 1728
DH, W, DIL = 20, 8, 2
NT = D // 128
HALO = 16
M = 128
NM = S // M
G = 16
NG = M // G
NSTAT, NP = 32, 8
QS, KS = M + 8, M + HALO
LOG2E = math.log2(math.e)
QSCALE = DH ** -0.5 * LOG2E
MASKED = -1e9 * LOG2E
EPS = float(np.asarray(1e-5, dtype=jnp.bfloat16).astype(np.float32))
f32, bf16, i32 = jnp.float32, jnp.bfloat16, jnp.int32
PLAIN_RHS, TRANSPOSED_RHS = (((1,), (0,)), ((), ())), (((1,), (1,)), ((), ()))

PIECE = M * NT // 4
LATENCY = 130
NF, NV, NX = 2, 5, 6
X_BOUNDS = (0, NF * M, NX * M, S)
WAIT_W, WAIT_X, WAIT_LATE = (0, 8, 44), 16, 144
SELECT_AT, SELECT_GAP, GATHER_GAP = (64, 260, 60), (12, 16, 24), (150, 150, 500)
LN_SPANS = ((NF, NF + 1, WAIT_X, 21), (NF + 1, NX, 21, 40))
LN_START, LN_PHASE, LN_SUM_STEPS = 48, (42, 56, 20, 56, 32, 94, 95), 4
ATT_START, ATT_RATE = 100, (1.0, 1e-6, 1.0, 1.0, 0.87)
QK_LAG, QK_AT, QK_GAP, QK_STORE, EXP_AT, PV_AT, PV_GAP = 2, 86, 19, 190, 224, 244, 20
FFN_CUTS = (0, 1, 3)
LOOSE, EXACT = 400, 1
STORE_LAG, OUT_LAG, WO_LEAD = 2, 4, 20


def _rb(x):
    return x.astype(bf16).astype(f32)


def _pack(x):
    return pltpu.bitcast(x.astype(bf16), i32)


def _unpack(x):
    return pltpu.bitcast(x, bf16)


def _tree(op, xs):
    while len(xs) > 1:
        xs = [op(a, b) for a, b in zip(xs[::2], xs[1::2])] + xs[len(xs) // 2 * 2:]
    return xs[0]


def _kernel(x_hbm, wqkv_hbm, wo_hbm, wr_hbm, wg_hbm, wu_hbm, wd_hbm, out_hbm,
            x_v, z_v, wqkv_raw, wqkv_t, wqkv_p, wo_raw, wo_p, wg_v, wu_v, wd_v, xn_v, q_s, k_s, v_s, o_v,
            m_s, d_s, i_s, f_s, p_s, out_v, d_v, xs_v, hid_v, wr_v, sem_x, sem_w, sem_o):
    x_copies = [pltpu.make_async_copy(x_hbm.at[pl.ds(a, b - a), :], x_v[j].bitcast(bf16), sem_x.at[j])
                for j, (a, b) in enumerate(zip(X_BOUNDS, X_BOUNDS[1:]))]
    qkv_copies = [pltpu.make_async_copy(wqkv_hbm.at[:, pl.ds(p * D, D)], wqkv_raw[p].bitcast(bf16), sem_w.at[p])
                  for p in range(3)]
    late = [(wo_hbm.at[:, pl.ds(t * 128, 128)], wo_raw[t]) for t in range(NT)]
    late += [(wg_hbm, wg_v), (wu_hbm, wu_v), (wd_hbm, wd_v)]
    late_copies = [pltpu.make_async_copy(src, dst.bitcast(bf16), sem_w.at[4 + j]) for j, (src, dst) in enumerate(late)]
    wr_copy = pltpu.make_async_copy(wr_hbm, wr_v, sem_w.at[3])

    written = set()

    def need(*keys):
        assert written.issuperset(keys), keys

    def dma_point(start, wait):
        for c in start:
            c.start()
        for c in wait:
            c.wait()
            written.add(id(c))

    dma_point([wr_copy, x_copies[0], qkv_copies[0]], x_copies[:1])

    lane = lax.broadcasted_iota(i32, (8, 128), 1)
    sub = lax.broadcasted_iota(i32, (8, 128), 0)
    bits = x_v[0][pl.ds(0, 8), pl.ds(0, 128)] >> 16
    zero = (bits * (bits + 1)) & 1
    zero0 = zero[0, 0]
    fresh, folds = itertools.count(1), itertools.count()
    st = dict(folded=[], sums=[], r=[jnp.zeros((8, 128), f32), jnp.zeros((8, 128), f32)])

    def opaque():
        return pl.multiple_of(zero0 * (next(fresh) * 8), 8)

    def after(ref, row=0):
        return pltpu.bitcast(ref[pl.ds(opaque() + row, 8), pl.ds(0, 128)], i32)

    def hold(ref, row):
        if st["go"] is not None:
            ref[pl.ds(row, 8), :] = pltpu.bitcast(st["go"], ref.dtype)

    def x_rows(row, n, cols=slice(None)):
        j = bisect.bisect_right(X_BOUNDS, row) - 1
        need(id(x_copies[j]))
        return _unpack(x_v[j][pl.ds((row - X_BOUNDS[j]) // 2 + opaque(), n // 2), cols]).astype(f32)

    def wide(v):
        return jnp.concatenate([v] * NT, axis=1)

    def get(refs, g):
        need((id(refs), g))
        return refs[g % NSTAT][pl.ds(opaque(), G), :]

    def put(refs, g, v):
        written.add((id(refs), g))
        refs[g % NSTAT][pl.ds(0, G), :] = jnp.broadcast_to(v, (G, 128))
        return after(refs[g % NSTAT])

    def fold(g, then, v):
        ref = f_s[next(folds) % NSTAT]
        ref[pl.ds(0, G), :] = _tree(jnp.add, [v[:, c * 128:(c + 1) * 128] for c in range(NT)])
        st["folded"].append((then, g, ref))
        return after(ref)

    def ln_reduce():
        sums = []
        for then, g, ref in st["folded"]:
            hold(ref, G)
            sums.append((then, g, jnp.sum(ref[pl.ds(opaque(), G), :], axis=1, keepdims=True)))
        st["folded"] = []
        st["sums"].append(sums)

    def ln_finish():
        tokens = [then(g, v) for then, g, v in st["sums"].pop(0)]
        return functools.reduce(jnp.bitwise_or, tokens) if tokens else None

    def ln_mean(g):
        return fold(g, lambda g, v: put(m_s, g, v * (1.0 / D)), x_rows(g * G, G))

    def ln_var(g):
        d = x_rows(g * G, G) - wide(_rb(get(m_s, g)))
        d_v[g % NSTAT].bitcast(bf16)[pl.ds(0, G), :] = d.astype(bf16)
        return fold(g, lambda g, v: put(d_s, g, v * (1.0 / D)), d * d)

    def ln_scale(g):
        hold(d_s[g % NSTAT], G)
        m = get(m_s, g)
        shift = m - _rb(m)
        var = jnp.maximum(get(d_s, g) - shift * shift, 0.0)
        den = jnp.minimum(_rb(jnp.sqrt(_rb(_rb(var) + EPS))), 3e38)
        inv = pltpu.reciprocal(den, approx=True)
        return put(i_s, g, inv * (2.0 - den * inv))

    def ln_norm(g):
        written.add(("xn", g))
        d = _unpack(d_v[g % NSTAT][pl.ds(opaque(), G // 2), :]).astype(f32)
        xn = (d * wide(get(i_s, g))).astype(bf16)
        z_v.bitcast(bf16)[pl.ds(g * G, G), :] = xn
        xn_v[g // NG].bitcast(bf16)[pl.ds(g % NG * G, G), :] = xn
        return after(xn_v[g // NG])

    def keep_score(g, r):
        written.add(("r", g))
        for s in range(G // 8):
            half, l = divmod(g * G // 8 + s, 128)
            st["r"][half] = jnp.where(lane == l, jnp.broadcast_to(r[s * 8:(s + 1) * 8], (8, 128)), st["r"][half])
        return pltpu.bitcast(st["r"][half], i32)

    def ln_dot(g):
        need(("xn", g))
        if g == 0:
            dma_point(qkv_copies[1:2], [wr_copy])
            st["wr"] = wr_v[...].astype(f32).reshape(1, D)
        xn = _unpack(z_v[pl.ds(g * G // 2 + opaque(), G // 2), :])
        return fold(g, keep_score, xn.astype(f32) * st["wr"])

    src_lane = [(20 * (lane & 31) + 5 * (lane >> 5) + c) & 127 for c in range(NT)]
    turn = (130 - lane) * 2
    turn = turn - ((turn * 205) >> 10) * 5
    turns = [(step, turn & step != 0) for step in (1, 2, 4)]

    def select(p, b, z):
        need(id(qkv_copies[p]))
        tiles = [wqkv_raw[p][pl.ds(z + b * 8, 8), pl.ds(t * 128, 128)] for t in range(NT)]
        for step, mask in turns:
            tiles = [jnp.where(mask, tiles[(t + step) % NT], tiles[t]) for t in range(NT)]
        return [tiles[2 * c % NT] for c in range(NT)]

    def gather_lanes(p, c, b, v):
        written.add(("w", p * NT + c))
        wqkv_p[p * NT + c][pl.ds(b * 8, 8), :] = jnp.take_along_axis(v, src_lane[c], axis=1, mode="promise_in_bounds")

    def prep_rush(p):
        z = opaque()
        for b in range(D // 16):
            tiles = select(p, b, z)
            gather_lanes(p, 0, b, tiles[0])
            wqkv_t[pl.ds(D // 2 + b * 8, 8), :] = tiles[1]

    def prep_select(p, j, first):
        z = opaque()
        for b in (2 * j, 2 * j + 1):
            tiles = select(p, b, z)
            for c in range(first, NT):
                wqkv_t[pl.ds(c * D // 2 + b * 8, 8), :] = tiles[c]
        return after(wqkv_t, (NT - 1) * D // 2)

    def prep_gather(p, c):
        hold(wqkv_t, NT * D // 2)
        z = opaque()
        for b in range(D // 16):
            gather_lanes(p, c, b, wqkv_t[pl.ds(z + (c * D // 2 + b * 8), 8), :])

    def wo_permute(t, c):
        need(id(late_copies[t]))
        written.add(("wo", t, c))
        z = opaque()
        for g in range(4):
            word, upper = divmod(5 * g + c, 2)
            even, odd = (wo_raw[t][pl.ds(z + (word + k), 16, stride=DH), :] for k in (0, DH // 2))
            if upper:
                pair = ((even >> 16) & 0xFFFF) | (odd & -0x10000)
            else:
                pair = (even & 0xFFFF) | (odd << 16)
            wo_p[t][pl.ds(c * 64 + g * 16, 16), :] = pair
        return after(wo_p[t])

    def window_pair(ref, z, c, row, w):
        t = ref[pl.ds(z + (row + c * KS + HALO - 8 - DIL * w), G + 8), :]
        return t[8:], t[:G]

    def attn_qk(g, w):
        mb, j = divmod(g, NG)
        need(*[("qkv", b, n) for b in (mb, max(mb - 1, 0)) for n in range(3 * NT)])
        z = opaque()
        if w == 0:
            hold(q_s[mb], M)
            st["q"] = [q_s[mb][pl.ds(z + (c * QS + j * G), G), :] for c in range(NT)]
        else:
            hold(k_s[mb], NT * KS)
        ps = None
        for c in range(NT):
            t = [st["q"][c] * k for k in window_pair(k_s[mb], z, c, j * G, w)]
            ps = t if ps is None else [a + b for a, b in zip(ps, t)]
        st["p", g, w] = [(p, pltpu.roll(p, 64, 1)) for p in ps]

    def attn_qk_store(g, w):
        written.add(("p", g, w))
        for slot, (p, r) in zip((w, w + W // 2), st.pop(("p", g, w))):
            p_s[g % NP][pl.ds(slot * G, G), :] = p + r
        return after(p_s[g % NP])

    def attn_logits(g):
        need(*[("p", g, w) for w in range(W // 2)])
        z = opaque()
        hold(p_s[g % NP], W * G)
        ps = [p_s[g % NP][pl.ds(z + w * G, G), :] for w in range(W)]
        st["l", g] = [p + pltpu.roll(p, 32, 1) for p in ps]

    def attn_softmax(g):
        logits = st.pop(("l", g))
        for w in range(W):
            if g * G < DIL * w:
                pos = g * G + lax.broadcasted_iota(i32, (G, 128), 0)
                logits[w] = jnp.where(pos >= DIL * w, logits[w], MASKED)
        m = _tree(jnp.maximum, logits)
        e = [jnp.exp2(l - m) for l in logits]
        inv = pltpu.reciprocal(_tree(jnp.add, e), approx=True)
        st["e", g] = e, inv
        return pltpu.bitcast(inv[:8], i32) | pltpu.bitcast(inv[8:], i32)

    def attn_pv(g, c):
        written.add(("o", g, c))
        mb, j = divmod(g, NG)
        z = opaque()
        e, inv = st["e", g]
        acc = None
        for w in range(W // 2):
            near, far = window_pair(v_s[mb], z, c, j * G, w)
            t = e[w] * near + e[w + W // 2] * far
            acc = t if acc is None else acc + t
        acc = acc * inv
        token = pltpu.bitcast(acc[:8], i32) | pltpu.bitcast(acc[8:], i32)
        o_v[mb].bitcast(bf16)[pl.ds(j * G, G), pl.ds(c * 128, 128)] = acc.astype(bf16)
        return token

    row = lax.broadcasted_iota(i32, (16, D), 0)

    def tile_of(t):
        return pl.ds(pl.multiple_of((t // 16) * 8, 8), 8)

    def token_of(v):
        return pltpu.bitcast(jnp.broadcast_to(v, (8, 128)), i32)

    def top(k):
        if k == 0:
            need(*[("r", g) for g in range(S // G)])
            st["score"] = _rb(jnp.concatenate(st["r"], axis=0))
            st["pos"] = jnp.concatenate([lane * 8 + sub, (lane + 128) * 8 + sub], axis=0).astype(f32)
            st["key"] = jnp.where(st["score"] == st["score"], st["score"], -jnp.inf)
            st["free"], st["i"] = jnp.full((16, 128), True), []
        if k % 2 == 0:
            st["max"] = jnp.max(st["key"], keepdims=True)
            return token_of(st["max"])
        i = jnp.min(jnp.where((st["key"] == st["max"]) & st["free"], st["pos"], S - 1.0), keepdims=True)
        st["i"].append(i)
        st["free"] = st["pos"] != i
        st["key"] = jnp.where(st["free"], st["key"], -jnp.inf)
        return token_of(i)

    def route():
        written.add("xs")
        st["rs"] = [jnp.sum(jnp.where(st["pos"] == i, st["score"], 0.0), keepdims=True) for i in st["i"]]
        st["t"] = [i.astype(i32)[0, 0] for i in st["i"]]

        def pick(t):
            z = _unpack(z_v[tile_of(t), :]).astype(f32)
            return jnp.sum(jnp.where(row == t % 16, z, 0.0), axis=0, keepdims=True)

        xs = jnp.where(lax.broadcasted_iota(i32, (8, D), 0) == 0, pick(st["t"][0]), pick(st["t"][1]))
        xs_v[pl.ds(0, 8), :] = xs
        return pltpu.bitcast(xs[:, :128], i32) | token_of(st["rs"][0]) | token_of(st["rs"][1])

    def ffn_cols(j):
        return pl.ds(j * 128, min(128, F - j * 128))

    def ffn_tile(key, lhs, ref, j, k, dims):
        need("xs", *map(id, late_copies))
        rhs = _unpack(ref[pl.ds(opaque() + j * 64, min(64, F // 2 - j * 64)), pl.ds(k * 128, 128)])
        part = lax.dot_general(lhs, rhs, dims, preferred_element_type=f32)
        st[key] = st[key] + part if key in st else part

    def ffn_in(key, ref, j, k):
        ffn_tile(key, xs_v[pl.ds(opaque(), 8), pl.ds(k * 128, 128)], ref, j, k, TRANSPOSED_RHS)
        if key == "up" and k == NT - 1:
            gate, up = _rb(st.pop("gate")), _rb(st.pop("up"))
            hid_v[pl.ds(0, 8), ffn_cols(j)] = _rb(_rb(gate * jax.nn.sigmoid(gate)) * up)

    def ffn_down(j, k):
        written.add(("y", j, k))
        ffn_tile(("y", k), hid_v[pl.ds(opaque(), 8), ffn_cols(j)], wd_v, j, k, PLAIN_RHS)

    def scatter():
        need(("y", pl.cdiv(F, 128) - 1, NT - 1))
        y = _rb(jnp.concatenate([st["y", k] for k in range(NT)], axis=1))
        written.add("z")
        for j, t in enumerate(st["t"]):
            upd = _rb(y[j:j + 1] * _rb(jax.nn.sigmoid(st["rs"][j])))
            z = _unpack(z_v[tile_of(t), :]).astype(f32)
            z_v[tile_of(t), :] = _pack(jnp.where(row == t % 16, z + upd, z))

    def piece_dot(lhs_ref, rhs_ref, ties, between=()):
        z = opaque()
        cols = []
        for k in range(NT):
            col = lhs_ref[pl.ds(z, M // 2), pl.ds(k * 128, 128)]
            if any(kk == k for kk, _ in ties):
                parts = [col[r * 8:(r + 1) * 8] for r in range(M // 16)]
                for (kk, r), token in ties.items():
                    if kk == k:
                        parts[r] = parts[r] | (token & zero)
                col = jnp.concatenate(parts, axis=0)
            cols.append(col)
        res = None
        cuts = FFN_CUTS if between else (0,)
        for n, (a, b) in enumerate(zip(cuts, cuts[1:] + (NT,))):
            if n < len(between):
                between[n][0](*between[n][1:])
            lhs = _unpack(jnp.concatenate(cols[a:b], axis=1))
            part = jnp.dot(lhs, _unpack(rhs_ref[pl.ds(z + a * 64, (b - a) * 64), :]), preferred_element_type=f32)
            res = part if res is None else res + part
        return res

    def qkv_dot(mb, n, ties, between):
        need(("w", n), *[("xn", mb * NG + j) for j in range(NG)])
        return piece_dot(xn_v[mb], wqkv_p[n], ties, between)

    def qkv_store(mb, n, res):
        written.add(("qkv", mb, n))
        p, c = divmod(n, NT)
        if p == 0:
            q_s[mb][pl.ds(c * QS, M), :] = res * QSCALE
            return
        dst = (k_s, v_s)[p - 1]
        dst[mb][pl.ds(c * KS + HALO, M), :] = res
        if mb == 0:
            dst[0][pl.ds(c * KS, HALO), :] = jnp.broadcast_to(res[0:1], (HALO, 128))
        if mb + 1 < NM:
            dst[mb + 1][pl.ds(c * KS, HALO), :] = res[M - HALO:]

    def out_dot(mb, c, ties, between):
        need(*[("wo", c, k) for k in range(NT)], *[("o", mb * NG + j, k) for j in range(NG) for k in range(NT)])
        return piece_dot(o_v[mb], wo_p[c], ties)

    def out_store(mb, c, s):
        need("z")
        rows, cols = pl.ds(mb * M, M), pl.ds(c * 128, 128)
        z = _unpack(z_v[pl.ds(mb * M // 2 + opaque(), M // 2), cols]).astype(f32)
        gate = z * pltpu.reciprocal(1.0 + jnp.exp2(z * -LOG2E), approx=True)
        res = x_rows(mb * M, M, cols) + s * gate
        out_v[rows, cols] = res.astype(bf16)
        if mb == NM - 1:
            pltpu.make_async_copy(out_v.at[rows, cols], out_hbm.at[rows, cols], sem_o).start()
        elif c == NT - 1:
            pltpu.make_async_copy(out_v.at[rows, :], out_hbm.at[rows, :], sem_o).start()
        return pltpu.bitcast(res[M - 8:], i32)

    qkv, out = (qkv_dot, qkv_store), (out_dot, out_store)
    pieces = [(qkv, mb, n) for n in range(2 * NT) for mb in range(NF)]
    pieces += [(qkv, mb, n) for mb in range(NF, NV) for n in range(2 * NT)]
    pieces += [(qkv, mb, n) for n in range(2 * NT, 3 * NT) for mb in range(NV)]
    pieces += [(qkv, mb, n) for mb in range(NV, NM) for n in range(3 * NT)]
    nq = len(pieces)
    pieces += [(out, mb, c) for mb in range(NM) for c in range(NT)]
    nf = pl.cdiv(F, 128)
    steps = [(ffn_in, key, ref, j, k) for j in range(nf) for key, ref in (("gate", wg_v), ("up", wu_v))
             for k in range(NT)]
    steps += [(ffn_down, j, k) for j in range(nf) for k in range(NT)]
    ffn = {WAIT_LATE + 1 + i: steps[j:j + len(FFN_CUTS)]
           for i, j in enumerate(range(0, len(steps), len(FFN_CUTS)))}
    busy, start = [0] * 4, []
    for i in range(len(pieces)):
        for k in range(NT):
            if k in FFN_CUTS[:len(ffn.get(i, ()))]:
                busy[busy.index(min(busy))] += 8
            m = busy.index(min(busy))
            start.append(busy[m])
            busy[m] += M
    start = np.reshape(start, (-1, NT)).tolist()
    begin = [0]
    for i in range(1, len(pieces)):
        begin.append(max(start[i][0], min(begin[-1] + PIECE, start[i - 1][-1] + M - 1)))
    tasks = []

    def at(t, limit, fn, *args):
        tasks.append((t, len(tasks), limit, fn, args))

    def piece_at(t):
        return bisect.bisect_right(begin, t) - 1

    def layernorm(lo, hi, t0, t1, sum_steps):
        stages = (ln_mean, ln_var, ln_scale, ln_norm, ln_dot)
        lags = (0, sum_steps + 1, 2 * sum_steps + 2, 2 * sum_steps + 6, 2 * sum_steps + 7)
        groups = (hi - lo) * NG
        n = groups + lags[-1] + sum_steps
        for t in range(n):
            when = [t0 + (t * 100 + phase) * (t1 - t0) // (100 * n) for phase in LN_PHASE]
            for k, fn, tk in zip(lags, stages, when):
                if 0 <= t - k < groups:
                    at(tk, t1 and (260 if fn is ln_scale else EXACT), fn, lo * NG + t - k)
            if t < n - sum_steps:
                at(when[5], t1 and EXACT, ln_reduce)
            if t >= sum_steps:
                at(when[6], t1 and EXACT, ln_finish)

    layernorm(0, NF, 0, 0, 3)
    starts = (x_copies[1:2], qkv_copies[2:], late_copies)
    waits = (qkv_copies[:1], qkv_copies[1:2], (qkv_copies[2], x_copies[2]))
    for p, first in enumerate(WAIT_W):
        t = first * PIECE
        at(t, 0, dma_point, starts[p], waits[p])
        rushed = 2 if p < 2 else 0
        if rushed:
            at(t, 0, prep_rush, p)
            at(t, 0, prep_gather, p, 1)
        for j in range(20):
            at(t + SELECT_AT[p] + j * SELECT_GAP[p], EXACT, prep_select, p, j, rushed)
        for c in range(rushed, NT):
            at(t + SELECT_AT[p] + 20 * SELECT_GAP[p] + (c - rushed) * GATHER_GAP[p], EXACT, prep_gather, p, c)
    at(WAIT_X * PIECE, 0, dma_point, x_copies[2:], x_copies[1:2])
    for lo, hi, first, last in LN_SPANS:
        layernorm(lo, hi, first * PIECE, last * PIECE, LN_SUM_STEPS)
    base = ATT_START * PIECE
    layernorm(NX, NM, LN_START * PIECE, base - 300, LN_SUM_STEPS)
    for k in range(4):
        at(base + k * 400, LOOSE, top, k)
    at(base + 4 * 400, LOOSE, route)

    knots = [base, begin[WAIT_LATE] - 580, begin[WAIT_LATE] - 380, begin[max(ffn)],
             begin[nq] + 600, begin[nq] + 600 + 65 * PIECE]
    work = np.cumsum([0] + [(b - a) * rate for a, b, rate in zip(knots, knots[1:], ATT_RATE)])

    def frame(g):
        return int(np.interp((g + QK_LAG) * work[-1] / (NM * NG + QK_LAG), work, knots))

    for g in range(NM * NG):
        for w in range(W // 2):
            at(frame(g - QK_LAG) + QK_AT + w * QK_GAP, LOOSE, attn_qk, g, w)
            at(frame(g - QK_LAG) + QK_AT + w * QK_GAP + QK_STORE, EXACT, attn_qk_store, g, w)
        at(frame(g), LOOSE, attn_logits, g)
        at(frame(g) + EXP_AT, EXACT, attn_softmax, g)
        for c in range(NT):
            at(frame(g) + PV_AT + c * PV_GAP, EXACT, attn_pv, g, c)
    at(begin[WAIT_LATE], 0, dma_point, [], late_copies)
    for j in range(NT * NT):
        at(begin[nq] - (WO_LEAD * (NT * NT - j) // (NT * NT) + 2) * PIECE, EXACT, wo_permute, *divmod(j, NT))
    at(begin[nq - 2], 0, scatter)

    due = collections.defaultdict(list)
    for task in sorted(tasks, key=lambda task: task[:2]):
        due[piece_at(task[0])].append(task)
    results = []
    ties = collections.defaultdict(dict)

    def result_at(t):
        i = len(results) - 1
        while i >= 0 and start[i][-1] + LATENCY > t:
            i -= 1
        if i < 0:
            return None
        r = min((t - LATENCY - start[i][-1]) // 8, M // 8 - 1)
        return results[i][r * 8:(r + 1) * 8]

    def tie(t, token):
        if token is not None:
            i = piece_at(t)
            k = 0 if t - start[i][0] < M else NT - 1
            key = k, min(max(t - start[i][k], 0) // 16, M // 16 - 1)
            ties[i][key] = ties[i][key] | token if key in ties[i] else token

    def store(i):
        (_, fn), mb, n = pieces[i]
        token = fn(mb, n, results[i])
        if i + OUT_LAG < len(pieces):
            tie(begin[i + OUT_LAG], token)

    for i, ((dot, _), mb, n) in enumerate(pieces):
        for t, _, limit, fn, args in due.pop(i, []):
            st["go"] = result_at(t) if limit else None
            token = fn(*args)
            if limit:
                tie(t + limit, token)
        if i >= STORE_LAG:
            store(i - STORE_LAG)
        results.append(dot(mb, n, ties.pop(i, {}), ffn.get(i, ())))
    for i in range(len(pieces) - STORE_LAG, len(pieces)):
        store(i)
    pltpu.make_async_copy(out_v, out_hbm, sem_o).wait()


def _fused():
    scratch = [
        [pltpu.VMEM(((b - a) // 2, D), i32) for a, b in zip(X_BOUNDS, X_BOUNDS[1:])],
        pltpu.VMEM((S // 2, D), i32),
        [pltpu.VMEM((D // 2, D), i32)] * 3,
        pltpu.VMEM((NT * D // 2 + 32, 128), i32),
        [pltpu.VMEM((D // 2, 128), i32)] * (3 * NT),
        [pltpu.VMEM((D // 2, 128), i32)] * NT,
        [pltpu.VMEM((D // 2, 128), i32)] * NT,
        pltpu.VMEM((F // 2, D), i32),
        pltpu.VMEM((F // 2, D), i32),
        pltpu.VMEM((F // 2, D), i32),
        [pltpu.VMEM((M // 2, D), i32)] * NM,
        [pltpu.VMEM((NT * QS + 24, 128), f32)] * NM,
        [pltpu.VMEM((NT * KS + 16, 128), f32)] * NM,
        [pltpu.VMEM((NT * KS + 16, 128), f32)] * NM,
        [pltpu.VMEM((M // 2, D), i32)] * NM,
        [pltpu.VMEM((32, 128), f32)] * NSTAT,
        [pltpu.VMEM((32, 128), f32)] * NSTAT,
        [pltpu.VMEM((32, 128), f32)] * NSTAT,
        [pltpu.VMEM((32, 128), f32)] * NSTAT,
        [pltpu.VMEM((W * G + 32, 128), f32)] * NP,
        pltpu.VMEM((S, D), bf16),
        [pltpu.VMEM((32, D), i32)] * NSTAT,
        pltpu.VMEM((32, D), f32),
        pltpu.VMEM((32, F), f32),
        pltpu.VMEM((D,), bf16),
        pltpu.SemaphoreType.DMA((3,)),
        pltpu.SemaphoreType.DMA((12,)),
        pltpu.SemaphoreType.DMA(()),
    ]
    hbm = pl.BlockSpec(memory_space=pltpu.HBM)
    return pl.pallas_call(
        _kernel,
        out_shape=jax.ShapeDtypeStruct((S, D), bf16),
        in_specs=[hbm] * 7,
        out_specs=hbm,
        scratch_shapes=scratch,
        compiler_params=pltpu.CompilerParams(vmem_limit_bytes=100 * 1024 * 1024),
        name="fused",
    )


@jax.jit
def pallas_recurrent_scan__sliding_local_dilated__moe_arch_mod__prompt_kernel(
    A_x: jax.Array,
    A_wqkv: jax.Array,
    A_wo: jax.Array,
    B_x: jax.Array,
    B_w_r: jax.Array,
    B_w_gate: jax.Array,
    B_w_up: jax.Array,
    B_w_down: jax.Array,
):
    del B_x
    out = _fused()(A_x.reshape(S, D), A_wqkv, A_wo, B_w_r, B_w_gate.T, B_w_up.T, B_w_down)
    return out.reshape(1, S, D)
```
